```python
import jax
import jax.numpy as jnp

def _softmax(x, axis=-1):
    return jax.nn.softmax(x, axis=axis)

def _gelu(x):
    return jax.nn.gelu(x, approximate=True)

def _silu(x):
    return jax.nn.silu(x)

def _sigmoid(x):
    return jax.nn.sigmoid(x)

def _layernorm(x, axis=-1, eps=1e-05):
    m = jnp.mean(x, axis=axis, keepdims=True)
    v = jnp.var(x, axis=axis, keepdims=True)
    return (x - m) / jnp.sqrt(v + eps)

def _scatter_add(tgt, idx, src, axis=0):
    return tgt.at[idx].add(src)

def _segment_sum(src, seg, n):
    return jax.ops.segment_sum(src, seg, n)

class _Rng:

    def __init__(self, key):
        self._k = key

    def _next(self):
        self._k, sub = jax.random.split(self._k)
        return sub

    def normal(self, shape):
        return jax.random.normal(self._next(), shape, dtype=jnp.bfloat16)

    def randint(self, lo, hi, shape):
        return jax.random.randint(self._next(), shape, lo, hi, dtype=jnp.int32)

    def uniform(self, shape, lo=0.0, hi=1.0):
        return jax.random.uniform(self._next(), shape, jnp.bfloat16, lo, hi)

    def permutation(self, n):
        return jax.random.permutation(self._next(), n)
kernel_name = 'standalone__conformer_family_conformer__speech'

def setup_inputs():
    _rng = _Rng(jax.random.key(int.from_bytes(__import__("os").urandom(4), "little")))
    _w = lambda a: (lambda t: t.astype(jnp.bfloat16) if jnp.issubdtype(t.dtype, jnp.floating) else t)(jnp.asarray(a))
    B, T, D, K = (2, 4000, 512, 15)
    F = 4 * D
    s = D ** (-0.5)
    sf = F ** (-0.5)
    return {'x': _w((lambda *s: _rng.normal(s) * 0.05)(B, T, D)), 'w_ff1_a': _w((lambda *s: _rng.normal(s) * 0.05)(D, F) * s), 'w_ff1_b': _w((lambda *s: _rng.normal(s) * 0.05)(F, D) * sf), 'w_q': _w((lambda *s: _rng.normal(s) * 0.05)(D, D) * s), 'w_k': _w((lambda *s: _rng.normal(s) * 0.05)(D, D) * s), 'w_v': _w((lambda *s: _rng.normal(s) * 0.05)(D, D) * s), 'w_o': _w((lambda *s: _rng.normal(s) * 0.05)(D, D) * s), 'w_pw1': _w((lambda *s: _rng.normal(s) * 0.05)(D, 2 * D) * s), 'dw': _w((lambda *s: _rng.normal(s) * 0.05)(K, D) * K ** (-0.5)), 'w_pw2': _w((lambda *s: _rng.normal(s) * 0.05)(D, D) * s), 'w_ff2_a': _w((lambda *s: _rng.normal(s) * 0.05)(D, F) * s), 'w_ff2_b': _w((lambda *s: _rng.normal(s) * 0.05)(F, D) * sf)}

def reference(x, w_ff1_a, w_ff1_b, w_q, w_k, w_v, w_o, w_pw1, dw, w_pw2, w_ff2_a, w_ff2_b):
    B, T, D = x.shape
    K = dw.shape[0]
    scale = D ** (-0.5)
    h = _layernorm(x, axis=-1)
    h = _silu(h @ w_ff1_a) @ w_ff1_b
    x1 = x + 0.5 * h
    h = _layernorm(x1, axis=-1)
    q = h @ w_q
    k = h @ w_k
    v = h @ w_v
    scores = jnp.einsum('btd,bsd->bts', q, k) * scale
    p = _softmax(scores, axis=-1)
    attn = jnp.einsum('bts,bsd->btd', p, v) @ w_o
    x2 = x1 + attn
    h = _layernorm(x2, axis=-1)
    h = h @ w_pw1
    a = h[..., :D].copy()
    b = h[..., D:].copy()
    h = a * _sigmoid(b)
    pad = K // 2
    hp = jnp.pad(h, ((0, 0), (pad, K - 1 - pad), (0, 0)))
    dc = jnp.zeros_like(h)
    for i in range(K):
        dc = dc + hp[:, i:i + T, :] * dw[i][None, None, :]
    flat = dc.reshape(-1, D)
    mu = flat.mean(0)
    var = ((flat - mu) ** 2).mean(0)
    dc = (dc - mu[None, None, :]) / jnp.sqrt(var[None, None, :] + 1e-05)
    h = _silu(dc) @ w_pw2
    x3 = x2 + h
    h = _layernorm(x3, axis=-1)
    h = _silu(h @ w_ff2_a) @ w_ff2_b
    x4 = x3 + 0.5 * h
    return _layernorm(x4, axis=-1)
```

```python
import functools
import math

import jax
import jax.numpy as jnp
from jax import lax
import jax.experimental.pallas as pl
import jax.experimental.pallas.tpu as pltpu

F32 = jnp.float32
BF16 = jnp.bfloat16
EPS = 1e-5
LOG2E = 1.4426950408889634


def _ln(xf, post):
    m = jnp.mean(xf, axis=-1, keepdims=True)
    xc = xf - m
    v = jnp.mean(xc * xc, axis=-1, keepdims=True)
    r = lax.rsqrt(v + EPS)
    if post != 1.0:
        r = r * post
    return xc * r


def _half_silu(h):
    return h * (1.0 + jnp.tanh(h))


def _dot(a, b):
    return jnp.dot(a, b, preferred_element_type=F32)


def _dot_nt(a, b):
    return lax.dot_general(a, b, (((1,), (1,)), ((), ())), preferred_element_type=F32)


def make_kernel(B, T, D, K, F, TM=400, phases="ABCD", ffc=512):
    TP = (T + 127) // 128 * 128
    NT = T // TM
    NTT = B * NT
    PAD = K // 2
    GH = 8
    scale = D ** -0.5

    def kernel(x_hbm, w1a_hbm, w1b_hbm, wq_hbm, wk_hbm, wv_hbm, wo_hbm, wp1_hbm, dw_hbm, wp2_hbm,
               w2a_hbm, w2b_hbm, o_hbm,
               x_v, w1a, w1b, wq, wk, wv, wo, wp1, dw_v, wp2, w2a, w2b, wqk, wvo,
               res, kbuf, vbuf, gbuf, dcb, obuf, xsem, wsem, osem):
        def xcopy(i):
            return pltpu.make_async_copy(x_hbm.at[pl.ds(i * TM, TM)], x_v.at[pl.ds(i * TM, TM)], xsem.at[i])

        wlist = [(w1a_hbm, w1a), (w1b_hbm, w1b), (wq_hbm, wq), (wk_hbm, wk), (wv_hbm, wv), (wo_hbm, wo),
                 (wp1_hbm, wp1), (dw_hbm, dw_v), (wp2_hbm, wp2), (w2a_hbm, w2a), (w2b_hbm, w2b)]
        wc = [pltpu.make_async_copy(s, d, wsem.at[j]) for j, (s, d) in enumerate(wlist)]
        xcopy(0).start()
        wc[0].start()
        wc[1].start()
        xcopy(1).start()
        for j in (4, 5, 2, 3):
            wc[j].start()
        for i in range(2, NTT):
            xcopy(i).start()
        for j in range(6, 11):
            wc[j].start()

        for b in range(B):
            kbuf[b, T:TP, :] = jnp.zeros((TP - T, D), BF16)
            vbuf[b, T:TP, :] = jnp.zeros((TP - T, D), BF16)
            for c in range(D // 128):
                gbuf[c, b, 0:GH, :] = jnp.zeros((GH, 128), F32)
                gbuf[c, b, GH + T:GH + T + GH, :] = jnp.zeros((GH, 128), F32)

        wc[0].wait()
        wc[1].wait()
        wc[4].wait()
        wc[5].wait()
        wvo[...] = _dot(wv[...], wo[...]).astype(BF16)

        def ff(xn, wa, wb):
            acc = None
            for c in range(F // ffc):
                h = _dot(xn, wa[:, c * ffc:(c + 1) * ffc])
                a = _half_silu(h).astype(BF16)
                y = _dot(a, wb[c * ffc:(c + 1) * ffc, :])
                acc = y if acc is None else acc + y
            return acc

        def phase_a(i, _):
            b = i // NT
            t0 = pl.multiple_of((i - b * NT) * TM, 16)
            r0 = pl.multiple_of(i * TM, 16)
            xcopy(i).wait()
            x = x_v[pl.ds(r0, TM), :].astype(F32)
            xn = _ln(x, 0.5).astype(BF16)
            x1 = x + 0.5 * ff(xn, w1a, w1b)
            res[pl.ds(r0, TM), :] = x1
            hn = _ln(x1, 1.0).astype(BF16)
            kbuf[b, pl.ds(t0, TM), :] = hn
            vbuf[b, pl.ds(t0, TM), :] = _dot(hn, wvo[...]).astype(BF16)

        if "A" in phases:
            lax.fori_loop(0, NTT, phase_a, None)
        else:
            for i in range(NTT):
                xcopy(i).wait()

        wc[2].wait()
        wc[3].wait()
        wqk[...] = (_dot_nt(wq[...], wk[...]) * (scale * LOG2E)).astype(BF16)
        wc[6].wait()
        wc[7].wait()

        def phase_b(i, _):
            b = i // NT
            t0 = pl.multiple_of((i - b * NT) * TM, 16)
            r0 = pl.multiple_of(i * TM, 16)
            q = _dot(kbuf[b, pl.ds(t0, TM), :], wqk[...]).astype(BF16)
            TL = TP - 128
            s0 = _dot_nt(q, kbuf[b, 0:TL, :])
            s1 = _dot_nt(q, kbuf[b, TL:TP, :])
            col = lax.broadcasted_iota(jnp.int32, (TM, 128), 1)
            s1 = jnp.where(col < (T - TL), s1, -jnp.inf)
            m = jnp.maximum(jnp.max(s0, axis=-1, keepdims=True), jnp.max(s1, axis=-1, keepdims=True))
            p0 = jnp.exp2(s0 - m)
            p1 = jnp.exp2(s1 - m)
            l = jnp.sum(p0, axis=-1, keepdims=True) + jnp.sum(p1, axis=-1, keepdims=True)
            o = _dot(p0.astype(BF16), vbuf[b, 0:TL, :]) + _dot(p1.astype(BF16), vbuf[b, TL:TP, :])
            x2 = res[pl.ds(r0, TM), :] + o / l
            res[pl.ds(r0, TM), :] = x2
            xn = _ln(x2, 0.5).astype(BF16)
            ab = _dot(xn, wp1[...])
            g = ab[:, :D] * (1.0 + jnp.tanh(ab[:, D:]))
            for c in range(D // 128):
                gbuf[c, b, pl.ds(GH + t0, TM), :] = g[:, c * 128:(c + 1) * 128]

        if "B" in phases:
            lax.fori_loop(0, NTT, phase_b, None)

        def phase_conv(i, carry):
            s1, s2 = carry
            b = i // NT
            t0 = pl.multiple_of((i - b * NT) * TM, 16)
            r0 = pl.multiple_of(i * TM, 16)
            outs1, outs2 = [], []
            for c in range(D // 128):
                acc = None
                for k in range(K):
                    w = dw_v[k:k + 1, c * 128:(c + 1) * 128].astype(F32)
                    t = gbuf[c, b, pl.ds(t0 + GH - PAD + k, TM), :] * w
                    acc = t if acc is None else acc + t
                dcb[pl.ds(r0, TM), c * 128:(c + 1) * 128] = acc
                outs1.append(jnp.sum(acc.reshape(TM // 8, 8, 128), axis=0))
                outs2.append(jnp.sum((acc * acc).reshape(TM // 8, 8, 128), axis=0))
            return s1 + jnp.concatenate(outs1, axis=1), s2 + jnp.concatenate(outs2, axis=1)

        if "C" in phases:
            s1, s2 = lax.fori_loop(0, NTT, phase_conv, (jnp.zeros((8, D), F32), jnp.zeros((8, D), F32)))
        else:
            s1, s2 = jnp.zeros((8, D), F32), jnp.ones((8, D), F32)
        n = float(B * T)
        mu = jnp.sum(s1, axis=0, keepdims=True) / n
        var = jnp.sum(s2, axis=0, keepdims=True) / n - mu * mu
        hr = 0.5 * lax.rsqrt(var + EPS)

        wc[8].wait()
        wc[9].wait()
        wc[10].wait()

        def ocopy(i, slot):
            return pltpu.make_async_copy(obuf.at[slot], o_hbm.at[pl.ds(pl.multiple_of(i * TM, 16), TM)], osem.at[slot])

        def phase_c(i, _):
            r0 = pl.multiple_of(i * TM, 16)
            slot = i % 2
            z = (dcb[pl.ds(r0, TM), :] - mu) * hr
            a = _half_silu(z).astype(BF16)
            x3 = res[pl.ds(r0, TM), :] + _dot(a, wp2[...])
            xn = _ln(x3, 0.5).astype(BF16)
            x4 = x3 + 0.5 * ff(xn, w2a, w2b)
            out = _ln(x4, 1.0).astype(BF16)

            @pl.when(i >= 2)
            def _():
                ocopy(i - 2, slot).wait()

            obuf[slot] = out
            ocopy(i, slot).start()

        if "D" in phases:
            lax.fori_loop(0, NTT, phase_c, None)
            ocopy(NTT - 2, 0).wait()
            ocopy(NTT - 1, 1).wait()

    def fn(x, w_ff1_a, w_ff1_b, w_q, w_k, w_v, w_o, w_pw1, dw, w_pw2, w_ff2_a, w_ff2_b):
        x2 = x.reshape(B * T, D)
        any_spec = pl.BlockSpec(memory_space=pl.ANY)
        out = pl.pallas_call(
            kernel,
            out_shape=jax.ShapeDtypeStruct((B * T, D), BF16),
            in_specs=[any_spec] * 12,
            out_specs=any_spec,
            scratch_shapes=[
                pltpu.VMEM((B * T, D), BF16),
                pltpu.VMEM((D, F), BF16), pltpu.VMEM((F, D), BF16),
                pltpu.VMEM((D, D), BF16), pltpu.VMEM((D, D), BF16), pltpu.VMEM((D, D), BF16), pltpu.VMEM((D, D), BF16),
                pltpu.VMEM((D, 2 * D), BF16), pltpu.VMEM((K, D), BF16), pltpu.VMEM((D, D), BF16),
                pltpu.VMEM((D, F), BF16), pltpu.VMEM((F, D), BF16),
                pltpu.VMEM((D, D), BF16), pltpu.VMEM((D, D), BF16),
                pltpu.VMEM((B * T, D), F32),
                pltpu.VMEM((B, TP, D), BF16), pltpu.VMEM((B, TP, D), BF16),
                pltpu.VMEM((D // 128, B, T + 2 * GH, 128), F32),
                pltpu.VMEM((B * T, D), F32),
                pltpu.VMEM((2, TM, D), BF16),
                pltpu.SemaphoreType.DMA((NTT,)),
                pltpu.SemaphoreType.DMA((11,)),
                pltpu.SemaphoreType.DMA((2,)),
            ],
            compiler_params=pltpu.CompilerParams(vmem_limit_bytes=120 * 1024 * 1024),
        )(x2, w_ff1_a, w_ff1_b, w_q, w_k, w_v, w_o, w_pw1, dw, w_pw2, w_ff2_a, w_ff2_b)
        return out.reshape(B, T, D)

    return fn


@jax.jit
def pallas_standalone__conformer_family_conformer__speech_kernel(
    x, w_ff1_a, w_ff1_b, w_q, w_k, w_v, w_o, w_pw1, dw, w_pw2, w_ff2_a, w_ff2_b):
    B, T, D = x.shape
    K = dw.shape[0]
    F = w_ff1_a.shape[1]
    return make_kernel(B, T, D, K, F)(
        x, w_ff1_a, w_ff1_b, w_q, w_k, w_v, w_o, w_pw1, dw, w_pw2, w_ff2_a, w_ff2_b)
```

```python
import functools
import math

import jax
import jax.numpy as jnp
from jax import lax
import jax.experimental.pallas as pl
import jax.experimental.pallas.tpu as pltpu

F32 = jnp.float32
BF16 = jnp.bfloat16
EPS = 1e-5
LOG2E = 1.4426950408889634


def _ln(xf, post):
    m = jnp.mean(xf, axis=-1, keepdims=True)
    xc = xf - m
    v = jnp.mean(xc * xc, axis=-1, keepdims=True)
    r = lax.rsqrt(v + EPS)
    if post != 1.0:
        r = r * post
    return xc * r


def _half_silu(h):
    return h * (1.0 + jnp.tanh(h))


def _dot(a, b):
    return jnp.dot(a, b, preferred_element_type=F32)


def _dot_nt(a, b):
    return lax.dot_general(a, b, (((1,), (1,)), ((), ())), preferred_element_type=F32)


def make_kernel(B, T, D, K, F, TM=400, phases="ABD", ffc=512, prewait=False, kc=512, qk_split=5,
                border="alpha", crc=16, cacc=5, cqk=8, do_conv=True, d_split=2, erc=80, qk_tail=0, e0pos=1, brep=0, dbg_aligned=False, dbg_taps=15, scopes=False):
    TP = (T + 127) // 128 * 128
    NT = T // TM
    NTT = B * NT
    assert NTT % 2 == 0 and NTT >= 6
    PAD = K // 2
    GH = 8
    scale = D ** -0.5
    NKC = TP // kc
    ND = D // 128
    NF = F // ffc

    def kernel(x_hbm, w1a_hbm, w1b_hbm, wq_hbm, wk_hbm, wv_hbm, wo_hbm, wp1_hbm, dw_hbm, wp2_hbm,
               w2a_hbm, w2b_hbm, o_hbm,
               x_v, w1a, w1b, wq, wk, wv, wo, wp1, dw_v, wp2, w2a, w2b, wqv, dwb,
               res, qbuf, kbuf, vbuf, gd,
               sbuf, pbuf, lbuf, mbuf, xnA, xnB, hA, hB, fA, fB, gA, gB, stat, obuf,
               xsem, wsem, osem):
        def rows(i):
            if isinstance(i, int):
                return pl.ds(i * TM, TM)
            return pl.ds(pl.multiple_of(i * TM, 16), TM)

        def bt(i):
            if isinstance(i, int):
                return i // NT, (i % NT) * TM
            b = lax.div(i, NT)
            return b, pl.multiple_of((i - b * NT) * TM, 16)

        def clamp_hi(i):
            if isinstance(i, int):
                return min(i, NTT - 1)
            return jnp.minimum(i, NTT - 1)

        def clamp_lo(i):
            if isinstance(i, int):
                return max(i, 0)
            return jnp.maximum(i, 0)

        XS = 2
        xc0 = pltpu.make_async_copy(x_hbm.at[pl.ds(0, XS * TM)], x_v.at[pl.ds(0, XS * TM)], xsem.at[0])
        xc1 = pltpu.make_async_copy(x_hbm.at[pl.ds(XS * TM, (NTT - XS) * TM)],
                                    x_v.at[pl.ds(XS * TM, (NTT - XS) * TM)], xsem.at[1])
        wlist = [(wq_hbm, wq), (wk_hbm, wk), (wv_hbm, wv), (wo_hbm, wo), (w1a_hbm, w1a), (w1b_hbm, w1b),
                 (wp1_hbm, wp1), (dw_hbm, dw_v), (wp2_hbm, wp2), (w2a_hbm, w2a), (w2b_hbm, w2b)]
        wc = [pltpu.make_async_copy(s, d, wsem.at[j]) for j, (s, d) in enumerate(wlist)]
        wc[0].start()
        wc[1].start()
        xc0.start()
        for j in (2, 3, 4, 5):
            wc[j].start()
        xc1.start()
        for j in range(6, 11):
            wc[j].start()

        if prewait:
            xc0.wait()
            xc1.wait()
            for j in range(11):
                wc[j].wait()

            class _C:
                def wait(self): pass
            wc = [_C() for _ in range(11)]
            xc0 = xc1 = _C()

        for b in range(B):
            kbuf[b, T:TP, :] = jnp.zeros((TP - T, D), BF16)
            vbuf[b, T:TP, :] = jnp.zeros((TP - T, D), BF16)
            for c in range(ND):
                gd[0, c, b, 0:GH, :] = jnp.zeros((GH, 128), F32)
                gd[0, c, b, GH + T:GH + T + GH, :] = jnp.zeros((GH, 128), F32)
        stat[...] = jnp.zeros(stat.shape, F32)

        def ff_chunk(xn_ref, wa, wb, c):
            h = _dot(xn_ref[...], wa[:, c * ffc:(c + 1) * ffc])
            a = _half_silu(h).astype(BF16)
            return _dot(a, wb[c * ffc:(c + 1) * ffc, :])

        def a_ln1(i, xn_w):
            xn_w[...] = _ln(x_v[rows(i), :].astype(F32), 0.5).astype(BF16)

        def a_ff(i, xn_r, h_w):
            y = None
            for c in range(NF):
                t = ff_chunk(xn_r, w1a, w1b, c)
                y = t if y is None else y + t
            x1 = x_v[rows(i), :].astype(F32) + 0.5 * y
            res[rows(i), :] = x1
            b, t0 = bt(i)
            hn = _ln(x1, 1.0).astype(BF16)
            kbuf[b, pl.ds(t0, TM), :] = hn
            if h_w is not None:
                h_w[...] = hn
            return hn

        def a_qv(i, hn):
            b, t0 = bt(i)
            qv = _dot(hn, wqv[...]).astype(BF16)
            qbuf[rows(i), :] = qv[:, :D]
            vbuf[b, pl.ds(t0, TM), :] = qv[:, D:]

        wc[0].wait()
        wc[1].wait()
        wqv[:, :D] = (_dot_nt(wq[...], wk[...]) * (scale * LOG2E)).astype(BF16)
        xc0.wait()
        a_ln1(0, xnA)
        wc[2].wait()
        wc[3].wait()
        wqv[:, D:] = _dot(wv[...], wo[...]).astype(BF16)
        wc[4].wait()
        wc[5].wait()

        def a_half(i, xn_r, xn_w, h_r, h_w, first=False, last=False):
            if not last:
                a_ln1(i + 1, xn_w)
            hn = a_ff(i, xn_r, None if last else h_w)
            if not first:
                a_qv(i - 1, h_r[...])
            if last:
                a_qv(i, hn)

        if "A" in phases:
            a_half(0, xnA, xnB, hB, hA, first=True)
            xc1.wait()

            def a_pair(p, _):
                i = 2 * p + 1
                a_half(i, xnB, xnA, hA, hB)
                a_half(i + 1, xnA, xnB, hB, hA)
            lax.fori_loop(0, (NTT - 2) // 2, a_pair, None)
            a_half(NTT - 1, xnB, xnA, hA, hB, last=True)
        else:
            xc1.wait()

        wc[6].wait()
        wc[7].wait()
        for k in range(K):
            dwb[k] = jnp.broadcast_to(dw_v[k:k + 1, :].astype(F32), (8, D))

        def kslice(j):
            return slice(j * kc, (j + 1) * kc)

        def lane_fold(v, op):
            r = v[:, 0:128]
            for c in range(1, v.shape[1] // 128):
                r = op(r, v[:, c * 128:(c + 1) * 128])
            return r

        def seed_of(t, tpos):
            n_, r_ = tpos // TM, (tpos % TM) // 8 * 8
            return t[r_:r_ + 8, n_ * 128:(n_ + 1) * 128]

        def b_qk(i, j, w):
            b, _ = bt(i)
            s = _dot_nt(qbuf[rows(i), :], kbuf[b, kslice(j), :])
            raw = s
            if (j + 1) * kc > T:
                col = lax.broadcasted_iota(jnp.int32, (TM, kc), 1)
                s = jnp.where(col < (T - j * kc), s, -jnp.inf)
            sbuf[w, 0:TM, kslice(j)] = s
            return lane_fold(s, jnp.maximum), raw

        def b_glu(i, xn):
            b, t0 = bt(i)
            ab = _dot(xn, wp1[...])
            g = ab[:, :D] * (1.0 + jnp.tanh(ab[:, D:]))
            for c in range(ND):
                gd[0, c, b, pl.ds(GH + t0, TM), :] = g[:, c * 128:(c + 1) * 128]

        def conv_pieces(i, valid=None):
            b, t0 = bt(i)
            st = {}

            def piece(c, rc, seed=None):
                cs = slice(c * 128, (c + 1) * 128)
                if seed is not None:
                    gd[1, 0, b, 0:8, :] = seed
                accs = [None] * cacc
                for k in range(K):
                    w = dwb[k, :, cs]
                    t = gd[0, c, b, pl.ds(t0 + GH - PAD + k + rc, crc), :]
                    t = t.reshape(crc // 8, 8, 128) * w[None]
                    accs[k % cacc] = t if accs[k % cacc] is None else accs[k % cacc] + t
                while len(accs) > 1:
                    accs = [accs[u] + accs[u + 1] if u + 1 < len(accs) else accs[u] for u in range(0, len(accs), 2)]
                acc = accs[0]
                gd[1, c, b, pl.ds(GH + t0 + rc, crc), :] = acc.reshape(crc, 128)
                a1 = jnp.sum(acc, axis=0)
                a2 = jnp.sum(acc * acc, axis=0)
                if rc == 0:
                    st[c] = (a1, a2)
                else:
                    st[c] = (st[c][0] + a1, st[c][1] + a2)
                if rc + crc == TM:
                    s1, s2 = st[c]
                    if valid is not None:
                        s1 = jnp.where(valid, s1, 0.0)
                        s2 = jnp.where(valid, s2, 0.0)
                    stat[0, :, cs] += s1
                    stat[1, :, cs] += s2

            return [functools.partial(piece, c, rc) for c in range(ND) for rc in range(0, TM, crc)]

        def conv(i):
            for p_ in conv_pieces(i):
                p_()

        nq = TM // erc

        def lsum(r, j, rs):
            t = lane_fold(pbuf[rs, kslice(j)].astype(F32), jnp.add)
            if j == 0:
                lbuf[r, rs, :] = t
            else:
                lbuf[r, rs, :] += t

        def exp_piece(r, z, m, j, q, seed):
            rs = slice(q * erc, (q + 1) * erc)
            if seed is not None:
                sbuf[r, pl.ds(pl.multiple_of(TM + 8 * z, 8), 8), 0:128] = seed
            p = jnp.exp2(sbuf[r, rs, kslice(j)] - m[rs])
            pbuf[rs, kslice(j)] = p.astype(BF16)
            lsum(r, j, rs)

        def spread(t, items, phase):
            n = len(items)
            for q, f in enumerate(items):
                f(seed_of(t, (q * ND * TM) // n + phase * (ND * TM) // (2 * n)))

        def b_tile(i, r, w, do_next=True, conv_on=True):
            b, _ = bt(i)
            pcs = []
            if conv_on and do_conv:
                if isinstance(i, int):
                    if i >= 2:
                        pcs = conv_pieces(i - 2)
                else:
                    pcs = conv_pieces(clamp_lo(i - 2), valid=(i >= 2))
            if scopes: sc_ = jax.named_scope("s_qk1"); sc_.__enter__()
            m = mbuf[r]
            z = 0 if isinstance(i, int) else lax.shift_right_logical(i, 20)
            mp = None
            if do_next:
                for j in range(qk_split):
                    t, raw = b_qk(i + 1, j, w)
                    mp = t if mp is None else jnp.maximum(mp, t)
                    if j == qk_split - 1 - e0pos:
                        spread(raw, [functools.partial(exp_piece, r, z, m, 0, q) for q in range(nq)], 0)
                    elif cqk and pcs:
                        take = [pcs.pop(0) for _ in range(min(cqk, len(pcs)))]
                        spread(raw, take, 1)
            else:
                for q in range(nq):
                    exp_piece(r, z, m, 0, q, None)
            if scopes: sc_.__exit__(None, None, None)
            o = None
            if scopes: sc_ = jax.named_scope("s_pv"); sc_.__enter__()
            for j in range(NKC):
                t = _dot(pbuf[0:TM, kslice(j)], vbuf[b, kslice(j), :])
                o = t if o is None else o + t
                npc = (len(pcs) + NKC - 1 - j) // (NKC - j) if pcs else 0
                evs = []
                if j + 1 < NKC:
                    for q in range(nq):
                        evs.append(((q * ND * TM) // nq, 0, q))
                for q in range(npc):
                    evs.append(((q * ND * TM) // npc + (ND * TM) // (2 * npc), 1, q))
                evs.sort()
                for tpos, kind, q in evs:
                    seed = seed_of(t, tpos)
                    if kind == 0:
                        exp_piece(r, z, m, j + 1, q, seed)
                    else:
                        pcs.pop(0)(seed)
            if scopes: sc_.__exit__(None, None, None); sc_ = jax.named_scope("s_rest"); sc_.__enter__()
            l = jnp.sum(lbuf[r], axis=-1, keepdims=True)
            x2 = res[rows(i), :] + o * (1.0 / l)
            res[rows(i), :] = x2
            xn = _ln(x2, 0.5).astype(BF16)
            if do_next:
                for j in range(qk_split, NKC - qk_tail):
                    t, _ = b_qk(i + 1, j, w)
                    mp = t if mp is None else jnp.maximum(mp, t)
            b_glu(i, xn)
            if do_next:
                for j in range(NKC - qk_tail, NKC):
                    t, _ = b_qk(i + 1, j, w)
                    mp = t if mp is None else jnp.maximum(mp, t)
                mbuf[w] = jnp.max(mp, axis=-1, keepdims=True)
            if scopes: sc_.__exit__(None, None, None)

        if "B" in phases:
            mp = None
            for j in range(NKC):
                t, _ = b_qk(0, j, 0)
                mp = t if mp is None else jnp.maximum(mp, t)
            mbuf[0] = jnp.max(mp, axis=-1, keepdims=True)

            def b_iter(i, _):
                r = lax.rem(i, 2)
                b_tile(i, r, 1 - r)
            lax.fori_loop(0, NTT - 1, b_iter, None)
            for _r in range(brep):
                lax.fori_loop(0, NTT - 1, b_iter, None)
            b_tile(NTT - 1, (NTT - 1) % 2, NTT % 2, do_next=False)
            if do_conv:
                conv(NTT - 2)
                conv(NTT - 1)

        n = float(B * T)
        mu = jnp.sum(stat[0], axis=0, keepdims=True) / n
        var = jnp.sum(stat[1], axis=0, keepdims=True) / n - mu * mu
        hr = 0.5 * lax.rsqrt(var + EPS)

        wc[8].wait()
        wc[9].wait()
        wc[10].wait()

        def ocopy(i, slot):
            return pltpu.make_async_copy(obuf.at[slot], o_hbm.at[rows(i)], osem.at[slot])

        def d_act(i, a_w):
            b, t0 = bt(i)
            dcv = jnp.concatenate([gd[1, c, b, pl.ds(GH + t0, TM), :] for c in range(ND)], axis=1)
            z = (dcv - mu) * hr
            a_w[...] = _half_silu(z).astype(BF16)

        def d_pw2(i, a_r, f_w, xn_w):
            x3 = res[rows(i), :] + _dot(a_r[...], wp2[...])
            f_w[...] = x3
            xn_w[...] = _ln(x3, 0.5).astype(BF16)

        def d_fin(x4, slot):
            obuf[slot] = _ln(x4, 1.0).astype(BF16)

        def d_half(i, slot, a_r, a_w, f_r, f_w, xn_r, xn_w, g_r, g_w, last=False, first_dyn=True):
            if isinstance(i, int):
                if i >= 3:
                    ocopy(i - 3, slot).wait()
            else:
                @pl.when(i >= 3)
                def _():
                    ocopy(i - 3, slot).wait()
            d_fin(g_r[...], slot)
            if not last:
                d_act(clamp_hi(i + 2), a_w)
            y = None
            for c in range(NF):
                if c == d_split and not last:
                    d_pw2(i + 1, a_r, f_w, xn_w)
                t = ff_chunk(xn_r, w2a, w2b, c)
                y = t if y is None else y + t
            x4 = f_r[...] + 0.5 * y
            if last:
                return x4
            g_w[...] = x4
            if isinstance(i, int):
                if i >= 1:
                    ocopy(i - 1, slot).start()
            else:
                @pl.when(i >= 1)
                def _():
                    ocopy(i - 1, slot).start()

        if "D" in phases:
            gB[...] = jnp.zeros(gB.shape, F32)
            d_act(0, hA)
            d_pw2(0, hA, fA, xnA)
            d_act(1, hB)

            def d_pair(p, _):
                i = 2 * p
                d_half(i, 1, hB, hA, fA, fB, xnA, xnB, gB, gA)
                d_half(i + 1, 0, hA, hB, fB, fA, xnB, xnA, gA, gB)
            lax.fori_loop(0, NTT // 2 - 1, d_pair, None)
            i = NTT - 2
            d_half(i, 1, hB, hA, fA, fB, xnA, xnB, gB, gA)
            ocopy(NTT - 2 - 1, 1).start() if False else None
            x4 = d_half(i + 1, 0, hA, hB, fB, fA, xnB, xnA, gA, gB, last=True)
            ocopy(NTT - 2, 0).start()
            ocopy(NTT - 3, 1).wait()
            d_fin(x4, 1)
            ocopy(NTT - 1, 1).start()
            ocopy(NTT - 2, 0).wait()
            ocopy(NTT - 1, 1).wait()
        else:
            obuf[0] = x_v[0:TM, :]
            ocopy(0, 0).start()
            ocopy(0, 0).wait()

    def fn(x, w_ff1_a, w_ff1_b, w_q, w_k, w_v, w_o, w_pw1, dw, w_pw2, w_ff2_a, w_ff2_b):
        x2 = x.reshape(B * T, D)
        any_spec = pl.BlockSpec(memory_space=pl.ANY)
        V = pltpu.VMEM
        out = pl.pallas_call(
            kernel,
            out_shape=jax.ShapeDtypeStruct((B * T, D), BF16),
            in_specs=[any_spec] * 12,
            out_specs=any_spec,
            scratch_shapes=[
                V((B * T, D), BF16),
                V((D, F), BF16), V((F, D), BF16),
                V((D, D), BF16), V((D, D), BF16), V((D, D), BF16), V((D, D), BF16),
                V((D, 2 * D), BF16), V((K, D), BF16), V((D, D), BF16),
                V((D, F), BF16), V((F, D), BF16),
                V((D, 2 * D), BF16),
                V((K, 8, D), F32),
                V((B * T, D), F32),
                V((B * T, D), BF16),
                V((B, TP, D), BF16), V((B, TP, D), BF16),
                V((2, ND, B, T + 2 * GH, 128), F32),
                V((2, TM + 8, TP), F32),
                V((TM, TP), BF16),
                V((2, TM, 128), F32),
                V((2, TM, 1), F32),
                V((TM, D), BF16), V((TM, D), BF16),
                V((TM, D), BF16), V((TM, D), BF16),
                V((TM, D), F32), V((TM, D), F32),
                V((TM, D), F32), V((TM, D), F32),
                V((2, 8, D), F32),
                V((2, TM, D), BF16),
                pltpu.SemaphoreType.DMA((2,)),
                pltpu.SemaphoreType.DMA((11,)),
                pltpu.SemaphoreType.DMA((2,)),
            ],
            compiler_params=pltpu.CompilerParams(vmem_limit_bytes=127 * 1024 * 1024),
        )(x2, w_ff1_a, w_ff1_b, w_q, w_k, w_v, w_o, w_pw1, dw, w_pw2, w_ff2_a, w_ff2_b)
        return out.reshape(B, T, D)

    return fn


@jax.jit
def pallas_standalone__conformer_family_conformer__speech_kernel(
    x, w_ff1_a, w_ff1_b, w_q, w_k, w_v, w_o, w_pw1, dw, w_pw2, w_ff2_a, w_ff2_b):
    B, T, D = x.shape
    K = dw.shape[0]
    F = w_ff1_a.shape[1]
    return make_kernel(B, T, D, K, F)(
        x, w_ff1_a, w_ff1_b, w_q, w_k, w_v, w_o, w_pw1, dw, w_pw2, w_ff2_a, w_ff2_b)
```

```python
import functools
import math
import numpy as np

import jax
import jax.numpy as jnp
from jax import lax
import jax.experimental.pallas as pl
import jax.experimental.pallas.tpu as pltpu

F32 = jnp.float32
BF16 = jnp.bfloat16
EPS = 1e-5
LOG2E = 1.4426950408889634


def _ln(xf, post):
    m = jnp.mean(xf, axis=-1, keepdims=True)
    xc = xf - m
    v = jnp.mean(xc * xc, axis=-1, keepdims=True)
    r = lax.rsqrt(v + EPS)
    if post != 1.0:
        r = r * post
    return xc * r


def _half_silu(h):
    return h * (1.0 + jnp.tanh(h))


U32 = jnp.uint32


def _pk(v):
    return pltpu.bitcast(v, U32)


def _un(v):
    return pltpu.bitcast(v, BF16)


def _dot(a, b):
    return jnp.dot(a, b, preferred_element_type=F32)


def _dot_nt(a, b):
    return lax.dot_general(a, b, (((1,), (1,)), ((), ())), preferred_element_type=F32)


def make_kernel(B, T, D, K, F, TM=400, phases="ABD", ffc=512, prewait=False, kc=512, qk_split=5,
                border="alpha", crc=16, cacc=5, aseed=True, arc=80, aplan=(1,1,1,1,1), dseed=True, drc=80, dplan=(1,1,1,1,1,1,1,1), cplan=(0,0,0,0,0, 1,1,1,1,1,1,1,1, 0,0,0, 0,0), cplan_last=(1,1,1,1,1,1,1,1), do_conv=True, d_split=2, erc=16, qk_tail=0, e0pos=1, brep=0, dbg_aligned=False, dbg_taps=15, scopes=False):
    TP = (T + 127) // 128 * 128
    NT = T // TM
    NTT = B * NT
    assert NTT % 2 == 0 and NTT >= 6
    PAD = K // 2
    GH = 8
    scale = D ** -0.5
    NKC = TP // kc
    ND = D // 128
    NF = F // ffc

    def kernel(x_hbm, w1a_hbm, w1b_hbm, wq_hbm, wk_hbm, wv_hbm, wo_hbm, wp1_hbm, dw_hbm, wp2_hbm,
               w2a_hbm, w2b_hbm, o_hbm,
               x_v, w1a, w1b, wq, wk, wv, wo, wp1, dw_v, wp2, w2a, w2b, wqv, dwb,
               res, qbuf, kbuf, vbuf, gd,
               sbuf, pbuf, lbuf, mbuf, xnA, xnB, hA, hB, fA, fB, gA, gB, stat, obuf,
               xsem, wsem, osem):
        def rows(i):
            if isinstance(i, int):
                return pl.ds(i * TM, TM)
            return pl.ds(pl.multiple_of(i * TM, 16), TM)

        def hrows(i):
            if isinstance(i, int):
                return pl.ds(i * (TM // 2), TM // 2)
            return pl.ds(pl.multiple_of(i * (TM // 2), 8), TM // 2)

        def bt(i):
            if isinstance(i, int):
                return i // NT, (i % NT) * TM
            b = lax.div(i, NT)
            return b, pl.multiple_of((i - b * NT) * TM, 16)

        def clamp_hi(i):
            if isinstance(i, int):
                return min(i, NTT - 1)
            return jnp.minimum(i, NTT - 1)

        def clamp_lo(i):
            if isinstance(i, int):
                return max(i, 0)
            return jnp.maximum(i, 0)

        def xcp(t0_, t1_, k_):
            return pltpu.make_async_copy(x_hbm.at[pl.ds(t0_ * TM, (t1_ - t0_) * TM)],
                                         x_v.at[pl.ds(t0_ * TM, (t1_ - t0_) * TM)], xsem.at[k_])
        xc0, xc1, xc2 = xcp(0, 1, 0), xcp(1, 3, 1), xcp(3, NTT, 2)
        wlist = [(wq_hbm, wq), (wk_hbm, wk), (wv_hbm, wv), (wo_hbm, wo), (w1a_hbm, w1a), (w1b_hbm, w1b),
                 (wp1_hbm, wp1), (dw_hbm, dw_v), (wp2_hbm, wp2), (w2a_hbm, w2a), (w2b_hbm, w2b)]
        wc = [pltpu.make_async_copy(s, d, wsem.at[j]) for j, (s, d) in enumerate(wlist)]
        def scope(name):
            class _S:
                def __enter__(self_):
                    if scopes: self_.s = jax.named_scope(name); self_.s.__enter__()
                def __exit__(self_, *a):
                    if scopes: self_.s.__exit__(*a)
            return _S()

        sc0 = scope("s_0start"); sc0.__enter__()
        wc[0].start()
        wc[1].start()
        xc0.start()
        wc[2].start()
        wc[3].start()
        wc[4].start()
        wc[5].start()
        xc1.start()
        xc2.start()
        for j in range(6, 11):
            wc[j].start()

        if prewait:
            xc0.wait()
            xc1.wait()
            xc2.wait()
            for j in range(11):
                wc[j].wait()

            class _C:
                def wait(self): pass
            wc = [_C() for _ in range(11)]
            xc0 = xc1 = xc2 = _C()

        for b in range(B):
            kbuf[b, T // 2:TP // 2, :] = jnp.zeros(((TP - T) // 2, D), U32)
            vbuf[b, T // 2:TP // 2, :] = jnp.zeros(((TP - T) // 2, D), U32)
            for c in range(ND):
                gd[0, c, b, 0:GH, :] = jnp.zeros((GH, 128), F32)
                gd[0, c, b, GH + T:GH + T + GH, :] = jnp.zeros((GH, 128), F32)
        stat[...] = jnp.zeros(stat.shape, F32)

        def seed_of(t, tpos):
            n_, r_ = tpos // TM, (tpos % TM) // 8 * 8
            return t[r_:r_ + 8, n_ * 128:(n_ + 1) * 128]

        class Releaser:
            def __init__(self, pieces, plan):
                self.pieces, self.cum, self.k = list(pieces), np.cumsum([0] + list(plan)), 0
                self.n = len(self.pieces)

            def __call__(self, t):
                k0 = self.k
                self.k += 1
                if self.k >= len(self.cum):
                    return
                tot = int(self.cum[-1])
                n = int(self.cum[k0 + 1]) * self.n // tot - int(self.cum[k0]) * self.n // tot
                span = t.shape[1] // 128 * TM
                for q in range(n):
                    self.pieces.pop(0)(seed_of(t, (2 * q + 1) * span // (2 * n)))

        def ff_chunk(xn_ref, wa, wb, c, rel=None):
            h = _dot(_un(xn_ref[...]), wa[:, c * ffc:(c + 1) * ffc])
            if rel is not None:
                rel(h)
            a = _half_silu(h).astype(BF16)
            y = _dot(a, wb[c * ffc:(c + 1) * ffc, :])
            if rel is not None:
                rel(y)
            return y

        def a_ln1(i, xn_w):
            xn_w[...] = _pk(_ln(x_v[rows(i), :].astype(F32), 0.5).astype(BF16))

        def a_ln1_pieces(i, xn_w):
            z = 0 if isinstance(i, int) else lax.shift_right_logical(i, 20)
            r0 = i * TM if isinstance(i, int) else pl.multiple_of(i * TM, 16)

            def piece(q, seed):
                if seed is not None:
                    x_v[pl.ds(pl.multiple_of(B * T + 16 * z, 16), 16), 0:128] = pltpu.bitcast(seed, BF16)
                rs = pl.ds(r0 + q * arc, arc)
                xn_w[q * arc // 2:(q + 1) * arc // 2, :] = _pk(_ln(x_v[rs, :].astype(F32), 0.5).astype(BF16))
            return [functools.partial(piece, q) for q in range(TM // arc)]

        def a_ff(i, xn_r, h_w, rel=None):
            y = None
            for c in range(NF):
                t = ff_chunk(xn_r, w1a, w1b, c, rel)
                y = t if y is None else y + t
            x1 = x_v[rows(i), :].astype(F32) + 0.5 * y
            res[rows(i), :] = x1
            b, t0 = bt(i)
            hn = _pk(_ln(x1, 1.0).astype(BF16))
            h0 = t0 // 2 if isinstance(t0, int) else pl.multiple_of(lax.shift_right_logical(t0, 1), 8)
            kbuf[b, pl.ds(h0, TM // 2), :] = hn
            if h_w is not None:
                h_w[...] = hn
            return hn

        def a_qv(i, hn):
            b, t0 = bt(i)
            qv = _pk(_dot(_un(hn), _un(wqv[...])).astype(BF16))
            h0 = t0 // 2 if isinstance(t0, int) else pl.multiple_of(lax.shift_right_logical(t0, 1), 8)
            qbuf[hrows(i), :] = qv[:, :D]
            vbuf[b, pl.ds(h0, TM // 2), :] = qv[:, D:]

        hB[...] = jnp.zeros(hB.shape, U32)
        wc[0].wait()
        wc[1].wait()
        wqv[:, :D] = _pk((_dot_nt(wq[...], wk[...]) * (scale * LOG2E)).astype(BF16))
        xc0.wait()
        a_ln1(0, xnA)
        wc[2].wait()
        wc[3].wait()
        wqv[:, D:] = _pk(_dot(wv[...], wo[...]).astype(BF16))
        wc[4].wait()
        wc[5].wait()
        xc1.wait()

        def a_half(i, xn_r, xn_w, h_r, h_w):
            rel = Releaser(a_ln1_pieces(clamp_hi(i + 1), xn_w), aplan)
            a_ff(i, xn_r, h_w, rel)
            a_qv(clamp_lo(i - 1), h_r[...])

        sc0.__exit__(None, None, None)
        if "A" in phases:
            def a_pair(p, _):
                @pl.when(p == 1)
                def _():
                    xc2.wait()
                i = 2 * p
                a_half(i, xnA, xnB, hB, hA)
                a_half(i + 1, xnB, xnA, hA, hB)
            with scope("s_3aloop"):
                lax.fori_loop(0, NTT // 2, a_pair, None)
            with scope("s_4alast"):
                a_qv(NTT - 1, hB[...])
        else:
            xc2.wait()

        wc[6].wait()
        wc[7].wait()
        for k in range(K):
            dwb[k] = jnp.broadcast_to(dw_v[k:k + 1, :].astype(F32), (8, D))

        def kslice(j):
            return slice(j * kc, (j + 1) * kc)

        def hslice(j):
            return slice(j * kc // 2, (j + 1) * kc // 2)

        def lane_fold(v, op):
            r = v[:, 0:128]
            for c in range(1, v.shape[1] // 128):
                r = op(r, v[:, c * 128:(c + 1) * 128])
            return r

        def b_qk(i, j, w):
            b, _ = bt(i)
            s = _dot_nt(_un(qbuf[hrows(i), :]), _un(kbuf[b, hslice(j), :]))
            raw = s
            if (j + 1) * kc > T:
                col = lax.broadcasted_iota(jnp.int32, (TM, kc), 1)
                s = jnp.where(col < (T - j * kc), s, -jnp.inf)
            sbuf[w, 0:TM, kslice(j)] = s
            return lane_fold(s, jnp.maximum), raw

        def b_glu(i, xn):
            b, t0 = bt(i)
            ab = _dot(xn, wp1[...])
            g = ab[:, :D] * (1.0 + jnp.tanh(ab[:, D:]))
            for c in range(ND):
                gd[0, c, b, pl.ds(GH + t0, TM), :] = g[:, c * 128:(c + 1) * 128]

        def conv_pieces(i, valid=None):
            b, t0 = bt(i)
            st = {}

            def piece(c, rc, seed=None):
                cs = slice(c * 128, (c + 1) * 128)
                if seed is not None:
                    gd[1, 0, b, 0:8, :] = seed
                accs = [None] * cacc
                for k in range(K):
                    w = dwb[k, :, cs]
                    t = gd[0, c, b, pl.ds(t0 + GH - PAD + k + rc, crc), :]
                    t = t.reshape(crc // 8, 8, 128) * w[None]
                    accs[k % cacc] = t if accs[k % cacc] is None else accs[k % cacc] + t
                while len(accs) > 1:
                    accs = [accs[u] + accs[u + 1] if u + 1 < len(accs) else accs[u] for u in range(0, len(accs), 2)]
                acc = accs[0]
                gd[1, c, b, pl.ds(GH + t0 + rc, crc), :] = acc.reshape(crc, 128)
                a1 = jnp.sum(acc, axis=0)
                a2 = jnp.sum(acc * acc, axis=0)
                if rc == 0:
                    st[c] = (a1, a2)
                else:
                    st[c] = (st[c][0] + a1, st[c][1] + a2)
                if rc + crc == TM:
                    s1, s2 = st[c]
                    if valid is not None:
                        s1 = jnp.where(valid, s1, 0.0)
                        s2 = jnp.where(valid, s2, 0.0)
                    stat[0, :, cs] += s1
                    stat[1, :, cs] += s2

            return [functools.partial(piece, c, rc) for c in range(ND) for rc in range(0, TM, crc)]

        def conv(i):
            for p_ in conv_pieces(i):
                p_()

        nq = TM // erc

        def lsum(r, j, rs):
            t = lane_fold(_un(pbuf[rs.start // 2:rs.stop // 2, kslice(j)]).astype(F32), jnp.add)
            if j == 0:
                lbuf[r, rs, :] = t
            else:
                lbuf[r, rs, :] += t

        def exp_piece(r, z, m, j, q, seed):
            rs = slice(q * erc, (q + 1) * erc)
            if seed is not None:
                sbuf[r, pl.ds(pl.multiple_of(TM + 8 * z, 8), 8), 0:128] = seed
            p = jnp.exp2(sbuf[r, rs, kslice(j)] - m[rs])
            pbuf[rs.start // 2:rs.stop // 2, kslice(j)] = _pk(p.astype(BF16))
            lsum(r, j, rs)

        def spread(t, items, phase):
            n = len(items)
            for q, f in enumerate(items):
                f(seed_of(t, (q * ND * TM) // n + phase * (ND * TM) // (2 * n)))

        def b_tile(i, r, w, do_next=True, conv_on=True):
            b, _ = bt(i)
            pcs = []
            if conv_on and do_conv:
                if isinstance(i, int):
                    if i >= 2:
                        pcs = conv_pieces(i - 2)
                else:
                    pcs = conv_pieces(clamp_lo(i - 2), valid=(i >= 2))
            m = mbuf[r]
            z = 0 if isinstance(i, int) else lax.shift_right_logical(i, 20)
            eps_ = {j: [functools.partial(exp_piece, r, z, m, j, q) for q in range(nq)] for j in range(NKC)}
            plan = list(cplan) if do_next else [0] * qk_split + list(cplan_last) + [0] * (NKC - qk_split) + [0, 0]
            tot = sum(plan)
            npcs = len(pcs)
            cum = [0]
            for v in plan:
                cum.append(cum[-1] + v)
            site = [0]

            def release(t, exps=()):
                k0 = site[0]
                site[0] += 1
                n = (cum[k0 + 1] * npcs) // tot - (cum[k0] * npcs) // tot if npcs else 0
                items = [(q * ND * TM // n + ND * TM // (2 * n), 1, pcs.pop(0)) for q in range(n)]
                ne = len(exps)
                items += [(q * ND * TM // ne, 0, f_) for q, f_ in enumerate(exps)]
                items.sort(key=lambda u: u[:2])
                for tpos, _k, f_ in items:
                    f_(seed_of(t, tpos))

            mp = None
            if do_next:
                for j in range(qk_split):
                    t, raw = b_qk(i + 1, j, w)
                    mp = t if mp is None else jnp.maximum(mp, t)
                    release(raw, eps_[0] if j == qk_split - 1 - e0pos else ())
            else:
                site[0] = qk_split
                for f_ in eps_[0]:
                    f_(None)
            o = None
            for j in range(NKC):
                t = _dot(_un(pbuf[:, kslice(j)]), _un(vbuf[b, hslice(j), :]))
                o = t if o is None else o + t
                release(t, eps_[j + 1] if j + 1 < NKC else ())
            l = jnp.sum(lbuf[r], axis=-1, keepdims=True)
            x2 = res[rows(i), :] + o * (1.0 / l)
            res[rows(i), :] = x2
            xn = _ln(x2, 0.5).astype(BF16)
            if do_next:
                for j in range(qk_split, NKC):
                    t, raw = b_qk(i + 1, j, w)
                    mp = t if mp is None else jnp.maximum(mp, t)
                    release(raw)
            else:
                site[0] = NKC + NKC
            bb, t0 = bt(i)
            a_ = _dot(xn, wp1[:, :D])
            release(a_)
            b_ = _dot(xn, wp1[:, D:])
            release(b_)
            g = a_ * (1.0 + jnp.tanh(b_))
            for c in range(ND):
                gd[0, c, bb, pl.ds(GH + t0, TM), :] = g[:, c * 128:(c + 1) * 128]
            assert not pcs
            if do_next:
                mbuf[w] = jnp.max(mp, axis=-1, keepdims=True)

        scb = scope("s_5B"); scb.__enter__()
        if "B" in phases:
            mp = None
            for j in range(NKC):
                t, _ = b_qk(0, j, 0)
                mp = t if mp is None else jnp.maximum(mp, t)
            mbuf[0] = jnp.max(mp, axis=-1, keepdims=True)

            def b_iter(i, _):
                r = lax.rem(i, 2)
                b_tile(i, r, 1 - r)
            lax.fori_loop(0, NTT - 1, b_iter, None)
            for _r in range(brep):
                lax.fori_loop(0, NTT - 1, b_iter, None)
            b_tile(NTT - 1, (NTT - 1) % 2, NTT % 2, do_next=False)
            if do_conv:
                lax.fori_loop(NTT - 2, NTT, lambda i_, _: conv(i_), None)

        scb.__exit__(None, None, None)
        scd = scope("s_6D"); scd.__enter__()
        n = float(B * T)
        mu = jnp.sum(stat[0], axis=0, keepdims=True) / n
        var = jnp.sum(stat[1], axis=0, keepdims=True) / n - mu * mu
        hr = 0.5 * lax.rsqrt(var + EPS)

        wc[8].wait()
        wc[9].wait()
        wc[10].wait()

        def ocopy(i, slot):
            return pltpu.make_async_copy(obuf.at[slot], o_hbm.at[rows(i)], osem.at[slot])

        def d_act_pieces(i, a_w):
            b, t0 = bt(i)
            z = 0 if isinstance(i, int) else lax.shift_right_logical(i, 20)

            def piece(q, seed):
                if seed is not None:
                    gd[0, 0, B - 1, pl.ds(pl.multiple_of(T + 2 * GH + 8 * z, 8), 8), :] = seed
                dcv = jnp.concatenate([gd[1, c, b, pl.ds(GH + t0 + q * drc, drc), :] for c in range(ND)], axis=1)
                a_w[q * drc // 2:(q + 1) * drc // 2, :] = _pk(_half_silu((dcv - mu) * hr).astype(BF16))
            return [functools.partial(piece, q) for q in range(TM // drc)]

        def d_act(i, a_w):
            for p_ in d_act_pieces(i, a_w):
                p_(None)

        def d_fin_pieces(i, g_r, slot):
            z = 0 if isinstance(i, int) else lax.shift_right_logical(i, 20)

            def piece(q, seed):
                if seed is not None:
                    g_r[pl.ds(pl.multiple_of(TM + 8 * z, 8), 8), 0:128] = seed
                rs = slice(q * drc, (q + 1) * drc)
                obuf[slot, rs, :] = _ln(g_r[rs, :], 1.0).astype(BF16)
            return [functools.partial(piece, q) for q in range(TM // drc)]

        def d_pw2(i, a_r, f_w, xn_w):
            x3 = res[rows(i), :] + _dot(_un(a_r[...]), wp2[...])
            f_w[...] = x3
            xn_w[...] = _pk(_ln(x3, 0.5).astype(BF16))

        def d_fin(x4, slot):
            obuf[slot] = _ln(x4, 1.0).astype(BF16)

        def d_half(i, slot, a_r, a_w, f_r, f_w, xn_r, xn_w, g_r, g_w, last=False, first_dyn=True):
            if isinstance(i, int):
                if i >= 3:
                    ocopy(i - 3, slot).wait()
            else:
                @pl.when(i >= 3)
                def _():
                    ocopy(i - 3, slot).wait()
            fins = d_fin_pieces(i, g_r, slot)
            acts = d_act_pieces(clamp_hi(i + 2), a_w) if not last else []
            mix = []
            for q in range(max(len(fins), len(acts))):
                mix += fins[q:q + 1] + acts[q:q + 1]
            rel = Releaser(mix, dplan)
            if not dseed:
                for p_ in mix:
                    p_(None)
                rel = None
            y = None
            for c in range(NF):
                if c == d_split and not last:
                    d_pw2(clamp_hi(i + 1), a_r, f_w, xn_w)
                t = ff_chunk(xn_r, w2a, w2b, c, rel)
                y = t if y is None else y + t
            x4 = f_r[...] + 0.5 * y
            if last:
                return x4
            g_w[0:TM, :] = x4
            if isinstance(i, int):
                if i >= 1:
                    ocopy(i - 1, slot).start()
            else:
                @pl.when(i >= 1)
                def _():
                    ocopy(i - 1, slot).start()

        if "D" in phases:
            gB[...] = jnp.zeros(gB.shape, F32)
            d_act(0, hA)
            d_pw2(0, hA, fA, xnA)
            d_act(1, hB)

            def d_pair(p, _):
                i = 2 * p
                d_half(i, 1, hB, hA, fA, fB, xnA, xnB, gB, gA)
                d_half(i + 1, 0, hA, hB, fB, fA, xnB, xnA, gA, gB)
            lax.fori_loop(0, NTT // 2, d_pair, None)
            ocopy(NTT - 3, 1).wait()
            d_fin(gB[0:TM, :], 1)
            ocopy(NTT - 1, 1).start()
            ocopy(NTT - 2, 0).wait()
            ocopy(NTT - 1, 1).wait()
        else:
            obuf[0] = x_v[0:TM, :].astype(obuf.dtype)
            ocopy(0, 0).start()
            ocopy(0, 0).wait()
        scd.__exit__(None, None, None)

    def fn(x, w_ff1_a, w_ff1_b, w_q, w_k, w_v, w_o, w_pw1, dw, w_pw2, w_ff2_a, w_ff2_b):
        x2 = x.reshape(B * T, D)
        any_spec = pl.BlockSpec(memory_space=pl.ANY)
        V = pltpu.VMEM
        out = pl.pallas_call(
            kernel,
            out_shape=jax.ShapeDtypeStruct((B * T, D), BF16),
            in_specs=[any_spec] * 12,
            out_specs=any_spec,
            scratch_shapes=[
                V((B * T + 16, D), BF16),
                V((D, F), BF16), V((F, D), BF16),
                V((D, D), BF16), V((D, D), BF16), V((D, D), BF16), V((D, D), BF16),
                V((D, 2 * D), BF16), V((K, D), BF16), V((D, D), BF16),
                V((D, F), BF16), V((F, D), BF16),
                V((D // 2, 2 * D), U32),
                V((K, 8, D), F32),
                V((B * T, D), F32),
                V((B * T // 2, D), U32),
                V((B, TP // 2, D), U32), V((B, TP // 2, D), U32),
                V((2, ND, B, T + 2 * GH + 16, 128), F32),
                V((2, TM + 8, TP), F32),
                V((TM // 2, TP), U32),
                V((2, TM, 128), F32),
                V((2, TM, 1), F32),
                V((TM // 2, D), U32), V((TM // 2, D), U32),
                V((TM // 2, D), U32), V((TM // 2, D), U32),
                V((TM, D), F32), V((TM, D), F32),
                V((TM + 16, D), F32), V((TM + 16, D), F32),
                V((2, 8, D), F32),
                V((2, TM, D), BF16),
                pltpu.SemaphoreType.DMA((2,)),
                pltpu.SemaphoreType.DMA((11,)),
                pltpu.SemaphoreType.DMA((2,)),
            ],
            compiler_params=pltpu.CompilerParams(vmem_limit_bytes=127 * 1024 * 1024),
        )(x2, w_ff1_a, w_ff1_b, w_q, w_k, w_v, w_o, w_pw1, dw, w_pw2, w_ff2_a, w_ff2_b)
        return out.reshape(B, T, D)

    return fn


@jax.jit
def pallas_standalone__conformer_family_conformer__speech_kernel(
    x, w_ff1_a, w_ff1_b, w_q, w_k, w_v, w_o, w_pw1, dw, w_pw2, w_ff2_a, w_ff2_b):
    B, T, D = x.shape
    K = dw.shape[0]
    F = w_ff1_a.shape[1]
    return make_kernel(B, T, D, K, F)(
        x, w_ff1_a, w_ff1_b, w_q, w_k, w_v, w_o, w_pw1, dw, w_pw2, w_ff2_a, w_ff2_b)
```

```python
import functools
import math
import numpy as np

import jax
import jax.numpy as jnp
from jax import lax
import jax.experimental.pallas as pl
import jax.experimental.pallas.tpu as pltpu

F32 = jnp.float32
BF16 = jnp.bfloat16
EPS = 1e-5
LOG2E = 1.4426950408889634


def _ln(xf, post):
    m = jnp.mean(xf, axis=-1, keepdims=True)
    xc = xf - m
    v = jnp.mean(xc * xc, axis=-1, keepdims=True)
    r = lax.rsqrt(v + EPS)
    if post != 1.0:
        r = r * post
    return xc * r


def _half_silu(h):
    return h * (1.0 + jnp.tanh(h))


U32 = jnp.uint32


def _pk(v):
    return pltpu.bitcast(v, U32)


def _un(v):
    return pltpu.bitcast(v, BF16)


def _dot(a, b):
    return jnp.dot(a, b, preferred_element_type=F32)


def _dot_nt(a, b):
    return lax.dot_general(a, b, (((1,), (1,)), ((), ())), preferred_element_type=F32)


def make_kernel(B, T, D, K, F, TM=400, phases="ABD", ffc=512, prewait=False, kc=512, qk_split=5,
                border="alpha", crc=16, cacc=5, aseed=True, arc=80, ln2span=2400, aplan=(1,1,1,1,1), dseed=True, drc=80, dplan=(2,2,2,2,2,2,2,1), cplan=(0,0,0,0,0, 1,1,1,1,1,1,1,1, 0,0,0, 0,0), cplan_last=(1,1,1,1,1,1,1,1), do_conv=True, d_split=2, erc=16, qk_tail=0, e0pos=1, brep=0, dbg_aligned=False, dbg_taps=15, scopes=False):
    TP = (T + 127) // 128 * 128
    NT = T // TM
    NTT = B * NT
    assert NTT % 2 == 0 and NTT >= 6
    PAD = K // 2
    GH = 8
    scale = D ** -0.5
    NKC = TP // kc
    ND = D // 128
    NF = F // ffc

    def kernel(x_hbm, w1a_hbm, w1b_hbm, wq_hbm, wk_hbm, wv_hbm, wo_hbm, wp1_hbm, dw_hbm, wp2_hbm,
               w2a_hbm, w2b_hbm, o_hbm,
               x_v, w1a, w1b, wq, wk, wv, wo, wp1, dw_v, wp2, w2a, w2b, wqv, dwb,
               res, qbuf, kbuf, vbuf, gd,
               sbuf, pbuf, lbuf, mbuf, xnS, hS, xnA, xnB, hA, hB, fA, fB, gA, gB, stat, obuf,
               xsem, wsem, osem):
        def rows(i):
            if isinstance(i, int):
                return pl.ds(i * TM, TM)
            return pl.ds(pl.multiple_of(i * TM, 16), TM)

        def hrows(i):
            if isinstance(i, int):
                return pl.ds(i * (TM // 2), TM // 2)
            return pl.ds(pl.multiple_of(i * (TM // 2), 8), TM // 2)

        def bt(i):
            if isinstance(i, int):
                return i // NT, (i % NT) * TM
            b = lax.div(i, NT)
            return b, pl.multiple_of((i - b * NT) * TM, 16)

        def clamp_hi(i):
            if isinstance(i, int):
                return min(i, NTT - 1)
            return jnp.minimum(i, NTT - 1)

        def clamp_lo(i):
            if isinstance(i, int):
                return max(i, 0)
            return jnp.maximum(i, 0)

        def xcp(t0_, t1_, k_):
            return pltpu.make_async_copy(x_hbm.at[pl.ds(t0_ * TM, (t1_ - t0_) * TM)],
                                         x_v.at[pl.ds(t0_ * TM, (t1_ - t0_) * TM)], xsem.at[k_])
        xc0, xc1, xc2, xc3 = xcp(0, 1, 0), xcp(1, 2, 1), xcp(2, 4, 2), xcp(4, NTT, 3)
        wlist = [(wq_hbm, wq), (wk_hbm, wk), (wv_hbm, wv), (wo_hbm, wo), (w1a_hbm, w1a), (w1b_hbm, w1b),
                 (wp1_hbm, wp1), (dw_hbm, dw_v), (wp2_hbm, wp2), (w2a_hbm, w2a), (w2b_hbm, w2b)]
        wc = [pltpu.make_async_copy(s_, d_, wsem.at[j]) for j, (s_, d_) in enumerate(wlist)]
        w1ac = [pltpu.make_async_copy(w1a_hbm.at[:, cs_], w1a.at[:, cs_], wsem.at[11 + c])
                for c in range(NF) for cs_ in [pl.ds(c * ffc, ffc)]]
        w1bc = [pltpu.make_async_copy(w1b_hbm.at[cs_, :], w1b.at[cs_, :], wsem.at[11 + NF + c])
                for c in range(NF) for cs_ in [pl.ds(c * ffc, ffc)]]

        def scope(name):
            class _S:
                def __enter__(self_):
                    if scopes: self_.s = jax.named_scope(name); self_.s.__enter__()
                def __exit__(self_, *a):
                    if scopes: self_.s.__exit__(*a)
            return _S()

        sc0 = scope("s_0start"); sc0.__enter__()
        late = wc[6:11]
        if not prewait:
            xc0.start()
            w1ac[0].start()
            w1bc[0].start()
        else:
            for c_ in [xc0, xc1, xc2, xc3] + w1ac + w1bc + wc[:4] + wc[6:]:
                c_.start()

        if prewait:
            allc = [xc0, xc1, xc2, xc3] + w1ac + w1bc + wc[:4] + wc[6:]
            for c_ in allc:
                c_.wait()

            class _C:
                def wait(self): pass
                def start(self): pass
            wc = [_C() for _ in range(11)]
            late = []
            xc0 = xc1 = xc2 = xc3 = _C()
            w1ac = [_C() for _ in range(NF)]
            w1bc = [_C() for _ in range(NF)]

        for b in range(B):
            kbuf[b, T // 2:TP // 2, :] = jnp.zeros(((TP - T) // 2, D), U32)
            vbuf[b, T // 2:TP // 2, :] = jnp.zeros(((TP - T) // 2, D), U32)
            for c in range(ND):
                gd[0, c, b, 0:GH, :] = jnp.zeros((GH, 128), F32)
                gd[0, c, b, GH + T:GH + T + GH, :] = jnp.zeros((GH, 128), F32)
        stat[...] = jnp.zeros(stat.shape, F32)

        def seed_of(t, tpos):
            n_, r_ = tpos // TM, (tpos % TM) // 8 * 8
            return t[r_:r_ + 8, n_ * 128:(n_ + 1) * 128]

        class Releaser:
            def __init__(self, pieces, plan, exact=False):
                self.pieces, self.cum, self.k = list(pieces), np.cumsum([0] + list(plan)), 0
                self.n = int(self.cum[-1]) if exact else len(self.pieces)

            def __call__(self, t):
                k0 = self.k
                self.k += 1
                if self.k >= len(self.cum):
                    return
                tot = int(self.cum[-1])
                n = int(self.cum[k0 + 1]) * self.n // tot - int(self.cum[k0]) * self.n // tot
                span = t.shape[1] // 128 * TM
                for q in range(n):
                    self.pieces.pop(0)(seed_of(t, (2 * q + 1) * span // (2 * n)))

        def ff_chunk(xn_ref, wa, wb, c, rel=None):
            h = _dot(_un(xn_ref[...]), wa[:, c * ffc:(c + 1) * ffc])
            if rel is not None:
                rel(h)
            a = _half_silu(h).astype(BF16)
            y = _dot(a, wb[c * ffc:(c + 1) * ffc, :])
            if rel is not None:
                rel(y)
            return y

        def a_ln1(i, sl):
            xnS[sl] = _pk(_ln(x_v[rows(i), :].astype(F32), 0.5).astype(BF16))

        def a_ln1_pieces(i, sl):
            z = 0 if isinstance(i, int) else lax.shift_right_logical(i, 20)
            r0 = i * TM if isinstance(i, int) else pl.multiple_of(i * TM, 16)

            def piece(q, seed):
                if seed is not None:
                    x_v[pl.ds(pl.multiple_of(B * T + 16 * z, 16), 16), 0:128] = pltpu.bitcast(seed, BF16)
                rs = pl.ds(r0 + q * arc, arc)
                xnS[sl, q * arc // 2:(q + 1) * arc // 2, :] = _pk(_ln(x_v[rs, :].astype(F32), 0.5).astype(BF16))
            return [functools.partial(piece, q) for q in range(TM // arc)]

        def a_ff(i, sl, rel, waits=False, mid=None):
            y = None
            for c in range(NF):
                if waits:
                    w1ac[c].wait()
                    for c_ in ([w1ac[c + 1]] if c + 1 < NF else [wc[0], wc[1]]):
                        c_.start()
                h = _dot(_un(xnS[sl]), w1a[:, c * ffc:(c + 1) * ffc])
                rel(h)
                a = _half_silu(h).astype(BF16)
                if waits:
                    w1bc[c].wait()
                    for c_ in ([w1bc[c + 1]] if c + 1 < NF else [wc[2], wc[3], xc2]):
                        c_.start()
                t = _dot(a, w1b[c * ffc:(c + 1) * ffc, :])
                rel(t)
                y = t if y is None else y + t
            res[rows(i), :] = x_v[rows(i), :].astype(F32) + 0.5 * y
            b, t0 = bt(i)
            h0 = t0 // 2 if isinstance(t0, int) else pl.multiple_of(lax.shift_right_logical(t0, 1), 8)
            z = 0 if isinstance(i, int) else lax.shift_right_logical(i, 20)
            r0 = i * TM if isinstance(i, int) else pl.multiple_of(i * TM, 16)

            def ln2(q, seed):
                if seed is not None:
                    res[pl.ds(pl.multiple_of(B * T + 8 * z, 8), 8), 0:128] = seed
                hn = _pk(_ln(res[pl.ds(r0 + q * arc, arc), :], 1.0).astype(BF16))
                kbuf[b, pl.ds(h0 + q * arc // 2, arc // 2), :] = hn
                hS[sl, q * arc // 2:(q + 1) * arc // 2, :] = hn
            pieces = [functools.partial(ln2, q) for q in range(TM // arc)]
            if mid is not None:
                t = mid()
                for q, f_ in enumerate(pieces):
                    f_(seed_of(t, ln2span * q // len(pieces)))
            else:
                for f_ in pieces:
                    f_(None)

        def a_qv(i, hn):
            b, t0 = bt(i)
            raw = _dot(_un(hn), _un(wqv[...]))
            qv = _pk(raw.astype(BF16))
            h0 = t0 // 2 if isinstance(t0, int) else pl.multiple_of(lax.shift_right_logical(t0, 1), 8)
            qbuf[hrows(i), :] = qv[:, :D]
            vbuf[b, pl.ds(h0, TM // 2), :] = qv[:, D:]
            return raw

        xc0.wait()
        xc1.start()
        a_ln1(0, 0)
        sc0.__exit__(None, None, None)
        if "A" in phases:
            with scope("s_1a0"):
                xc1.wait()
                a_ff(0, 0, Releaser(a_ln1_pieces(1, 1), aplan), waits=True)
                wc[0].wait()
                wc[1].wait()
                wqv[:, :D] = _pk((_dot_nt(wq[...], wk[...]) * (scale * LOG2E)).astype(BF16))
                wc[2].wait()
                wc[3].wait()
                xc3.start()
                wqv[:, D:] = _pk(_dot(wv[...], wo[...]).astype(BF16))
                xc2.wait()

            def a_iter(i, _):
                @pl.when(i == 3)
                def _():
                    xc3.wait()
                    for c_ in late:
                        c_.start()
                sl = lax.rem(i, 2)
                a_ff(i, sl, Releaser(a_ln1_pieces(clamp_hi(i + 1), 1 - sl), aplan),
                     mid=lambda: a_qv(i - 1, hS[1 - sl]))
            with scope("s_3aloop"):
                lax.fori_loop(1, NTT, a_iter, None)
            with scope("s_4alast"):
                a_qv(NTT - 1, hS[(NTT - 1) % 2])
        else:
            if not prewait:
                for c_ in [xc2, xc3] + w1ac[1:] + w1bc[1:] + wc[:4] + late:
                    c_.start()
            for c_ in [xc1, xc2, xc3] + w1ac + w1bc + wc[:4]:
                c_.wait()

        wc[6].wait()
        wc[7].wait()
        for k in range(K):
            dwb[k] = jnp.broadcast_to(dw_v[k:k + 1, :].astype(F32), (8, D))

        def kslice(j):
            return slice(j * kc, (j + 1) * kc)

        def hslice(j):
            return slice(j * kc // 2, (j + 1) * kc // 2)

        def lane_fold(v, op):
            r = v[:, 0:128]
            for c in range(1, v.shape[1] // 128):
                r = op(r, v[:, c * 128:(c + 1) * 128])
            return r

        def b_qk(i, j, w):
            b, _ = bt(i)
            s = _dot_nt(_un(qbuf[hrows(i), :]), _un(kbuf[b, hslice(j), :]))
            raw = s
            if (j + 1) * kc > T:
                col = lax.broadcasted_iota(jnp.int32, (TM, kc), 1)
                s = jnp.where(col < (T - j * kc), s, -jnp.inf)
            sbuf[w, 0:TM, kslice(j)] = s
            return lane_fold(s, jnp.maximum), raw

        def b_glu(i, xn):
            b, t0 = bt(i)
            ab = _dot(xn, wp1[...])
            g = ab[:, :D] * (1.0 + jnp.tanh(ab[:, D:]))
            for c in range(ND):
                gd[0, c, b, pl.ds(GH + t0, TM), :] = g[:, c * 128:(c + 1) * 128]

        def conv_pieces(i, valid=None):
            b, t0 = bt(i)
            st = {}

            def piece(c, rc, seed=None):
                cs = slice(c * 128, (c + 1) * 128)
                if seed is not None:
                    gd[1, 0, b, 0:8, :] = seed
                accs = [None] * cacc
                for k in range(K):
                    w = dwb[k, :, cs]
                    t = gd[0, c, b, pl.ds(t0 + GH - PAD + k + rc, crc), :]
                    t = t.reshape(crc // 8, 8, 128) * w[None]
                    accs[k % cacc] = t if accs[k % cacc] is None else accs[k % cacc] + t
                while len(accs) > 1:
                    accs = [accs[u] + accs[u + 1] if u + 1 < len(accs) else accs[u] for u in range(0, len(accs), 2)]
                acc = accs[0]
                gd[1, c, b, pl.ds(GH + t0 + rc, crc), :] = acc.reshape(crc, 128)
                a1 = jnp.sum(acc, axis=0)
                a2 = jnp.sum(acc * acc, axis=0)
                if rc == 0:
                    st[c] = (a1, a2)
                else:
                    st[c] = (st[c][0] + a1, st[c][1] + a2)
                if rc + crc == TM:
                    s1, s2 = st[c]
                    if valid is not None:
                        s1 = jnp.where(valid, s1, 0.0)
                        s2 = jnp.where(valid, s2, 0.0)
                    stat[0, :, cs] += s1
                    stat[1, :, cs] += s2

            return [functools.partial(piece, c, rc) for c in range(ND) for rc in range(0, TM, crc)]

        def conv(i):
            for p_ in conv_pieces(i):
                p_()

        nq = TM // erc

        def lsum(r, j, rs):
            t = lane_fold(_un(pbuf[rs.start // 2:rs.stop // 2, kslice(j)]).astype(F32), jnp.add)
            if j == 0:
                lbuf[r, rs, :] = t
            else:
                lbuf[r, rs, :] += t

        def exp_piece(r, z, m, j, q, seed):
            rs = slice(q * erc, (q + 1) * erc)
            if seed is not None:
                sbuf[r, pl.ds(pl.multiple_of(TM + 8 * z, 8), 8), 0:128] = seed
            p = jnp.exp2(sbuf[r, rs, kslice(j)] - m[rs])
            pbuf[rs.start // 2:rs.stop // 2, kslice(j)] = _pk(p.astype(BF16))
            lsum(r, j, rs)

        def spread(t, items, phase):
            n = len(items)
            for q, f in enumerate(items):
                f(seed_of(t, (q * ND * TM) // n + phase * (ND * TM) // (2 * n)))

        def b_tile(i, r, w, do_next=True, conv_on=True):
            b, _ = bt(i)
            pcs = []
            if conv_on and do_conv:
                if isinstance(i, int):
                    if i >= 2:
                        pcs = conv_pieces(i - 2)
                else:
                    pcs = conv_pieces(clamp_lo(i - 2), valid=(i >= 2))
            m = mbuf[r]
            z = 0 if isinstance(i, int) else lax.shift_right_logical(i, 20)
            eps_ = {j: [functools.partial(exp_piece, r, z, m, j, q) for q in range(nq)] for j in range(NKC)}
            plan = list(cplan) if do_next else [0] * qk_split + list(cplan_last) + [0] * (NKC - qk_split) + [0, 0]
            tot = sum(plan)
            npcs = len(pcs)
            cum = [0]
            for v in plan:
                cum.append(cum[-1] + v)
            site = [0]

            def release(t, exps=()):
                k0 = site[0]
                site[0] += 1
                n = (cum[k0 + 1] * npcs) // tot - (cum[k0] * npcs) // tot if npcs else 0
                items = [(q * ND * TM // n + ND * TM // (2 * n), 1, pcs.pop(0)) for q in range(n)]
                ne = len(exps)
                items += [(q * ND * TM // ne, 0, f_) for q, f_ in enumerate(exps)]
                items.sort(key=lambda u: u[:2])
                for tpos, _k, f_ in items:
                    f_(seed_of(t, tpos))

            mp = None
            if do_next:
                for j in range(qk_split):
                    t, raw = b_qk(i + 1, j, w)
                    mp = t if mp is None else jnp.maximum(mp, t)
                    release(raw, eps_[0] if j == qk_split - 1 - e0pos else ())
            else:
                site[0] = qk_split
                for f_ in eps_[0]:
                    f_(None)
            o = None
            for j in range(NKC):
                t = _dot(_un(pbuf[:, kslice(j)]), _un(vbuf[b, hslice(j), :]))
                o = t if o is None else o + t
                release(t, eps_[j + 1] if j + 1 < NKC else ())
            l = jnp.sum(lbuf[r], axis=-1, keepdims=True)
            x2 = res[rows(i), :] + o * (1.0 / l)
            res[rows(i), :] = x2
            xn = _ln(x2, 0.5).astype(BF16)
            if do_next:
                for j in range(qk_split, NKC):
                    t, raw = b_qk(i + 1, j, w)
                    mp = t if mp is None else jnp.maximum(mp, t)
                    release(raw)
            else:
                site[0] = NKC + NKC
            bb, t0 = bt(i)
            a_ = _dot(xn, wp1[:, :D])
            release(a_)
            b_ = _dot(xn, wp1[:, D:])
            release(b_)
            g = a_ * (1.0 + jnp.tanh(b_))
            for c in range(ND):
                gd[0, c, bb, pl.ds(GH + t0, TM), :] = g[:, c * 128:(c + 1) * 128]
            assert not pcs
            if do_next:
                mbuf[w] = jnp.max(mp, axis=-1, keepdims=True)

        if "B" in phases:
            scx = scope("s_5aBpro"); scx.__enter__()
            mp = None
            for j in range(NKC):
                t, _ = b_qk(0, j, 0)
                mp = t if mp is None else jnp.maximum(mp, t)
            mbuf[0] = jnp.max(mp, axis=-1, keepdims=True)
            scx.__exit__(None, None, None)

            def b_iter(i, _):
                r = lax.rem(i, 2)
                b_tile(i, r, 1 - r)
            with scope("s_5bBloop"):
                lax.fori_loop(0, NTT - 1, b_iter, None)
            with scope("s_5cBlast"):
                b_tile(NTT - 1, (NTT - 1) % 2, NTT % 2, do_next=False)
            if do_conv:
                with scope("s_5dconv"):
                    lax.fori_loop(NTT - 2, NTT, lambda i_, _: conv(i_), None)

        scd = scope("s_6aDpro"); scd.__enter__()
        n = float(B * T)
        mu = jnp.sum(stat[0], axis=0, keepdims=True) / n
        var = jnp.sum(stat[1], axis=0, keepdims=True) / n - mu * mu
        hr = 0.5 * lax.rsqrt(var + EPS)

        wc[8].wait()
        wc[9].wait()
        wc[10].wait()

        def ocopy(i, slot):
            return pltpu.make_async_copy(obuf.at[slot], o_hbm.at[rows(i)], osem.at[slot])

        def d_act_pieces(i, a_w):
            b, t0 = bt(i)
            z = 0 if isinstance(i, int) else lax.shift_right_logical(i, 20)

            def piece(q, seed):
                if seed is not None:
                    gd[0, 0, B - 1, pl.ds(pl.multiple_of(T + 2 * GH + 8 * z, 8), 8), :] = seed
                dcv = jnp.concatenate([gd[1, c, b, pl.ds(GH + t0 + q * drc, drc), :] for c in range(ND)], axis=1)
                a_w[q * drc // 2:(q + 1) * drc // 2, :] = _pk(_half_silu((dcv - mu) * hr).astype(BF16))
            return [functools.partial(piece, q) for q in range(TM // drc)]

        def d_act(i, a_w):
            for p_ in d_act_pieces(i, a_w):
                p_(None)

        def d_fin_pieces(i, g_r, slot):
            z = 0 if isinstance(i, int) else lax.shift_right_logical(i, 20)

            def piece(q, seed):
                if seed is not None:
                    g_r[pl.ds(pl.multiple_of(TM + 8 * z, 8), 8), 0:128] = seed
                rs = slice(q * drc, (q + 1) * drc)
                obuf[slot, rs, :] = _ln(g_r[rs, :], 1.0).astype(BF16)
            return [functools.partial(piece, q) for q in range(TM // drc)]

        def d_pw2(i, a_r, f_w, xn_w, seeded=True):
            f_w[0:TM, :] = res[rows(i), :] + _dot(_un(a_r[...]), wp2[...])
            z = 0 if isinstance(i, int) else lax.shift_right_logical(i, 20)

            def piece(q, seed):
                if seed is not None:
                    f_w[pl.ds(pl.multiple_of(TM + 8 * z, 8), 8), 0:128] = seed
                rs = slice(q * drc, (q + 1) * drc)
                xn_w[q * drc // 2:(q + 1) * drc // 2, :] = _pk(_ln(f_w[rs, :], 0.5).astype(BF16))
            pieces = [functools.partial(piece, q) for q in range(TM // drc)]
            if seeded:
                return pieces
            for f_ in pieces:
                f_(None)

        def d_fin(x4, slot):
            obuf[slot] = _ln(x4, 1.0).astype(BF16)

        def d_half(i, slot, a_r, a_w, f_r, f_w, xn_r, xn_w, g_r, g_w):
            fins = d_fin_pieces(i, g_r, slot)
            acts = d_act_pieces(clamp_hi(i + 2), a_w)
            mix = []
            for q in range(max(len(fins), len(acts))):
                mix += fins[q:q + 1] + acts[q:q + 1]
            rel = Releaser(mix, dplan, exact=True)
            y = None
            for c in range(NF):
                if c == d_split:
                    lnp = d_pw2(clamp_hi(i + 1), a_r, f_w, xn_w)
                    rel.pieces = lnp + rel.pieces
                t = ff_chunk(xn_r, w2a, w2b, c, rel)
                y = t if y is None else y + t
            g_w[0:TM, :] = f_r[0:TM, :] + 0.5 * y

        if "D" in phases:
            gB[...] = jnp.zeros(gB.shape, F32)
            d_act(0, hA)
            d_pw2(0, hA, fA, xnA, seeded=False)
            d_act(1, hB)

            def d_pair(p, _):
                i = 2 * p
                sb = 2 * lax.rem(p, 2)

                @pl.when(p >= 2)
                def _():
                    ocopy(i - 4, sb).wait()

                @pl.when(p >= 3)
                def _():
                    ocopy(i - 5, sb + 1).wait()
                d_half(i, sb + 1, hB, hA, fA, fB, xnA, xnB, gB, gA)
                d_half(i + 1, sb, hA, hB, fB, fA, xnB, xnA, gA, gB)

                @pl.when(p >= 1)
                def _():
                    ocopy(i - 1, sb + 1).start()
                ocopy(i, sb).start()
            scd.__exit__(None, None, None)
            with scope("s_6bDloop"):
                lax.fori_loop(0, NTT // 2, d_pair, None)
            scd = scope("s_6cDepi"); scd.__enter__()
            P = NTT // 2

            def oslot(t):
                pp = (t + 1) // 2
                return 2 * (pp % 2) + (t % 2)
            ocopy(NTT - 5, oslot(NTT - 5)).wait()
            d_fin(gB[0:TM, :], oslot(NTT - 5))
            ocopy(NTT - 1, oslot(NTT - 5)).start()
            for t in (NTT - 4, NTT - 3, NTT - 2):
                ocopy(t, oslot(t)).wait()
            ocopy(NTT - 1, oslot(NTT - 5)).wait()
        else:
            obuf[0] = x_v[0:TM, :].astype(obuf.dtype)
            ocopy(0, 0).start()
            ocopy(0, 0).wait()
        scd.__exit__(None, None, None)

    def fn(x, w_ff1_a, w_ff1_b, w_q, w_k, w_v, w_o, w_pw1, dw, w_pw2, w_ff2_a, w_ff2_b):
        x2 = x.reshape(B * T, D)
        any_spec = pl.BlockSpec(memory_space=pl.ANY)
        V = pltpu.VMEM
        out = pl.pallas_call(
            kernel,
            out_shape=jax.ShapeDtypeStruct((B * T, D), BF16),
            in_specs=[any_spec] * 12,
            out_specs=any_spec,
            scratch_shapes=[
                V((B * T + 16, D), BF16),
                V((D, F), BF16), V((F, D), BF16),
                V((D, D), BF16), V((D, D), BF16), V((D, D), BF16), V((D, D), BF16),
                V((D, 2 * D), BF16), V((K, D), BF16), V((D, D), BF16),
                V((D, F), BF16), V((F, D), BF16),
                V((D // 2, 2 * D), U32),
                V((K, 8, D), F32),
                V((B * T + 16, D), F32),
                V((B * T // 2, D), U32),
                V((B, TP // 2, D), U32), V((B, TP // 2, D), U32),
                V((2, ND, B, T + 2 * GH + 16, 128), F32),
                V((2, TM + 8, TP), F32),
                V((TM // 2, TP), U32),
                V((2, TM, 128), F32),
                V((2, TM, 1), F32),
                V((2, TM // 2, D), U32), V((2, TM // 2, D), U32),
                V((TM // 2, D), U32), V((TM // 2, D), U32),
                V((TM // 2, D), U32), V((TM // 2, D), U32),
                V((TM + 16, D), F32), V((TM + 16, D), F32),
                V((TM + 16, D), F32), V((TM + 16, D), F32),
                V((2, 8, D), F32),
                V((4, TM, D), BF16),
                pltpu.SemaphoreType.DMA((4,)),
                pltpu.SemaphoreType.DMA((11 + 2 * NF,)),
                pltpu.SemaphoreType.DMA((4,)),
            ],
            compiler_params=pltpu.CompilerParams(vmem_limit_bytes=127 * 1024 * 1024),
        )(x2, w_ff1_a, w_ff1_b, w_q, w_k, w_v, w_o, w_pw1, dw, w_pw2, w_ff2_a, w_ff2_b)
        return out.reshape(B, T, D)

    return fn


@jax.jit
def pallas_standalone__conformer_family_conformer__speech_kernel(
    x, w_ff1_a, w_ff1_b, w_q, w_k, w_v, w_o, w_pw1, dw, w_pw2, w_ff2_a, w_ff2_b):
    B, T, D = x.shape
    K = dw.shape[0]
    F = w_ff1_a.shape[1]
    return make_kernel(B, T, D, K, F)(
        x, w_ff1_a, w_ff1_b, w_q, w_k, w_v, w_o, w_pw1, dw, w_pw2, w_ff2_a, w_ff2_b)
```

```python
import functools
import math
import numpy as np

import jax
import jax.numpy as jnp
from jax import lax
import jax.experimental.pallas as pl
import jax.experimental.pallas.tpu as pltpu

F32 = jnp.float32
BF16 = jnp.bfloat16
EPS = 1e-5
LOG2E = 1.4426950408889634


def _ln(xf, post):
    m = jnp.mean(xf, axis=-1, keepdims=True)
    xc = xf - m
    v = jnp.mean(xc * xc, axis=-1, keepdims=True)
    r = lax.rsqrt(v + EPS)
    if post != 1.0:
        r = r * post
    return xc * r


def _half_silu(h):
    return h * (1.0 + jnp.tanh(h))


U32 = jnp.uint32


def _pk(v):
    return pltpu.bitcast(v, U32)


def _un(v):
    return pltpu.bitcast(v, BF16)


def _dot(a, b):
    return jnp.dot(a, b, preferred_element_type=F32)


def _dot_nt(a, b):
    return lax.dot_general(a, b, (((1,), (1,)), ((), ())), preferred_element_type=F32)


def make_kernel(B, T, D, K, F, TM=400, phases="ABD", ffc=512, prewait=False, kc=512, qk_split=5,
                border="alpha", crc=16, cacc=5, brc=16, lplan=(10,10,5), lmode='mem', aseed=True, arc=80, arc2=80, ln2span=2000, aplan=(1,1,1,1,1), dseed=True, drc=16, dplan=(10,10,10,10,10,10,10,5), cplan=(0,0,0,0,0, 1,1,1,1,1,1,1,3, 0,0,0, 0,0), cplan_last=(1,1,1,1,1,1,1,1), do_conv=True, d_split=2, erc=16, qk_tail=0, e0pos=1, brep=0, dbg_aligned=False, dbg_taps=15, scopes=False):
    TP = (T + 127) // 128 * 128
    NT = T // TM
    NTT = B * NT
    assert NTT % 2 == 0 and NTT >= 6
    PAD = K // 2
    GH = 8
    scale = D ** -0.5
    NKC = TP // kc
    ND = D // 128
    NF = F // ffc

    def kernel(x_hbm, w1a_hbm, w1b_hbm, wq_hbm, wk_hbm, wv_hbm, wo_hbm, wp1_hbm, dw_hbm, wp2_hbm,
               w2a_hbm, w2b_hbm, o_hbm,
               x_v, w1a, w1b, wq, wk, wv, wo, wp1, dw_v, wp2, w2a, w2b, wqv, dwb,
               res, qbuf, kbuf, vbuf, gd,
               sbuf, pbuf, lbuf, mbuf, xnS, hS, xnA, xnB, hA, hB, fA, fB, gA, gB, stat, obuf,
               xsem, wsem, osem):
        def rows(i):
            if isinstance(i, int):
                return pl.ds(i * TM, TM)
            return pl.ds(pl.multiple_of(i * TM, 16), TM)

        def hrows(i):
            if isinstance(i, int):
                return pl.ds(i * (TM // 2), TM // 2)
            return pl.ds(pl.multiple_of(i * (TM // 2), 8), TM // 2)

        def bt(i):
            if isinstance(i, int):
                return i // NT, (i % NT) * TM
            b = lax.div(i, NT)
            return b, pl.multiple_of((i - b * NT) * TM, 16)

        def clamp_hi(i):
            if isinstance(i, int):
                return min(i, NTT - 1)
            return jnp.minimum(i, NTT - 1)

        def clamp_lo(i):
            if isinstance(i, int):
                return max(i, 0)
            return jnp.maximum(i, 0)

        def xcp(t0_, t1_, k_):
            return pltpu.make_async_copy(x_hbm.at[pl.ds(t0_ * TM, (t1_ - t0_) * TM)],
                                         x_v.at[pl.ds(t0_ * TM, (t1_ - t0_) * TM)], xsem.at[k_])
        xc0, xc1, xc2, xc3 = xcp(0, 1, 0), xcp(1, 2, 1), xcp(2, 4, 2), xcp(4, NTT, 3)
        wlist = [(wq_hbm, wq), (wk_hbm, wk), (wv_hbm, wv), (wo_hbm, wo), (w1a_hbm, w1a), (w1b_hbm, w1b),
                 (wp1_hbm, wp1), (dw_hbm, dw_v), (wp2_hbm, wp2), (w2a_hbm, w2a), (w2b_hbm, w2b)]
        wc = [pltpu.make_async_copy(s_, d_, wsem.at[j]) for j, (s_, d_) in enumerate(wlist)]
        w1ac = [pltpu.make_async_copy(w1a_hbm.at[:, cs_], w1a.at[:, cs_], wsem.at[11 + c])
                for c in range(NF) for cs_ in [pl.ds(c * ffc, ffc)]]
        w1bc = [pltpu.make_async_copy(w1b_hbm.at[cs_, :], w1b.at[cs_, :], wsem.at[11 + NF + c])
                for c in range(NF) for cs_ in [pl.ds(c * ffc, ffc)]]

        def scope(name):
            class _S:
                def __enter__(self_):
                    if scopes: self_.s = jax.named_scope(name); self_.s.__enter__()
                def __exit__(self_, *a):
                    if scopes: self_.s.__exit__(*a)
            return _S()

        sc0 = scope("s_0start"); sc0.__enter__()
        zdyn = lax.fori_loop(0, 2, lambda i_, c_: c_ + lax.shift_right_logical(i_, 20), jnp.int32(0))
        late = wc[6:11]
        if not prewait:
            xc0.start()
            w1ac[0].start()
            w1bc[0].start()
        else:
            for c_ in [xc0, xc1, xc2, xc3] + w1ac + w1bc + wc[:4] + wc[6:]:
                c_.start()

        if prewait:
            allc = [xc0, xc1, xc2, xc3] + w1ac + w1bc + wc[:4] + wc[6:]
            for c_ in allc:
                c_.wait()

            class _C:
                def wait(self): pass
                def start(self): pass
            wc = [_C() for _ in range(11)]
            late = []
            xc0 = xc1 = xc2 = xc3 = _C()
            w1ac = [_C() for _ in range(NF)]
            w1bc = [_C() for _ in range(NF)]

        for b in range(B):
            kbuf[b, T // 2:TP // 2, :] = jnp.zeros(((TP - T) // 2, D), U32)
            vbuf[b, T // 2:TP // 2, :] = jnp.zeros(((TP - T) // 2, D), U32)
            for c in range(ND):
                gd[0, c, b, 0:GH, :] = jnp.zeros((GH, 128), F32)
                gd[0, c, b, GH + T:GH + T + GH, :] = jnp.zeros((GH, 128), F32)
        stat[...] = jnp.zeros(stat.shape, F32)

        def seed_of(t, tpos):
            n_, r_ = tpos // TM, (tpos % TM) // 8 * 8
            return t[r_:r_ + 8, n_ * 128:(n_ + 1) * 128]

        class Releaser:
            def __init__(self, pieces, plan, exact=False):
                self.pieces, self.cum, self.k = list(pieces), np.cumsum([0] + list(plan)), 0
                self.n = int(self.cum[-1]) if exact else len(self.pieces)

            def __call__(self, t):
                k0 = self.k
                self.k += 1
                if self.k >= len(self.cum):
                    return
                tot = int(self.cum[-1])
                n = int(self.cum[k0 + 1]) * self.n // tot - int(self.cum[k0]) * self.n // tot
                span = t.shape[1] // 128 * TM
                for q in range(n):
                    self.pieces.pop(0)(seed_of(t, (2 * q + 1) * span // (2 * n)))

        def ff_chunk(xn_ref, wa, wb, c, rel=None):
            h = _dot(_un(xn_ref[...]), wa[:, c * ffc:(c + 1) * ffc])
            if rel is not None:
                rel(h)
            a = _half_silu(h).astype(BF16)
            y = _dot(a, wb[c * ffc:(c + 1) * ffc, :])
            if rel is not None:
                rel(y)
            return y

        def a_ln1(i, sl):
            xnS[sl] = _pk(_ln(x_v[rows(i), :].astype(F32), 0.5).astype(BF16))

        def a_ln1_pieces(i, sl):
            z = zdyn
            r0 = i * TM if isinstance(i, int) else pl.multiple_of(i * TM, 16)

            def piece(q, seed):
                if seed is not None:
                    x_v[pl.ds(pl.multiple_of(B * T + 16 * z, 16), 16), 0:128] = pltpu.bitcast(seed, BF16)
                rs = pl.ds(r0 + q * arc, arc)
                xnS[sl, q * arc // 2:(q + 1) * arc // 2, :] = _pk(_ln(x_v[rs, :].astype(F32), 0.5).astype(BF16))
            return [functools.partial(piece, q) for q in range(TM // arc)]

        def a_ff(i, sl, rel, waits=False, mid=None):
            y = None
            for c in range(NF):
                if waits:
                    w1ac[c].wait()
                    for c_ in ([w1ac[c + 1]] if c + 1 < NF else [wc[0], wc[1]]):
                        c_.start()
                h = _dot(_un(xnS[sl]), w1a[:, c * ffc:(c + 1) * ffc])
                rel(h)
                a = _half_silu(h).astype(BF16)
                if waits:
                    w1bc[c].wait()
                    for c_ in ([w1bc[c + 1]] if c + 1 < NF else [wc[2], wc[3], xc2]):
                        c_.start()
                t = _dot(a, w1b[c * ffc:(c + 1) * ffc, :])
                rel(t)
                y = t if y is None else y + t
            res[rows(i), :] = x_v[rows(i), :].astype(F32) + 0.5 * y
            b, t0 = bt(i)
            h0 = t0 // 2 if isinstance(t0, int) else pl.multiple_of(lax.shift_right_logical(t0, 1), 8)
            z = zdyn
            r0 = i * TM if isinstance(i, int) else pl.multiple_of(i * TM, 16)

            def ln2(q, seed):
                if seed is not None:
                    res[pl.ds(pl.multiple_of(B * T + 8 * z, 8), 8), 0:128] = seed
                hn = _pk(_ln(res[pl.ds(r0 + q * arc2, arc2), :], 1.0).astype(BF16))
                kbuf[b, pl.ds(h0 + q * arc2 // 2, arc2 // 2), :] = hn
                hS[sl, q * arc2 // 2:(q + 1) * arc2 // 2, :] = hn
            pieces = [functools.partial(ln2, q) for q in range(TM // arc2)]
            if mid is not None:
                t = mid()
                for q, f_ in enumerate(pieces):
                    f_(seed_of(t, ln2span * q // len(pieces)))
            else:
                for f_ in pieces:
                    f_(None)

        def a_qv(i, hn):
            b, t0 = bt(i)
            raw = _dot(_un(hn), _un(wqv[...]))
            qv = _pk(raw.astype(BF16))
            h0 = t0 // 2 if isinstance(t0, int) else pl.multiple_of(lax.shift_right_logical(t0, 1), 8)
            qbuf[hrows(i), :] = qv[:, :D]
            vbuf[b, pl.ds(h0, TM // 2), :] = qv[:, D:]
            return raw

        xc0.wait()
        xc1.start()
        a_ln1(0, 0)
        sc0.__exit__(None, None, None)
        if "A" in phases:
            with scope("s_1a0"):
                xc1.wait()
                a_ff(0, 0, Releaser(a_ln1_pieces(1, 1), aplan), waits=True)
                wc[0].wait()
                wc[1].wait()
                wqv[:, :D] = _pk((_dot_nt(wq[...], wk[...]) * (scale * LOG2E)).astype(BF16))
                wc[2].wait()
                wc[3].wait()
                xc3.start()
                wqv[:, D:] = _pk(_dot(wv[...], wo[...]).astype(BF16))
                xc2.wait()

            def a_iter(i, _):
                @pl.when(i == 3)
                def _():
                    xc3.wait()
                    for c_ in late:
                        c_.start()
                sl = lax.rem(i, 2)
                a_ff(i, sl, Releaser(a_ln1_pieces(clamp_hi(i + 1), 1 - sl), aplan),
                     mid=lambda: a_qv(i - 1, hS[1 - sl]))
            with scope("s_3aloop"):
                lax.fori_loop(1, NTT, a_iter, None)
            with scope("s_4alast"):
                a_qv(NTT - 1, hS[(NTT - 1) % 2])
        else:
            if not prewait:
                for c_ in [xc2, xc3] + w1ac[1:] + w1bc[1:] + wc[:4] + late:
                    c_.start()
            for c_ in [xc1, xc2, xc3] + w1ac + w1bc + wc[:4]:
                c_.wait()

        wc[6].wait()
        wc[7].wait()
        for k in range(K):
            dwb[k] = jnp.broadcast_to(dw_v[k:k + 1, :].astype(F32), (8, D))

        def kslice(j):
            return slice(j * kc, (j + 1) * kc)

        def hslice(j):
            return slice(j * kc // 2, (j + 1) * kc // 2)

        def lane_fold(v, op):
            r = v[:, 0:128]
            for c in range(1, v.shape[1] // 128):
                r = op(r, v[:, c * 128:(c + 1) * 128])
            return r

        def b_qk(i, j, w):
            b, _ = bt(i)
            s = _dot_nt(_un(qbuf[hrows(i), :]), _un(kbuf[b, hslice(j), :]))
            raw = s
            if (j + 1) * kc > T:
                col = lax.broadcasted_iota(jnp.int32, (TM, kc), 1)
                s = jnp.where(col < (T - j * kc), s, -jnp.inf)
            sbuf[w, 0:TM, kslice(j)] = s
            return lane_fold(s, jnp.maximum), raw

        def b_glu(i, xn):
            b, t0 = bt(i)
            ab = _dot(xn, wp1[...])
            g = ab[:, :D] * (1.0 + jnp.tanh(ab[:, D:]))
            for c in range(ND):
                gd[0, c, b, pl.ds(GH + t0, TM), :] = g[:, c * 128:(c + 1) * 128]

        def conv_pieces(i, valid=None):
            b, t0 = bt(i)
            st = {}

            def piece(c, rc, seed=None):
                cs = slice(c * 128, (c + 1) * 128)
                if seed is not None:
                    gd[1, 0, b, pl.ds(pl.multiple_of(8 * zdyn, 8), 8), :] = seed
                accs = [None] * cacc
                for k in range(K):
                    w = dwb[k, :, cs]
                    t = gd[0, c, b, pl.ds(t0 + GH - PAD + k + rc, crc), :]
                    t = t.reshape(crc // 8, 8, 128) * w[None]
                    accs[k % cacc] = t if accs[k % cacc] is None else accs[k % cacc] + t
                while len(accs) > 1:
                    accs = [accs[u] + accs[u + 1] if u + 1 < len(accs) else accs[u] for u in range(0, len(accs), 2)]
                acc = accs[0]
                gd[1, c, b, pl.ds(GH + t0 + rc, crc), :] = acc.reshape(crc, 128)
                a1 = jnp.sum(acc, axis=0)
                a2 = jnp.sum(acc * acc, axis=0)
                if rc == 0:
                    st[c] = (a1, a2)
                else:
                    st[c] = (st[c][0] + a1, st[c][1] + a2)
                if rc + crc == TM:
                    s1, s2 = st[c]
                    if valid is not None:
                        s1 = jnp.where(valid, s1, 0.0)
                        s2 = jnp.where(valid, s2, 0.0)
                    stat[0, :, cs] += s1
                    stat[1, :, cs] += s2

            return [functools.partial(piece, c, rc) for c in range(ND) for rc in range(0, TM, crc)]

        def conv(i):
            for p_ in conv_pieces(i):
                p_()

        nq = TM // erc

        def lsum(r, j, rs):
            t = lane_fold(_un(pbuf[rs.start // 2:rs.stop // 2, kslice(j)]).astype(F32), jnp.add)
            if j == 0:
                lbuf[r, rs, :] = t
            else:
                lbuf[r, rs, :] += t

        def exp_piece(r, z, m, j, q, seed):
            rs = slice(q * erc, (q + 1) * erc)
            if seed is not None:
                sbuf[r, pl.ds(pl.multiple_of(TM + 8 * z, 8), 8), 0:128] = seed
            p = jnp.exp2(sbuf[r, rs, kslice(j)] - m[rs])
            pk = _pk(p.astype(BF16))
            pbuf[rs.start // 2:rs.stop // 2, kslice(j)] = pk
            if lmode == "mem":
                lsum(r, j, rs)
            else:
                t = lane_fold(_un(pk).astype(F32) if lmode.startswith("val") else p, jnp.add)
                sl = r + z if (j % 2 and lmode.endswith("pin")) else r
                if j == 0:
                    lbuf[sl, rs, :] = t
                else:
                    lbuf[sl, rs, :] += t

        def spread(t, items, phase):
            n = len(items)
            for q, f in enumerate(items):
                f(seed_of(t, (q * ND * TM) // n + phase * (ND * TM) // (2 * n)))

        def b_tile(i, r, w, do_next=True, conv_on=True):
            b, _ = bt(i)
            pcs = []
            if conv_on and do_conv:
                if isinstance(i, int):
                    if i >= 2:
                        pcs = conv_pieces(i - 2)
                else:
                    pcs = conv_pieces(clamp_lo(i - 2), valid=(i >= 2))
            m = mbuf[r]
            z = zdyn
            eps_ = {j: [functools.partial(exp_piece, r, z, m, j, q) for q in range(nq)] for j in range(NKC)}
            plan = list(cplan) if do_next else [0] * qk_split + list(cplan_last) + [0] * (NKC - qk_split) + [0, 0]
            tot = sum(plan)
            npcs = len(pcs)
            cum = [0]
            for v in plan:
                cum.append(cum[-1] + v)
            site = [0]

            def release(t, exps=()):
                k0 = site[0]
                site[0] += 1
                n = (cum[k0 + 1] * npcs) // tot - (cum[k0] * npcs) // tot if npcs else 0
                items = [(q * ND * TM // n + ND * TM // (2 * n), 1, pcs.pop(0)) for q in range(n)]
                ne = len(exps)
                items += [(q * ND * TM // ne, 0, f_) for q, f_ in enumerate(exps)]
                items.sort(key=lambda u: u[:2])
                for tpos, _k, f_ in items:
                    f_(seed_of(t, tpos))

            mp = None
            if do_next:
                for j in range(qk_split):
                    t, raw = b_qk(i + 1, j, w)
                    mp = t if mp is None else jnp.maximum(mp, t)
                    release(raw, eps_[0] if j == qk_split - 1 - e0pos else ())
            else:
                site[0] = qk_split
                for f_ in eps_[0]:
                    f_(None)
            o = None
            for j in range(NKC):
                t = _dot(_un(pbuf[:, kslice(j)]), _un(vbuf[b, hslice(j), :]))
                o = t if o is None else o + t
                release(t, eps_[j + 1] if j + 1 < NKC else ())
            l = jnp.sum(lbuf[r], axis=-1, keepdims=True)
            res[rows(i), :] = res[rows(i), :] + o * (1.0 / l)
            r0 = i * TM if isinstance(i, int) else pl.multiple_of(i * TM, 16)

            def lnb(q, seed):
                if seed is not None:
                    res[pl.ds(pl.multiple_of(B * T + 8 * z, 8), 8), 0:128] = seed
                xnA[q * brc // 2:(q + 1) * brc // 2, :] = _pk(_ln(res[pl.ds(r0 + q * brc, brc), :], 0.5).astype(BF16))
            lps = [functools.partial(lnb, q) for q in range(TM // brc)]
            if do_next:
                for j in range(qk_split, NKC):
                    t, raw = b_qk(i + 1, j, w)
                    mp = t if mp is None else jnp.maximum(mp, t)
                    k_ = j - qk_split
                    if k_ < len(lplan):
                        n_ = lplan[k_]
                        release(raw, [functools.partial(lambda f_, sd: f_(sd), lps.pop(0)) for _ in range(n_)])
                    else:
                        release(raw)
                assert not lps
            else:
                site[0] = NKC + NKC
                for f_ in lps:
                    f_(None)
            xn = _un(xnA[...])
            bb, t0 = bt(i)
            a_ = _dot(xn, wp1[:, :D])
            release(a_)
            b_ = _dot(xn, wp1[:, D:])
            release(b_)
            g = a_ * (1.0 + jnp.tanh(b_))
            for c in range(ND):
                gd[0, c, bb, pl.ds(GH + t0, TM), :] = g[:, c * 128:(c + 1) * 128]
            assert not pcs
            if do_next:
                mbuf[w] = jnp.max(mp, axis=-1, keepdims=True)

        if "B" in phases:
            scx = scope("s_5aBpro"); scx.__enter__()
            mp = None
            for j in range(NKC):
                t, _ = b_qk(0, j, 0)
                mp = t if mp is None else jnp.maximum(mp, t)
            mbuf[0] = jnp.max(mp, axis=-1, keepdims=True)
            scx.__exit__(None, None, None)

            def b_iter(i, _):
                r = lax.rem(i, 2)
                b_tile(i, r, 1 - r)
            with scope("s_5bBloop"):
                lax.fori_loop(0, NTT - 1, b_iter, None)
            with scope("s_5cBlast"):
                b_tile(NTT - 1, (NTT - 1) % 2, NTT % 2, do_next=False)
            if do_conv:
                with scope("s_5dconv"):
                    lax.fori_loop(NTT - 2, NTT, lambda i_, _: conv(i_), None)

        scd = scope("s_6aDpro"); scd.__enter__()
        n = float(B * T)
        mu = jnp.sum(stat[0], axis=0, keepdims=True) / n
        var = jnp.sum(stat[1], axis=0, keepdims=True) / n - mu * mu
        hr = 0.5 * lax.rsqrt(var + EPS)

        wc[8].wait()
        wc[9].wait()
        wc[10].wait()

        def ocopy(i, slot):
            return pltpu.make_async_copy(obuf.at[slot], o_hbm.at[rows(i)], osem.at[slot])

        def d_act_pieces(i, a_w):
            b, t0 = bt(i)
            z = zdyn

            def piece(q, seed):
                if seed is not None:
                    gd[0, 0, B - 1, pl.ds(pl.multiple_of(T + 2 * GH + 8 * z, 8), 8), :] = seed
                dcv = jnp.concatenate([gd[1, c, b, pl.ds(GH + t0 + q * drc, drc), :] for c in range(ND)], axis=1)
                a_w[q * drc // 2:(q + 1) * drc // 2, :] = _pk(_half_silu((dcv - mu) * hr).astype(BF16))
            return [functools.partial(piece, q) for q in range(TM // drc)]

        def d_act(i, a_w):
            for p_ in d_act_pieces(i, a_w):
                p_(None)

        def d_fin_pieces(i, g_r, slot):
            z = zdyn

            def piece(q, seed):
                if seed is not None:
                    g_r[pl.ds(pl.multiple_of(TM + 8 * z, 8), 8), 0:128] = seed
                rs = slice(q * drc, (q + 1) * drc)
                obuf[slot, rs, :] = _ln(g_r[rs, :], 1.0).astype(BF16)
            return [functools.partial(piece, q) for q in range(TM // drc)]

        def d_pw2(i, a_r, f_w, xn_w, seeded=True):
            f_w[0:TM, :] = res[rows(i), :] + _dot(_un(a_r[...]), wp2[...])
            z = zdyn

            def piece(q, seed):
                if seed is not None:
                    f_w[pl.ds(pl.multiple_of(TM + 8 * z, 8), 8), 0:128] = seed
                rs = slice(q * drc, (q + 1) * drc)
                xn_w[q * drc // 2:(q + 1) * drc // 2, :] = _pk(_ln(f_w[rs, :], 0.5).astype(BF16))
            pieces = [functools.partial(piece, q) for q in range(TM // drc)]
            if seeded:
                return pieces
            for f_ in pieces:
                f_(None)

        def d_fin(x4, slot):
            obuf[slot] = _ln(x4, 1.0).astype(BF16)

        def d_half(i, slot, a_r, a_w, f_r, f_w, xn_r, xn_w, g_r, g_w):
            fins = d_fin_pieces(i, g_r, slot)
            acts = d_act_pieces(clamp_hi(i + 2), a_w)
            mix = []
            for q in range(max(len(fins), len(acts))):
                mix += fins[q:q + 1] + acts[q:q + 1]
            rel = Releaser(mix, dplan, exact=True)
            y = None
            for c in range(NF):
                if c == d_split:
                    lnp = d_pw2(clamp_hi(i + 1), a_r, f_w, xn_w)
                    rel.pieces = lnp + rel.pieces
                t = ff_chunk(xn_r, w2a, w2b, c, rel)
                y = t if y is None else y + t
            g_w[0:TM, :] = f_r[0:TM, :] + 0.5 * y

        if "D" in phases:
            gB[...] = jnp.zeros(gB.shape, F32)
            d_act(0, hA)
            d_pw2(0, hA, fA, xnA, seeded=False)
            d_act(1, hB)

            def d_pair(p, _):
                i = 2 * p
                sb = 2 * lax.rem(p, 2)

                @pl.when(p >= 2)
                def _():
                    ocopy(i - 4, sb).wait()

                @pl.when(p >= 3)
                def _():
                    ocopy(i - 5, sb + 1).wait()
                d_half(i, sb + 1, hB, hA, fA, fB, xnA, xnB, gB, gA)
                d_half(i + 1, sb, hA, hB, fB, fA, xnB, xnA, gA, gB)

                @pl.when(p >= 1)
                def _():
                    ocopy(i - 1, sb + 1).start()
                ocopy(i, sb).start()
            scd.__exit__(None, None, None)
            with scope("s_6bDloop"):
                lax.fori_loop(0, NTT // 2, d_pair, None)
            scd = scope("s_6cDepi"); scd.__enter__()
            P = NTT // 2

            def oslot(t):
                pp = (t + 1) // 2
                return 2 * (pp % 2) + (t % 2)
            ocopy(NTT - 5, oslot(NTT - 5)).wait()
            d_fin(gB[0:TM, :], oslot(NTT - 5))
            ocopy(NTT - 1, oslot(NTT - 5)).start()
            for t in (NTT - 4, NTT - 3, NTT - 2):
                ocopy(t, oslot(t)).wait()
            ocopy(NTT - 1, oslot(NTT - 5)).wait()
        else:
            obuf[0] = x_v[0:TM, :].astype(obuf.dtype)
            ocopy(0, 0).start()
            ocopy(0, 0).wait()
        scd.__exit__(None, None, None)

    def fn(x, w_ff1_a, w_ff1_b, w_q, w_k, w_v, w_o, w_pw1, dw, w_pw2, w_ff2_a, w_ff2_b):
        x2 = x.reshape(B * T, D)
        any_spec = pl.BlockSpec(memory_space=pl.ANY)
        V = pltpu.VMEM
        out = pl.pallas_call(
            kernel,
            out_shape=jax.ShapeDtypeStruct((B * T, D), BF16),
            in_specs=[any_spec] * 12,
            out_specs=any_spec,
            scratch_shapes=[
                V((B * T + 16, D), BF16),
                V((D, F), BF16), V((F, D), BF16),
                V((D, D), BF16), V((D, D), BF16), V((D, D), BF16), V((D, D), BF16),
                V((D, 2 * D), BF16), V((K, D), BF16), V((D, D), BF16),
                V((D, F), BF16), V((F, D), BF16),
                V((D // 2, 2 * D), U32),
                V((K, 8, D), F32),
                V((B * T + 16, D), F32),
                V((B * T // 2, D), U32),
                V((B, TP // 2, D), U32), V((B, TP // 2, D), U32),
                V((2, ND, B, T + 2 * GH + 16, 128), F32),
                V((2, TM + 8, TP), F32),
                V((TM // 2, TP), U32),
                V((2, TM, 128), F32),
                V((2, TM, 1), F32),
                V((2, TM // 2, D), U32), V((2, TM // 2, D), U32),
                V((TM // 2, D), U32), V((TM // 2, D), U32),
                V((TM // 2, D), U32), V((TM // 2, D), U32),
                V((TM + 16, D), F32), V((TM + 16, D), F32),
                V((TM + 16, D), F32), V((TM + 16, D), F32),
                V((2, 8, D), F32),
                V((4, TM, D), BF16),
                pltpu.SemaphoreType.DMA((4,)),
                pltpu.SemaphoreType.DMA((11 + 2 * NF,)),
                pltpu.SemaphoreType.DMA((4,)),
            ],
            compiler_params=pltpu.CompilerParams(vmem_limit_bytes=127 * 1024 * 1024),
        )(x2, w_ff1_a, w_ff1_b, w_q, w_k, w_v, w_o, w_pw1, dw, w_pw2, w_ff2_a, w_ff2_b)
        return out.reshape(B, T, D)

    return fn


@jax.jit
def pallas_standalone__conformer_family_conformer__speech_kernel(
    x, w_ff1_a, w_ff1_b, w_q, w_k, w_v, w_o, w_pw1, dw, w_pw2, w_ff2_a, w_ff2_b):
    B, T, D = x.shape
    K = dw.shape[0]
    F = w_ff1_a.shape[1]
    return make_kernel(B, T, D, K, F)(
        x, w_ff1_a, w_ff1_b, w_q, w_k, w_v, w_o, w_pw1, dw, w_pw2, w_ff2_a, w_ff2_b)
```

```python
import functools
import math
import numpy as np

import jax
import jax.numpy as jnp
from jax import lax
import jax.experimental.pallas as pl
import jax.experimental.pallas.tpu as pltpu

F32 = jnp.float32
BF16 = jnp.bfloat16
EPS = 1e-5
LOG2E = 1.4426950408889634


def _ln(xf, post):
    m = jnp.mean(xf, axis=-1, keepdims=True)
    xc = xf - m
    v = jnp.mean(xc * xc, axis=-1, keepdims=True)
    r = lax.rsqrt(v + EPS)
    if post != 1.0:
        r = r * post
    return xc * r


def _half_silu(h):
    return h * (1.0 + jnp.tanh(h))


U32 = jnp.uint32


def _pk(v):
    return pltpu.bitcast(v, U32)


def _un(v):
    return pltpu.bitcast(v, BF16)


def _dot(a, b):
    return jnp.dot(a, b, preferred_element_type=F32)


def _dot_nt(a, b):
    return lax.dot_general(a, b, (((1,), (1,)), ((), ())), preferred_element_type=F32)


def make_kernel(B, T, D, K, F, TM=400, phases="ABD", ffc=512, prewait=False, kc=512, qk_split=5,
                border="alpha", crc=16, cacc=5, brc=16, lplan=(10,10,5), lmode='mem', aseed=True, dq=3, aplan0=(0,0,0,2,1,1,1), arc=80, arc2=80, ln2span=2000, aplan=(1,1,1,1,1), dseed=True, drc=16, dplan=(10,10,10,10,10,10,10,5), cplan=(0,0,0,0,0, 1,1,1,1,1,1,1,3, 0,0,0, 0,0), cplan_last=(1,1,1,1,1,1,1,1), do_conv=True, d_split=2, erc=16, qk_tail=0, e0pos=1, brep=0, dbg_aligned=False, dbg_taps=15, scopes=False):
    TP = (T + 127) // 128 * 128
    NT = T // TM
    NTT = B * NT
    assert NTT % 2 == 0 and NTT >= 6
    PAD = K // 2
    GH = 8
    scale = D ** -0.5
    NKC = TP // kc
    ND = D // 128
    NF = F // ffc

    def kernel(x_hbm, w1a_hbm, w1b_hbm, wq_hbm, wk_hbm, wv_hbm, wo_hbm, wp1_hbm, dw_hbm, wp2_hbm,
               w2a_hbm, w2b_hbm, o_hbm,
               x_v, w1a, w1b, wq, wk, wv, wo, wp1, dw_v, wp2, w2a, w2b, wqv, dwb,
               res, qbuf, kbuf, vbuf, gd,
               sbuf, pbuf, lbuf, mbuf, xnS, hS, xnA, xnB, hA, hB, fA, fB, gA, gB, stat, obuf,
               xsem, wsem, osem):
        def rows(i):
            if isinstance(i, int):
                return pl.ds(i * TM, TM)
            return pl.ds(pl.multiple_of(i * TM, 16), TM)

        def hrows(i):
            if isinstance(i, int):
                return pl.ds(i * (TM // 2), TM // 2)
            return pl.ds(pl.multiple_of(i * (TM // 2), 8), TM // 2)

        def bt(i):
            if isinstance(i, int):
                return i // NT, (i % NT) * TM
            b = lax.div(i, NT)
            return b, pl.multiple_of((i - b * NT) * TM, 16)

        def clamp_hi(i):
            if isinstance(i, int):
                return min(i, NTT - 1)
            return jnp.minimum(i, NTT - 1)

        def clamp_lo(i):
            if isinstance(i, int):
                return max(i, 0)
            return jnp.maximum(i, 0)

        def xcp(t0_, t1_, k_):
            return pltpu.make_async_copy(x_hbm.at[pl.ds(t0_ * TM, (t1_ - t0_) * TM)],
                                         x_v.at[pl.ds(t0_ * TM, (t1_ - t0_) * TM)], xsem.at[k_])
        xc0, xc1, xc2, xc3 = xcp(0, 1, 0), xcp(1, 2, 1), xcp(2, 4, 2), xcp(4, NTT, 3)
        wlist = [(wq_hbm, wq), (wk_hbm, wk), (wv_hbm, wv), (wo_hbm, wo), (w1a_hbm, w1a), (w1b_hbm, w1b),
                 (wp1_hbm, wp1), (dw_hbm, dw_v), (wp2_hbm, wp2), (w2a_hbm, w2a), (w2b_hbm, w2b)]
        wc = [pltpu.make_async_copy(s_, d_, wsem.at[j]) for j, (s_, d_) in enumerate(wlist)]
        w1ac = [pltpu.make_async_copy(w1a_hbm.at[:, cs_], w1a.at[:, cs_], wsem.at[11 + c])
                for c in range(NF) for cs_ in [pl.ds(c * ffc, ffc)]]
        w1bc = [pltpu.make_async_copy(w1b_hbm.at[cs_, :], w1b.at[cs_, :], wsem.at[11 + NF + c])
                for c in range(NF) for cs_ in [pl.ds(c * ffc, ffc)]]

        def scope(name):
            class _S:
                def __enter__(self_):
                    if scopes: self_.s = jax.named_scope(name); self_.s.__enter__()
                def __exit__(self_, *a):
                    if scopes: self_.s.__exit__(*a)
            return _S()

        sc0 = scope("s_0start"); sc0.__enter__()
        zdyn = lax.fori_loop(0, 2, lambda i_, c_: c_ + lax.shift_right_logical(i_, 20), jnp.int32(0))
        late = wc[6:11]
        if not prewait:
            xc0.start()
            w1ac[0].start()
            if dq == 0:
                w1bc[0].start()
        else:
            for c_ in [xc0, xc1, xc2, xc3] + w1ac + w1bc + wc[:4] + wc[6:]:
                c_.start()

        if prewait:
            allc = [xc0, xc1, xc2, xc3] + w1ac + w1bc + wc[:4] + wc[6:]
            for c_ in allc:
                c_.wait()

            class _C:
                def wait(self): pass
                def start(self): pass
            wc = [_C() for _ in range(11)]
            late = []
            xc0 = xc1 = xc2 = xc3 = _C()
            w1ac = [_C() for _ in range(NF)]
            w1bc = [_C() for _ in range(NF)]

        for b in range(B):
            kbuf[b, T // 2:TP // 2, :] = jnp.zeros(((TP - T) // 2, D), U32)
            vbuf[b, T // 2:TP // 2, :] = jnp.zeros(((TP - T) // 2, D), U32)
            for c in range(ND):
                gd[0, c, b, 0:GH, :] = jnp.zeros((GH, 128), F32)
                gd[0, c, b, GH + T:GH + T + GH, :] = jnp.zeros((GH, 128), F32)
        stat[...] = jnp.zeros(stat.shape, F32)

        def seed_of(t, tpos):
            n_, r_ = tpos // TM, (tpos % TM) // 8 * 8
            return t[r_:r_ + 8, n_ * 128:(n_ + 1) * 128]

        class Releaser:
            def __init__(self, pieces, plan, exact=False):
                self.pieces, self.cum, self.k = list(pieces), np.cumsum([0] + list(plan)), 0
                self.n = int(self.cum[-1]) if exact else len(self.pieces)

            def __call__(self, t):
                k0 = self.k
                self.k += 1
                if self.k >= len(self.cum):
                    return
                tot = int(self.cum[-1])
                n = int(self.cum[k0 + 1]) * self.n // tot - int(self.cum[k0]) * self.n // tot
                span = t.shape[1] // 128 * TM
                for q in range(n):
                    self.pieces.pop(0)(seed_of(t, (2 * q + 1) * span // (2 * n)))

        def ff_chunk(xn_ref, wa, wb, c, rel=None):
            h = _dot(_un(xn_ref[...]), wa[:, c * ffc:(c + 1) * ffc])
            if rel is not None:
                rel(h)
            a = _half_silu(h).astype(BF16)
            y = _dot(a, wb[c * ffc:(c + 1) * ffc, :])
            if rel is not None:
                rel(y)
            return y

        def a_ln1(i, sl):
            xnS[sl] = _pk(_ln(x_v[rows(i), :].astype(F32), 0.5).astype(BF16))

        def a_ln1_pieces(i, sl, first_wait=None):
            z = zdyn
            r0 = i * TM if isinstance(i, int) else pl.multiple_of(i * TM, 16)

            def piece(q, seed):
                if q == 0 and first_wait is not None:
                    first_wait.wait()
                if seed is not None:
                    x_v[pl.ds(pl.multiple_of(B * T + 16 * z, 16), 16), 0:128] = pltpu.bitcast(seed, BF16)
                rs = pl.ds(r0 + q * arc, arc)
                xnS[sl, q * arc // 2:(q + 1) * arc // 2, :] = _pk(_ln(x_v[rs, :].astype(F32), 0.5).astype(BF16))
            return [functools.partial(piece, q) for q in range(TM // arc)]

        def a_ff(i, sl, rel, waits=False, mid=None):
            y = None
            for c in range(NF):
                if waits:
                    w1ac[c].wait()
                    startq()
                h = _dot(_un(xnS[sl]), w1a[:, c * ffc:(c + 1) * ffc])
                rel(h)
                a = _half_silu(h).astype(BF16)
                if waits:
                    w1bc[c].wait()
                    startq()
                t = _dot(a, w1b[c * ffc:(c + 1) * ffc, :])
                rel(t)
                y = t if y is None else y + t
            res[rows(i), :] = x_v[rows(i), :].astype(F32) + 0.5 * y
            b, t0 = bt(i)
            h0 = t0 // 2 if isinstance(t0, int) else pl.multiple_of(lax.shift_right_logical(t0, 1), 8)
            z = zdyn
            r0 = i * TM if isinstance(i, int) else pl.multiple_of(i * TM, 16)

            def ln2(q, seed):
                if seed is not None:
                    res[pl.ds(pl.multiple_of(B * T + 8 * z, 8), 8), 0:128] = seed
                hn = _pk(_ln(res[pl.ds(r0 + q * arc2, arc2), :], 1.0).astype(BF16))
                kbuf[b, pl.ds(h0 + q * arc2 // 2, arc2 // 2), :] = hn
                hS[sl, q * arc2 // 2:(q + 1) * arc2 // 2, :] = hn
            pieces = [functools.partial(ln2, q) for q in range(TM // arc2)]
            if mid is not None:
                t = mid()
                for q, f_ in enumerate(pieces):
                    f_(seed_of(t, ln2span * q // len(pieces)))
            else:
                for f_ in pieces:
                    f_(None)

        def a_qv(i, hn):
            b, t0 = bt(i)
            raw = _dot(_un(hn), _un(wqv[...]))
            qv = _pk(raw.astype(BF16))
            h0 = t0 // 2 if isinstance(t0, int) else pl.multiple_of(lax.shift_right_logical(t0, 1), 8)
            qbuf[hrows(i), :] = qv[:, :D]
            vbuf[b, pl.ds(h0, TM // 2), :] = qv[:, D:]
            return raw

        if dq == 0:
            queue = [[w1ac[1]], [w1bc[1], xc1]]
            for c in range(2, NF):
                queue += [[w1ac[c]], [w1bc[c]]]
        elif dq == 1:
            queue = [[w1bc[0], w1ac[1]], [w1bc[1], xc1]]
            for c in range(2, NF):
                queue += [[w1ac[c]], [w1bc[c]]]
        elif dq == 2:
            queue = [[w1bc[0]], [w1ac[1], w1bc[1]], [w1ac[2], xc1]]
            for c in range(2, NF - 1):
                queue += [[w1bc[c]], [w1ac[c + 1]]]
            queue += [[w1bc[NF - 1]]]
        elif dq == 3:
            queue = [[w1bc[0], w1ac[1]], [w1bc[1], w1ac[2]], [xc1, w1bc[2]], [w1ac[3]], [w1bc[3]]]
        queue += [[wc[0], wc[1]], [wc[2], wc[3]], [xc2]]

        def startq():
            if queue:
                for c_ in queue.pop(0):
                    c_.start()

        xc0.wait()
        startq()
        a_ln1(0, 0)
        sc0.__exit__(None, None, None)
        if "A" in phases:
            with scope("s_1a0"):
                a_ff(0, 0, Releaser(a_ln1_pieces(1, 1, first_wait=xc1), aplan0), waits=True)
                while queue:
                    startq()
                xc2.wait()

            def a_iter(i, _):
                @pl.when(i == 1)
                def _():
                    wc[0].wait()
                    wc[1].wait()
                    wc[2].wait()
                    wc[3].wait()
                    xc3.start()
                    wqv[:, :D] = _pk((_dot_nt(wq[...], wk[...]) * (scale * LOG2E)).astype(BF16))
                    wqv[:, D:] = _pk(_dot(wv[...], wo[...]).astype(BF16))

                @pl.when(i == 3)
                def _():
                    xc3.wait()
                    for c_ in late:
                        c_.start()
                sl = lax.rem(i, 2)
                a_ff(i, sl, Releaser(a_ln1_pieces(clamp_hi(i + 1), 1 - sl), aplan),
                     mid=lambda: a_qv(i - 1, hS[1 - sl]))
            with scope("s_3aloop"):
                lax.fori_loop(1, NTT, a_iter, None)
            with scope("s_4alast"):
                a_qv(NTT - 1, hS[(NTT - 1) % 2])
        else:
            if not prewait:
                while queue:
                    startq()
                for c_ in [xc3] + late:
                    c_.start()
            for c_ in [xc1, xc2, xc3] + w1ac + w1bc + wc[:4]:
                c_.wait()

        wc[6].wait()
        wc[7].wait()
        for k in range(K):
            dwb[k] = jnp.broadcast_to(dw_v[k:k + 1, :].astype(F32), (8, D))

        def kslice(j):
            return slice(j * kc, (j + 1) * kc)

        def hslice(j):
            return slice(j * kc // 2, (j + 1) * kc // 2)

        def lane_fold(v, op):
            r = v[:, 0:128]
            for c in range(1, v.shape[1] // 128):
                r = op(r, v[:, c * 128:(c + 1) * 128])
            return r

        def b_qk(i, j, w):
            b, _ = bt(i)
            s = _dot_nt(_un(qbuf[hrows(i), :]), _un(kbuf[b, hslice(j), :]))
            raw = s
            if (j + 1) * kc > T:
                col = lax.broadcasted_iota(jnp.int32, (TM, kc), 1)
                s = jnp.where(col < (T - j * kc), s, -jnp.inf)
            sbuf[w, 0:TM, kslice(j)] = s
            return lane_fold(s, jnp.maximum), raw

        def b_glu(i, xn):
            b, t0 = bt(i)
            ab = _dot(xn, wp1[...])
            g = ab[:, :D] * (1.0 + jnp.tanh(ab[:, D:]))
            for c in range(ND):
                gd[0, c, b, pl.ds(GH + t0, TM), :] = g[:, c * 128:(c + 1) * 128]

        def conv_pieces(i, valid=None):
            b, t0 = bt(i)
            st = {}

            def piece(c, rc, seed=None):
                cs = slice(c * 128, (c + 1) * 128)
                if seed is not None:
                    gd[1, 0, b, pl.ds(pl.multiple_of(8 * zdyn, 8), 8), :] = seed
                accs = [None] * cacc
                for k in range(K):
                    w = dwb[k, :, cs]
                    t = gd[0, c, b, pl.ds(t0 + GH - PAD + k + rc, crc), :]
                    t = t.reshape(crc // 8, 8, 128) * w[None]
                    accs[k % cacc] = t if accs[k % cacc] is None else accs[k % cacc] + t
                while len(accs) > 1:
                    accs = [accs[u] + accs[u + 1] if u + 1 < len(accs) else accs[u] for u in range(0, len(accs), 2)]
                acc = accs[0]
                gd[1, c, b, pl.ds(GH + t0 + rc, crc), :] = acc.reshape(crc, 128)
                a1 = jnp.sum(acc, axis=0)
                a2 = jnp.sum(acc * acc, axis=0)
                if rc == 0:
                    st[c] = (a1, a2)
                else:
                    st[c] = (st[c][0] + a1, st[c][1] + a2)
                if rc + crc == TM:
                    s1, s2 = st[c]
                    if valid is not None:
                        s1 = jnp.where(valid, s1, 0.0)
                        s2 = jnp.where(valid, s2, 0.0)
                    stat[0, :, cs] += s1
                    stat[1, :, cs] += s2

            return [functools.partial(piece, c, rc) for c in range(ND) for rc in range(0, TM, crc)]

        def conv(i):
            for p_ in conv_pieces(i):
                p_()

        nq = TM // erc

        def lsum(r, j, rs):
            t = lane_fold(_un(pbuf[rs.start // 2:rs.stop // 2, kslice(j)]).astype(F32), jnp.add)
            if j == 0:
                lbuf[r, rs, :] = t
            else:
                lbuf[r, rs, :] += t

        def exp_piece(r, z, m, j, q, seed):
            rs = slice(q * erc, (q + 1) * erc)
            if seed is not None:
                sbuf[r, pl.ds(pl.multiple_of(TM + 8 * z, 8), 8), 0:128] = seed
            p = jnp.exp2(sbuf[r, rs, kslice(j)] - m[rs])
            pk = _pk(p.astype(BF16))
            pbuf[rs.start // 2:rs.stop // 2, kslice(j)] = pk
            if lmode == "mem":
                lsum(r, j, rs)
            else:
                t = lane_fold(_un(pk).astype(F32) if lmode.startswith("val") else p, jnp.add)
                sl = r + z if (j % 2 and lmode.endswith("pin")) else r
                if j == 0:
                    lbuf[sl, rs, :] = t
                else:
                    lbuf[sl, rs, :] += t

        def spread(t, items, phase):
            n = len(items)
            for q, f in enumerate(items):
                f(seed_of(t, (q * ND * TM) // n + phase * (ND * TM) // (2 * n)))

        def b_tile(i, r, w, do_next=True, conv_on=True):
            b, _ = bt(i)
            pcs = []
            if conv_on and do_conv:
                if isinstance(i, int):
                    if i >= 2:
                        pcs = conv_pieces(i - 2)
                else:
                    pcs = conv_pieces(clamp_lo(i - 2), valid=(i >= 2))
            m = mbuf[r]
            z = zdyn
            eps_ = {j: [functools.partial(exp_piece, r, z, m, j, q) for q in range(nq)] for j in range(NKC)}
            plan = list(cplan) if do_next else [0] * qk_split + list(cplan_last) + [0] * (NKC - qk_split) + [0, 0]
            tot = sum(plan)
            npcs = len(pcs)
            cum = [0]
            for v in plan:
                cum.append(cum[-1] + v)
            site = [0]

            def release(t, exps=()):
                k0 = site[0]
                site[0] += 1
                n = (cum[k0 + 1] * npcs) // tot - (cum[k0] * npcs) // tot if npcs else 0
                items = [(q * ND * TM // n + ND * TM // (2 * n), 1, pcs.pop(0)) for q in range(n)]
                ne = len(exps)
                items += [(q * ND * TM // ne, 0, f_) for q, f_ in enumerate(exps)]
                items.sort(key=lambda u: u[:2])
                for tpos, _k, f_ in items:
                    f_(seed_of(t, tpos))

            mp = None
            if do_next:
                for j in range(qk_split):
                    t, raw = b_qk(i + 1, j, w)
                    mp = t if mp is None else jnp.maximum(mp, t)
                    release(raw, eps_[0] if j == qk_split - 1 - e0pos else ())
            else:
                site[0] = qk_split
                for f_ in eps_[0]:
                    f_(None)
            o = None
            for j in range(NKC):
                t = _dot(_un(pbuf[:, kslice(j)]), _un(vbuf[b, hslice(j), :]))
                o = t if o is None else o + t
                release(t, eps_[j + 1] if j + 1 < NKC else ())
            l = jnp.sum(lbuf[r], axis=-1, keepdims=True)
            res[rows(i), :] = res[rows(i), :] + o * (1.0 / l)
            r0 = i * TM if isinstance(i, int) else pl.multiple_of(i * TM, 16)

            def lnb(q, seed):
                if seed is not None:
                    res[pl.ds(pl.multiple_of(B * T + 8 * z, 8), 8), 0:128] = seed
                xnA[q * brc // 2:(q + 1) * brc // 2, :] = _pk(_ln(res[pl.ds(r0 + q * brc, brc), :], 0.5).astype(BF16))
            lps = [functools.partial(lnb, q) for q in range(TM // brc)]
            if do_next:
                for j in range(qk_split, NKC):
                    t, raw = b_qk(i + 1, j, w)
                    mp = t if mp is None else jnp.maximum(mp, t)
                    k_ = j - qk_split
                    if k_ < len(lplan):
                        n_ = lplan[k_]
                        release(raw, [functools.partial(lambda f_, sd: f_(sd), lps.pop(0)) for _ in range(n_)])
                    else:
                        release(raw)
                assert not lps
            else:
                site[0] = NKC + NKC
                for f_ in lps:
                    f_(None)
            xn = _un(xnA[...])
            bb, t0 = bt(i)
            a_ = _dot(xn, wp1[:, :D])
            release(a_)
            b_ = _dot(xn, wp1[:, D:])
            release(b_)
            g = a_ * (1.0 + jnp.tanh(b_))
            for c in range(ND):
                gd[0, c, bb, pl.ds(GH + t0, TM), :] = g[:, c * 128:(c + 1) * 128]
            assert not pcs
            if do_next:
                mbuf[w] = jnp.max(mp, axis=-1, keepdims=True)

        if "B" in phases:
            scx = scope("s_5aBpro"); scx.__enter__()
            mp = None
            for j in range(NKC):
                t, _ = b_qk(0, j, 0)
                mp = t if mp is None else jnp.maximum(mp, t)
            mbuf[0] = jnp.max(mp, axis=-1, keepdims=True)
            scx.__exit__(None, None, None)

            def b_iter(i, _):
                r = lax.rem(i, 2)
                b_tile(i, r, 1 - r)
            with scope("s_5bBloop"):
                lax.fori_loop(0, NTT - 1, b_iter, None)
            with scope("s_5cBlast"):
                b_tile(NTT - 1, (NTT - 1) % 2, NTT % 2, do_next=False)
            if do_conv:
                with scope("s_5dconv"):
                    lax.fori_loop(NTT - 2, NTT, lambda i_, _: conv(i_), None)

        scd = scope("s_6aDpro"); scd.__enter__()
        n = float(B * T)
        mu = jnp.sum(stat[0], axis=0, keepdims=True) / n
        var = jnp.maximum(jnp.sum(stat[1], axis=0, keepdims=True) / n - mu * mu, 0.0)
        hr = 0.5 * lax.rsqrt(var + EPS)

        wc[8].wait()
        wc[9].wait()
        wc[10].wait()

        def ocopy(i, slot):
            return pltpu.make_async_copy(obuf.at[slot], o_hbm.at[rows(i)], osem.at[slot])

        def d_act_pieces(i, a_w):
            b, t0 = bt(i)
            z = zdyn

            def piece(q, seed):
                if seed is not None:
                    gd[0, 0, B - 1, pl.ds(pl.multiple_of(T + 2 * GH + 8 * z, 8), 8), :] = seed
                dcv = jnp.concatenate([gd[1, c, b, pl.ds(GH + t0 + q * drc, drc), :] for c in range(ND)], axis=1)
                a_w[q * drc // 2:(q + 1) * drc // 2, :] = _pk(_half_silu((dcv - mu) * hr).astype(BF16))
            return [functools.partial(piece, q) for q in range(TM // drc)]

        def d_act(i, a_w):
            for p_ in d_act_pieces(i, a_w):
                p_(None)

        def d_fin_pieces(i, g_r, slot):
            z = zdyn

            def piece(q, seed):
                if seed is not None:
                    g_r[pl.ds(pl.multiple_of(TM + 8 * z, 8), 8), 0:128] = seed
                rs = slice(q * drc, (q + 1) * drc)
                obuf[slot, rs, :] = _ln(g_r[rs, :], 1.0).astype(BF16)
            return [functools.partial(piece, q) for q in range(TM // drc)]

        def d_pw2(i, a_r, f_w, xn_w, seeded=True):
            f_w[0:TM, :] = res[rows(i), :] + _dot(_un(a_r[...]), wp2[...])
            z = zdyn

            def piece(q, seed):
                if seed is not None:
                    f_w[pl.ds(pl.multiple_of(TM + 8 * z, 8), 8), 0:128] = seed
                rs = slice(q * drc, (q + 1) * drc)
                xn_w[q * drc // 2:(q + 1) * drc // 2, :] = _pk(_ln(f_w[rs, :], 0.5).astype(BF16))
            pieces = [functools.partial(piece, q) for q in range(TM // drc)]
            if seeded:
                return pieces
            for f_ in pieces:
                f_(None)

        def d_fin(x4, slot):
            obuf[slot] = _ln(x4, 1.0).astype(BF16)

        def d_half(i, slot, a_r, a_w, f_r, f_w, xn_r, xn_w, g_r, g_w):
            fins = d_fin_pieces(i, g_r, slot)
            acts = d_act_pieces(clamp_hi(i + 2), a_w)
            mix = []
            for q in range(max(len(fins), len(acts))):
                mix += fins[q:q + 1] + acts[q:q + 1]
            rel = Releaser(mix, dplan, exact=True)
            y = None
            for c in range(NF):
                if c == d_split:
                    lnp = d_pw2(clamp_hi(i + 1), a_r, f_w, xn_w)
                    rel.pieces = lnp + rel.pieces
                t = ff_chunk(xn_r, w2a, w2b, c, rel)
                y = t if y is None else y + t
            g_w[0:TM, :] = f_r[0:TM, :] + 0.5 * y

        if "D" in phases:
            gB[...] = jnp.zeros(gB.shape, F32)
            d_act(0, hA)
            d_pw2(0, hA, fA, xnA, seeded=False)
            d_act(1, hB)

            def d_pair(p, _):
                i = 2 * p
                sb = 2 * lax.rem(p, 2)

                @pl.when(p >= 2)
                def _():
                    ocopy(i - 4, sb).wait()

                @pl.when(p >= 3)
                def _():
                    ocopy(i - 5, sb + 1).wait()
                d_half(i, sb + 1, hB, hA, fA, fB, xnA, xnB, gB, gA)
                d_half(i + 1, sb, hA, hB, fB, fA, xnB, xnA, gA, gB)

                @pl.when(p >= 1)
                def _():
                    ocopy(i - 1, sb + 1).start()
                ocopy(i, sb).start()
            scd.__exit__(None, None, None)
            with scope("s_6bDloop"):
                lax.fori_loop(0, NTT // 2, d_pair, None)
            scd = scope("s_6cDepi"); scd.__enter__()
            P = NTT // 2

            def oslot(t):
                pp = (t + 1) // 2
                return 2 * (pp % 2) + (t % 2)
            ocopy(NTT - 5, oslot(NTT - 5)).wait()
            d_fin(gB[0:TM, :], oslot(NTT - 5))
            ocopy(NTT - 1, oslot(NTT - 5)).start()
            for t in (NTT - 4, NTT - 3, NTT - 2):
                ocopy(t, oslot(t)).wait()
            ocopy(NTT - 1, oslot(NTT - 5)).wait()
        else:
            obuf[0] = x_v[0:TM, :].astype(obuf.dtype)
            ocopy(0, 0).start()
            ocopy(0, 0).wait()
        scd.__exit__(None, None, None)

    def fn(x, w_ff1_a, w_ff1_b, w_q, w_k, w_v, w_o, w_pw1, dw, w_pw2, w_ff2_a, w_ff2_b):
        x2 = x.reshape(B * T, D)
        any_spec = pl.BlockSpec(memory_space=pl.ANY)
        V = pltpu.VMEM
        out = pl.pallas_call(
            kernel,
            out_shape=jax.ShapeDtypeStruct((B * T, D), BF16),
            in_specs=[any_spec] * 12,
            out_specs=any_spec,
            scratch_shapes=[
                V((B * T + 16, D), BF16),
                V((D, F), BF16), V((F, D), BF16),
                V((D, D), BF16), V((D, D), BF16), V((D, D), BF16), V((D, D), BF16),
                V((D, 2 * D), BF16), V((K, D), BF16), V((D, D), BF16),
                V((D, F), BF16), V((F, D), BF16),
                V((D // 2, 2 * D), U32),
                V((K, 8, D), F32),
                V((B * T + 16, D), F32),
                V((B * T // 2, D), U32),
                V((B, TP // 2, D), U32), V((B, TP // 2, D), U32),
                V((2, ND, B, T + 2 * GH + 16, 128), F32),
                V((2, TM + 8, TP), F32),
                V((TM // 2, TP), U32),
                V((2, TM, 128), F32),
                V((2, TM, 1), F32),
                V((2, TM // 2, D), U32), V((2, TM // 2, D), U32),
                V((TM // 2, D), U32), V((TM // 2, D), U32),
                V((TM // 2, D), U32), V((TM // 2, D), U32),
                V((TM + 16, D), F32), V((TM + 16, D), F32),
                V((TM + 16, D), F32), V((TM + 16, D), F32),
                V((2, 8, D), F32),
                V((4, TM, D), BF16),
                pltpu.SemaphoreType.DMA((4,)),
                pltpu.SemaphoreType.DMA((11 + 2 * NF,)),
                pltpu.SemaphoreType.DMA((4,)),
            ],
            compiler_params=pltpu.CompilerParams(vmem_limit_bytes=127 * 1024 * 1024),
        )(x2, w_ff1_a, w_ff1_b, w_q, w_k, w_v, w_o, w_pw1, dw, w_pw2, w_ff2_a, w_ff2_b)
        return out.reshape(B, T, D)

    return fn


@jax.jit
def pallas_standalone__conformer_family_conformer__speech_kernel(
    x, w_ff1_a, w_ff1_b, w_q, w_k, w_v, w_o, w_pw1, dw, w_pw2, w_ff2_a, w_ff2_b):
    B, T, D = x.shape
    K = dw.shape[0]
    F = w_ff1_a.shape[1]
    return make_kernel(B, T, D, K, F)(
        x, w_ff1_a, w_ff1_b, w_q, w_k, w_v, w_o, w_pw1, dw, w_pw2, w_ff2_a, w_ff2_b)
```

```python
import functools
import math
import numpy as np

import jax
import jax.numpy as jnp
from jax import lax
import jax.experimental.pallas as pl
import jax.experimental.pallas.tpu as pltpu

F32 = jnp.float32
BF16 = jnp.bfloat16
EPS = 1e-5
LOG2E = 1.4426950408889634


def _ln(xf, post):
    m = jnp.mean(xf, axis=-1, keepdims=True)
    xc = xf - m
    v = jnp.mean(xc * xc, axis=-1, keepdims=True)
    r = lax.rsqrt(v + EPS)
    if post != 1.0:
        r = r * post
    return xc * r


def _half_silu(h):
    return h * (1.0 + jnp.tanh(h))


U32 = jnp.uint32


def _pk(v):
    return pltpu.bitcast(v, U32)


def _un(v):
    return pltpu.bitcast(v, BF16)


def _dot(a, b):
    return jnp.dot(a, b, preferred_element_type=F32)


def _dot_nt(a, b):
    return lax.dot_general(a, b, (((1,), (1,)), ((), ())), preferred_element_type=F32)


def make_kernel(B, T, D, K, F, TM=400, phases="ABD", ffc=512, prewait=False, kc=512, qk_split=5,
                border="alpha", crc=16, cacc=5, brc=16, lplan=(10,10,5), lmode='mem', fold_conv=True, aseed=True, dq=1, aplan0=(0,0,0,0,2,2,1), arc=80, arc2=80, ln2span=2000, aplan=(1,1,1,1,1), dseed=True, drc=16, dplan=(10,10,10,10,10,10,10,5), cplan=(0,0,0,0,0, 1,1,1,1,1,1,1,3, 0,0,0, 0,0), cplan_last=(1,1,1,1,1,1,1,1), do_conv=True, d_split=2, erc=16, qk_tail=0, e0pos=1, brep=0, dbg_aligned=False, dbg_taps=15, scopes=False):
    TP = (T + 127) // 128 * 128
    NT = T // TM
    NTT = B * NT
    assert NTT % 2 == 0 and NTT >= 6
    PAD = K // 2
    GH = 8
    scale = D ** -0.5
    NKC = TP // kc
    ND = D // 128
    NF = F // ffc

    def kernel(x_hbm, w1a_hbm, w1b_hbm, wq_hbm, wk_hbm, wv_hbm, wo_hbm, wp1_hbm, dw_hbm, wp2_hbm,
               w2a_hbm, w2b_hbm, o_hbm,
               x_v, w1a, w1b, wq, wk, wv, wo, wp1, dw_v, wp2, w2a, w2b, wqv, dwb,
               res, qbuf, kbuf, vbuf, gd,
               sbuf, pbuf, lbuf, mbuf, xnS, hS, xnA, xnB, hA, hB, fA, fB, gA, gB, stat, obuf,
               xsem, wsem, osem):
        def rows(i):
            if isinstance(i, int):
                return pl.ds(i * TM, TM)
            return pl.ds(pl.multiple_of(i * TM, 16), TM)

        def hrows(i):
            if isinstance(i, int):
                return pl.ds(i * (TM // 2), TM // 2)
            return pl.ds(pl.multiple_of(i * (TM // 2), 8), TM // 2)

        def bt(i):
            if isinstance(i, int):
                return i // NT, (i % NT) * TM
            b = lax.div(i, NT)
            return b, pl.multiple_of((i - b * NT) * TM, 16)

        def clamp_hi(i):
            if isinstance(i, int):
                return min(i, NTT - 1)
            return jnp.minimum(i, NTT - 1)

        def clamp_lo(i):
            if isinstance(i, int):
                return max(i, 0)
            return jnp.maximum(i, 0)

        def xcp(t0_, t1_, k_):
            return pltpu.make_async_copy(x_hbm.at[pl.ds(t0_ * TM, (t1_ - t0_) * TM)],
                                         x_v.at[pl.ds(t0_ * TM, (t1_ - t0_) * TM)], xsem.at[k_])
        xc0, xc1, xc2, xc3 = xcp(0, 1, 0), xcp(1, 2, 1), xcp(2, 4, 2), xcp(4, NTT, 3)
        wlist = [(wq_hbm, wq), (wk_hbm, wk), (wv_hbm, wv), (wo_hbm, wo), (w1a_hbm, w1a), (w1b_hbm, w1b),
                 (wp1_hbm, wp1), (dw_hbm, dw_v), (wp2_hbm, wp2), (w2a_hbm, w2a), (w2b_hbm, w2b)]
        wc = [pltpu.make_async_copy(s_, d_, wsem.at[j]) for j, (s_, d_) in enumerate(wlist)]
        w1ac = [pltpu.make_async_copy(w1a_hbm.at[:, cs_], w1a.at[:, cs_], wsem.at[11 + c])
                for c in range(NF) for cs_ in [pl.ds(c * ffc, ffc)]]
        w1bc = [pltpu.make_async_copy(w1b_hbm.at[cs_, :], w1b.at[cs_, :], wsem.at[11 + NF + c])
                for c in range(NF) for cs_ in [pl.ds(c * ffc, ffc)]]

        def scope(name):
            class _S:
                def __enter__(self_):
                    if scopes: self_.s = jax.named_scope(name); self_.s.__enter__()
                def __exit__(self_, *a):
                    if scopes: self_.s.__exit__(*a)
            return _S()

        sc0 = scope("s_0start"); sc0.__enter__()
        zdyn = lax.fori_loop(0, 2, lambda i_, c_: c_ + lax.shift_right_logical(i_, 20), jnp.int32(0))
        late = wc[6:11]
        if not prewait:
            xc0.start()
            w1ac[0].start()
            if dq == 0:
                w1bc[0].start()
        else:
            for c_ in [xc0, xc1, xc2, xc3] + w1ac + w1bc + wc[:4] + wc[6:]:
                c_.start()

        if prewait:
            allc = [xc0, xc1, xc2, xc3] + w1ac + w1bc + wc[:4] + wc[6:]
            for c_ in allc:
                c_.wait()

            class _C:
                def wait(self): pass
                def start(self): pass
            wc = [_C() for _ in range(11)]
            late = []
            xc0 = xc1 = xc2 = xc3 = _C()
            w1ac = [_C() for _ in range(NF)]
            w1bc = [_C() for _ in range(NF)]

        for b in range(B):
            kbuf[b, T // 2:TP // 2, :] = jnp.zeros(((TP - T) // 2, D), U32)
            vbuf[b, T // 2:TP // 2, :] = jnp.zeros(((TP - T) // 2, D), U32)
            for c in range(ND):
                gd[0, c, b, 0:GH, :] = jnp.zeros((GH, 128), F32)
                gd[0, c, b, GH + T:GH + T + GH, :] = jnp.zeros((GH, 128), F32)
        stat[...] = jnp.zeros(stat.shape, F32)

        def seed_of(t, tpos):
            n_, r_ = tpos // TM, (tpos % TM) // 8 * 8
            return t[r_:r_ + 8, n_ * 128:(n_ + 1) * 128]

        class Releaser:
            def __init__(self, pieces, plan, exact=False):
                self.pieces, self.cum, self.k = list(pieces), np.cumsum([0] + list(plan)), 0
                self.n = int(self.cum[-1]) if exact else len(self.pieces)

            def __call__(self, t):
                k0 = self.k
                self.k += 1
                if self.k >= len(self.cum):
                    return
                tot = int(self.cum[-1])
                n = int(self.cum[k0 + 1]) * self.n // tot - int(self.cum[k0]) * self.n // tot
                span = t.shape[1] // 128 * TM
                for q in range(n):
                    self.pieces.pop(0)(seed_of(t, (2 * q + 1) * span // (2 * n)))

        def ff_chunk(xn_ref, wa, wb, c, rel=None):
            h = _dot(_un(xn_ref[...]), wa[:, c * ffc:(c + 1) * ffc])
            if rel is not None:
                rel(h)
            a = _half_silu(h).astype(BF16)
            y = _dot(a, wb[c * ffc:(c + 1) * ffc, :])
            if rel is not None:
                rel(y)
            return y

        def a_ln1(i, sl):
            xnS[sl] = _pk(_ln(x_v[rows(i), :].astype(F32), 0.5).astype(BF16))

        def a_ln1_pieces(i, sl, first_wait=None):
            z = zdyn
            r0 = i * TM if isinstance(i, int) else pl.multiple_of(i * TM, 16)

            def piece(q, seed):
                if q == 0 and first_wait is not None:
                    first_wait.wait()
                if seed is not None:
                    x_v[pl.ds(pl.multiple_of(B * T + 16 * z, 16), 16), 0:128] = pltpu.bitcast(seed, BF16)
                rs = pl.ds(r0 + q * arc, arc)
                xnS[sl, q * arc // 2:(q + 1) * arc // 2, :] = _pk(_ln(x_v[rs, :].astype(F32), 0.5).astype(BF16))
            return [functools.partial(piece, q) for q in range(TM // arc)]

        def a_ff(i, sl, rel, waits=False, mid=None):
            y = None
            for c in range(NF):
                if waits:
                    w1ac[c].wait()
                    startq()
                h = _dot(_un(xnS[sl]), w1a[:, c * ffc:(c + 1) * ffc])
                rel(h)
                a = _half_silu(h).astype(BF16)
                if waits:
                    w1bc[c].wait()
                    startq()
                t = _dot(a, w1b[c * ffc:(c + 1) * ffc, :])
                rel(t)
                y = t if y is None else y + t
            res[rows(i), :] = x_v[rows(i), :].astype(F32) + 0.5 * y
            b, t0 = bt(i)
            h0 = t0 // 2 if isinstance(t0, int) else pl.multiple_of(lax.shift_right_logical(t0, 1), 8)
            z = zdyn
            r0 = i * TM if isinstance(i, int) else pl.multiple_of(i * TM, 16)

            def ln2(q, seed):
                if seed is not None:
                    res[pl.ds(pl.multiple_of(B * T + 8 * z, 8), 8), 0:128] = seed
                hn = _pk(_ln(res[pl.ds(r0 + q * arc2, arc2), :], 1.0).astype(BF16))
                kbuf[b, pl.ds(h0 + q * arc2 // 2, arc2 // 2), :] = hn
                hS[sl, q * arc2 // 2:(q + 1) * arc2 // 2, :] = hn
            pieces = [functools.partial(ln2, q) for q in range(TM // arc2)]
            if mid is not None:
                t = mid()
                for q, f_ in enumerate(pieces):
                    f_(seed_of(t, ln2span * q // len(pieces)))
            else:
                for f_ in pieces:
                    f_(None)

        def a_qv(i, hn):
            b, t0 = bt(i)
            raw = _dot(_un(hn), _un(wqv[...]))
            qv = _pk(raw.astype(BF16))
            h0 = t0 // 2 if isinstance(t0, int) else pl.multiple_of(lax.shift_right_logical(t0, 1), 8)
            qbuf[hrows(i), :] = qv[:, :D]
            vbuf[b, pl.ds(h0, TM // 2), :] = qv[:, D:]
            return raw

        if dq == 0:
            queue = [[w1ac[1]], [w1bc[1], xc1]]
            for c in range(2, NF):
                queue += [[w1ac[c]], [w1bc[c]]]
        elif dq == 1:
            queue = [[w1bc[0], w1ac[1]], [w1bc[1], xc1]]
            for c in range(2, NF):
                queue += [[w1ac[c]], [w1bc[c]]]
        elif dq == 2:
            queue = [[w1bc[0]], [w1ac[1], w1bc[1]], [w1ac[2], xc1]]
            for c in range(2, NF - 1):
                queue += [[w1bc[c]], [w1ac[c + 1]]]
            queue += [[w1bc[NF - 1]]]
        elif dq == 3:
            queue = [[w1bc[0], w1ac[1]], [w1bc[1], w1ac[2]], [xc1, w1bc[2]], [w1ac[3]], [w1bc[3]]]
        queue += [[wc[0], wc[1]], [wc[2], wc[3]], [xc2]]

        def startq():
            if queue:
                for c_ in queue.pop(0):
                    c_.start()

        xc0.wait()
        startq()
        a_ln1(0, 0)
        sc0.__exit__(None, None, None)
        if "A" in phases:
            with scope("s_1a0"):
                a_ff(0, 0, Releaser(a_ln1_pieces(1, 1, first_wait=xc1), aplan0), waits=True)
                while queue:
                    startq()
                xc2.wait()

            def a_iter(i, _):
                @pl.when(i == 1)
                def _():
                    wc[0].wait()
                    wc[1].wait()
                    wc[2].wait()
                    wc[3].wait()
                    xc3.start()
                    wqv[:, :D] = _pk((_dot_nt(wq[...], wk[...]) * (scale * LOG2E)).astype(BF16))
                    wqv[:, D:] = _pk(_dot(wv[...], wo[...]).astype(BF16))

                @pl.when(i == 3)
                def _():
                    xc3.wait()
                    for c_ in late:
                        c_.start()
                sl = lax.rem(i, 2)
                a_ff(i, sl, Releaser(a_ln1_pieces(clamp_hi(i + 1), 1 - sl), aplan),
                     mid=lambda: a_qv(i - 1, hS[1 - sl]))
            with scope("s_3aloop"):
                lax.fori_loop(1, NTT, a_iter, None)
            with scope("s_4alast"):
                a_qv(NTT - 1, hS[(NTT - 1) % 2])
        else:
            if not prewait:
                while queue:
                    startq()
                for c_ in [xc3] + late:
                    c_.start()
            for c_ in [xc1, xc2, xc3] + w1ac + w1bc + wc[:4]:
                c_.wait()

        wc[6].wait()
        wc[7].wait()
        for k in range(K):
            dwb[k] = jnp.broadcast_to(dw_v[k:k + 1, :].astype(F32), (8, D))

        def kslice(j):
            return slice(j * kc, (j + 1) * kc)

        def hslice(j):
            return slice(j * kc // 2, (j + 1) * kc // 2)

        def lane_fold(v, op):
            r = v[:, 0:128]
            for c in range(1, v.shape[1] // 128):
                r = op(r, v[:, c * 128:(c + 1) * 128])
            return r

        def b_qk(i, j, w):
            b, _ = bt(i)
            s = _dot_nt(_un(qbuf[hrows(i), :]), _un(kbuf[b, hslice(j), :]))
            raw = s
            if (j + 1) * kc > T:
                col = lax.broadcasted_iota(jnp.int32, (TM, kc), 1)
                s = jnp.where(col < (T - j * kc), s, -jnp.inf)
            sbuf[w, 0:TM, kslice(j)] = s
            return lane_fold(s, jnp.maximum), raw

        def b_glu(i, xn):
            b, t0 = bt(i)
            ab = _dot(xn, wp1[...])
            g = ab[:, :D] * (1.0 + jnp.tanh(ab[:, D:]))
            for c in range(ND):
                gd[0, c, b, pl.ds(GH + t0, TM), :] = g[:, c * 128:(c + 1) * 128]

        def conv_pieces(i, valid=None):
            b, t0 = bt(i)
            st = {}

            def piece(c, rc, seed=None):
                cs = slice(c * 128, (c + 1) * 128)
                if seed is not None:
                    gd[1, 0, b, pl.ds(pl.multiple_of(8 * zdyn, 8), 8), :] = seed
                accs = [None] * cacc
                for k in range(K):
                    w = dwb[k, :, cs]
                    t = gd[0, c, b, pl.ds(t0 + GH - PAD + k + rc, crc), :]
                    t = t.reshape(crc // 8, 8, 128) * w[None]
                    accs[k % cacc] = t if accs[k % cacc] is None else accs[k % cacc] + t
                while len(accs) > 1:
                    accs = [accs[u] + accs[u + 1] if u + 1 < len(accs) else accs[u] for u in range(0, len(accs), 2)]
                acc = accs[0]
                gd[1, c, b, pl.ds(GH + t0 + rc, crc), :] = acc.reshape(crc, 128)
                a1 = jnp.sum(acc, axis=0)
                a2 = jnp.sum(acc * acc, axis=0)
                if rc == 0:
                    st[c] = (a1, a2)
                else:
                    st[c] = (st[c][0] + a1, st[c][1] + a2)
                if rc + crc == TM:
                    s1, s2 = st[c]
                    if valid is not None:
                        s1 = jnp.where(valid, s1, 0.0)
                        s2 = jnp.where(valid, s2, 0.0)
                    stat[0, :, cs] += s1
                    stat[1, :, cs] += s2

            return [functools.partial(piece, c, rc) for c in range(ND) for rc in range(0, TM, crc)]

        def conv_pieces_by_col(i):
            p_ = conv_pieces(i)
            n_ = TM // crc
            return [p_[c * n_:(c + 1) * n_] for c in range(ND)]

        def conv(i):
            for p_ in conv_pieces(i):
                p_()

        nq = TM // erc

        def lsum(r, j, rs):
            t = lane_fold(_un(pbuf[rs.start // 2:rs.stop // 2, kslice(j)]).astype(F32), jnp.add)
            if j == 0:
                lbuf[r, rs, :] = t
            else:
                lbuf[r, rs, :] += t

        def exp_piece(r, z, m, j, q, seed):
            rs = slice(q * erc, (q + 1) * erc)
            if seed is not None:
                sbuf[r, pl.ds(pl.multiple_of(TM + 8 * z, 8), 8), 0:128] = seed
            p = jnp.exp2(sbuf[r, rs, kslice(j)] - m[rs])
            pk = _pk(p.astype(BF16))
            pbuf[rs.start // 2:rs.stop // 2, kslice(j)] = pk
            if lmode == "mem":
                lsum(r, j, rs)
            else:
                t = lane_fold(_un(pk).astype(F32) if lmode.startswith("val") else p, jnp.add)
                sl = r + z if (j % 2 and lmode.endswith("pin")) else r
                if j == 0:
                    lbuf[sl, rs, :] = t
                else:
                    lbuf[sl, rs, :] += t

        def spread(t, items, phase):
            n = len(items)
            for q, f in enumerate(items):
                f(seed_of(t, (q * ND * TM) // n + phase * (ND * TM) // (2 * n)))

        def b_tile(i, r, w, do_next=True, conv_on=True):
            b, _ = bt(i)
            pcs = []
            if conv_on and do_conv:
                if isinstance(i, int):
                    if i >= 2:
                        pcs = conv_pieces(i - 2)
                else:
                    pcs = conv_pieces(clamp_lo(i - 2), valid=(i >= 2))
            tail_cols = None
            if not do_next and fold_conv and do_conv:
                p1, p0 = conv_pieces_by_col(i - 1), conv_pieces_by_col(i)
                pcs = pcs + [f_ for c in range(ND) for f_ in p1[c][:-1]]
                tail_cols = [[p1[c][-1]] + p0[c] for c in range(ND)]
            m = mbuf[r]
            z = zdyn
            eps_ = {j: [functools.partial(exp_piece, r, z, m, j, q) for q in range(nq)] for j in range(NKC)}
            plan = list(cplan) if do_next else [0] * qk_split + list(cplan_last) + [0] * (NKC - qk_split) + [0, 0]
            tot = sum(plan)
            npcs = len(pcs)
            cum = [0]
            for v in plan:
                cum.append(cum[-1] + v)
            site = [0]

            def release(t, exps=()):
                k0 = site[0]
                site[0] += 1
                n = (cum[k0 + 1] * npcs) // tot - (cum[k0] * npcs) // tot if npcs else 0
                items = [(q * ND * TM // n + ND * TM // (2 * n), 1, pcs.pop(0)) for q in range(n)]
                ne = len(exps)
                items += [(q * ND * TM // ne, 0, f_) for q, f_ in enumerate(exps)]
                items.sort(key=lambda u: u[:2])
                for tpos, _k, f_ in items:
                    f_(seed_of(t, tpos))

            mp = None
            if do_next:
                for j in range(qk_split):
                    t, raw = b_qk(i + 1, j, w)
                    mp = t if mp is None else jnp.maximum(mp, t)
                    release(raw, eps_[0] if j == qk_split - 1 - e0pos else ())
            else:
                site[0] = qk_split
                for f_ in eps_[0]:
                    f_(None)
            o = None
            for j in range(NKC):
                t = _dot(_un(pbuf[:, kslice(j)]), _un(vbuf[b, hslice(j), :]))
                o = t if o is None else o + t
                release(t, eps_[j + 1] if j + 1 < NKC else ())
            l = jnp.sum(lbuf[r], axis=-1, keepdims=True)
            res[rows(i), :] = res[rows(i), :] + o * (1.0 / l)
            r0 = i * TM if isinstance(i, int) else pl.multiple_of(i * TM, 16)

            def lnb(q, seed):
                if seed is not None:
                    res[pl.ds(pl.multiple_of(B * T + 8 * z, 8), 8), 0:128] = seed
                xnA[q * brc // 2:(q + 1) * brc // 2, :] = _pk(_ln(res[pl.ds(r0 + q * brc, brc), :], 0.5).astype(BF16))
            lps = [functools.partial(lnb, q) for q in range(TM // brc)]
            if do_next:
                for j in range(qk_split, NKC):
                    t, raw = b_qk(i + 1, j, w)
                    mp = t if mp is None else jnp.maximum(mp, t)
                    k_ = j - qk_split
                    if k_ < len(lplan):
                        n_ = lplan[k_]
                        release(raw, [functools.partial(lambda f_, sd: f_(sd), lps.pop(0)) for _ in range(n_)])
                    else:
                        release(raw)
                assert not lps
            else:
                site[0] = NKC + NKC
                for f_ in lps:
                    f_(None)
            xn = _un(xnA[...])
            bb, t0 = bt(i)
            if do_next or not fold_conv:
                a_ = _dot(xn, wp1[:, :D])
                release(a_)
                b_ = _dot(xn, wp1[:, D:])
                release(b_)
                g = a_ * (1.0 + jnp.tanh(b_))
                for c in range(ND):
                    gd[0, c, bb, pl.ds(GH + t0, TM), :] = g[:, c * 128:(c + 1) * 128]
            else:
                prev = []
                for c in range(ND):
                    cs = slice(c * 128, (c + 1) * 128)
                    wab = jnp.concatenate([wp1[:, cs], wp1[:, D + c * 128:D + (c + 1) * 128]], axis=1)
                    ab = _dot(xn, wab)
                    for q, f_ in enumerate(prev):
                        f_(seed_of(ab, (2 * TM * q) // len(prev)))
                    gd[0, c, bb, pl.ds(GH + t0, TM), :] = ab[:, :128] * (1.0 + jnp.tanh(ab[:, 128:]))
                    prev = tail_cols[c]
                for f_ in prev:
                    f_(None)
            assert not pcs
            if do_next:
                mbuf[w] = jnp.max(mp, axis=-1, keepdims=True)

        if "B" in phases:
            scx = scope("s_5aBpro"); scx.__enter__()
            mp = None
            for j in range(NKC):
                t, _ = b_qk(0, j, 0)
                mp = t if mp is None else jnp.maximum(mp, t)
            mbuf[0] = jnp.max(mp, axis=-1, keepdims=True)
            scx.__exit__(None, None, None)

            def b_iter(i, _):
                r = lax.rem(i, 2)
                b_tile(i, r, 1 - r)
            with scope("s_5bBloop"):
                lax.fori_loop(0, NTT - 1, b_iter, None)
            with scope("s_5cBlast"):
                b_tile(NTT - 1, (NTT - 1) % 2, NTT % 2, do_next=False)
            if do_conv and not fold_conv:
                with scope("s_5dconv"):
                    lax.fori_loop(NTT - 2, NTT, lambda i_, _: conv(i_), None)

        scd = scope("s_6aDpro"); scd.__enter__()
        n = float(B * T)
        mu = jnp.sum(stat[0], axis=0, keepdims=True) / n
        var = jnp.maximum(jnp.sum(stat[1], axis=0, keepdims=True) / n - mu * mu, 0.0)
        hr = 0.5 * lax.rsqrt(var + EPS)

        wc[8].wait()
        wc[9].wait()
        wc[10].wait()

        def ocopy(i, slot):
            return pltpu.make_async_copy(obuf.at[slot], o_hbm.at[rows(i)], osem.at[slot])

        def d_act_pieces(i, a_w):
            b, t0 = bt(i)
            z = zdyn

            def piece(q, seed):
                if seed is not None:
                    gd[0, 0, B - 1, pl.ds(pl.multiple_of(T + 2 * GH + 8 * z, 8), 8), :] = seed
                dcv = jnp.concatenate([gd[1, c, b, pl.ds(GH + t0 + q * drc, drc), :] for c in range(ND)], axis=1)
                a_w[q * drc // 2:(q + 1) * drc // 2, :] = _pk(_half_silu((dcv - mu) * hr).astype(BF16))
            return [functools.partial(piece, q) for q in range(TM // drc)]

        def d_act(i, a_w):
            for p_ in d_act_pieces(i, a_w):
                p_(None)

        def d_fin_pieces(i, g_r, slot):
            z = zdyn

            def piece(q, seed):
                if seed is not None:
                    g_r[pl.ds(pl.multiple_of(TM + 8 * z, 8), 8), 0:128] = seed
                rs = slice(q * drc, (q + 1) * drc)
                obuf[slot, rs, :] = _ln(g_r[rs, :], 1.0).astype(BF16)
            return [functools.partial(piece, q) for q in range(TM // drc)]

        def d_pw2(i, a_r, f_w, xn_w, seeded=True):
            f_w[0:TM, :] = res[rows(i), :] + _dot(_un(a_r[...]), wp2[...])
            z = zdyn

            def piece(q, seed):
                if seed is not None:
                    f_w[pl.ds(pl.multiple_of(TM + 8 * z, 8), 8), 0:128] = seed
                rs = slice(q * drc, (q + 1) * drc)
                xn_w[q * drc // 2:(q + 1) * drc // 2, :] = _pk(_ln(f_w[rs, :], 0.5).astype(BF16))
            pieces = [functools.partial(piece, q) for q in range(TM // drc)]
            if seeded:
                return pieces
            for f_ in pieces:
                f_(None)

        def d_fin(x4, slot):
            obuf[slot] = _ln(x4, 1.0).astype(BF16)

        def d_half(i, slot, a_r, a_w, f_r, f_w, xn_r, xn_w, g_r, g_w):
            fins = d_fin_pieces(i, g_r, slot)
            acts = d_act_pieces(clamp_hi(i + 2), a_w)
            mix = []
            for q in range(max(len(fins), len(acts))):
                mix += fins[q:q + 1] + acts[q:q + 1]
            rel = Releaser(mix, dplan, exact=True)
            y = None
            for c in range(NF):
                if c == d_split:
                    lnp = d_pw2(clamp_hi(i + 1), a_r, f_w, xn_w)
                    rel.pieces = lnp + rel.pieces
                t = ff_chunk(xn_r, w2a, w2b, c, rel)
                y = t if y is None else y + t
            g_w[0:TM, :] = f_r[0:TM, :] + 0.5 * y

        if "D" in phases:
            gB[...] = jnp.zeros(gB.shape, F32)
            d_act(0, hA)
            d_pw2(0, hA, fA, xnA, seeded=False)
            d_act(1, hB)

            def d_pair(p, _):
                i = 2 * p
                sb = 2 * lax.rem(p, 2)

                @pl.when(p >= 2)
                def _():
                    ocopy(i - 4, sb).wait()

                @pl.when(p >= 3)
                def _():
                    ocopy(i - 5, sb + 1).wait()
                d_half(i, sb + 1, hB, hA, fA, fB, xnA, xnB, gB, gA)
                d_half(i + 1, sb, hA, hB, fB, fA, xnB, xnA, gA, gB)

                @pl.when(p >= 1)
                def _():
                    ocopy(i - 1, sb + 1).start()
                ocopy(i, sb).start()
            scd.__exit__(None, None, None)
            with scope("s_6bDloop"):
                lax.fori_loop(0, NTT // 2, d_pair, None)
            scd = scope("s_6cDepi"); scd.__enter__()
            P = NTT // 2

            def oslot(t):
                pp = (t + 1) // 2
                return 2 * (pp % 2) + (t % 2)
            ocopy(NTT - 5, oslot(NTT - 5)).wait()
            d_fin(gB[0:TM, :], oslot(NTT - 5))
            ocopy(NTT - 1, oslot(NTT - 5)).start()
            for t in (NTT - 4, NTT - 3, NTT - 2):
                ocopy(t, oslot(t)).wait()
            ocopy(NTT - 1, oslot(NTT - 5)).wait()
        else:
            obuf[0] = x_v[0:TM, :].astype(obuf.dtype)
            ocopy(0, 0).start()
            ocopy(0, 0).wait()
        scd.__exit__(None, None, None)

    def fn(x, w_ff1_a, w_ff1_b, w_q, w_k, w_v, w_o, w_pw1, dw, w_pw2, w_ff2_a, w_ff2_b):
        x2 = x.reshape(B * T, D)
        any_spec = pl.BlockSpec(memory_space=pl.ANY)
        V = pltpu.VMEM
        out = pl.pallas_call(
            kernel,
            out_shape=jax.ShapeDtypeStruct((B * T, D), BF16),
            in_specs=[any_spec] * 12,
            out_specs=any_spec,
            scratch_shapes=[
                V((B * T + 16, D), BF16),
                V((D, F), BF16), V((F, D), BF16),
                V((D, D), BF16), V((D, D), BF16), V((D, D), BF16), V((D, D), BF16),
                V((D, 2 * D), BF16), V((K, D), BF16), V((D, D), BF16),
                V((D, F), BF16), V((F, D), BF16),
                V((D // 2, 2 * D), U32),
                V((K, 8, D), F32),
                V((B * T + 16, D), F32),
                V((B * T // 2, D), U32),
                V((B, TP // 2, D), U32), V((B, TP // 2, D), U32),
                V((2, ND, B, T + 2 * GH + 16, 128), F32),
                V((2, TM + 8, TP), F32),
                V((TM // 2, TP), U32),
                V((2, TM, 128), F32),
                V((2, TM, 1), F32),
                V((2, TM // 2, D), U32), V((2, TM // 2, D), U32),
                V((TM // 2, D), U32), V((TM // 2, D), U32),
                V((TM // 2, D), U32), V((TM // 2, D), U32),
                V((TM + 16, D), F32), V((TM + 16, D), F32),
                V((TM + 16, D), F32), V((TM + 16, D), F32),
                V((2, 8, D), F32),
                V((4, TM, D), BF16),
                pltpu.SemaphoreType.DMA((4,)),
                pltpu.SemaphoreType.DMA((11 + 2 * NF,)),
                pltpu.SemaphoreType.DMA((4,)),
            ],
            compiler_params=pltpu.CompilerParams(vmem_limit_bytes=127 * 1024 * 1024),
        )(x2, w_ff1_a, w_ff1_b, w_q, w_k, w_v, w_o, w_pw1, dw, w_pw2, w_ff2_a, w_ff2_b)
        return out.reshape(B, T, D)

    return fn


@jax.jit
def pallas_standalone__conformer_family_conformer__speech_kernel(
    x, w_ff1_a, w_ff1_b, w_q, w_k, w_v, w_o, w_pw1, dw, w_pw2, w_ff2_a, w_ff2_b):
    B, T, D = x.shape
    K = dw.shape[0]
    F = w_ff1_a.shape[1]
    return make_kernel(B, T, D, K, F)(
        x, w_ff1_a, w_ff1_b, w_q, w_k, w_v, w_o, w_pw1, dw, w_pw2, w_ff2_a, w_ff2_b)
```

```python
import functools
import math
import numpy as np

import jax
import jax.numpy as jnp
from jax import lax
import jax.experimental.pallas as pl
import jax.experimental.pallas.tpu as pltpu

F32 = jnp.float32
BF16 = jnp.bfloat16
EPS = 1e-5
LOG2E = 1.4426950408889634


def _ln(xf, post):
    m = jnp.mean(xf, axis=-1, keepdims=True)
    xc = xf - m
    v = jnp.mean(xc * xc, axis=-1, keepdims=True)
    r = lax.rsqrt(v + EPS)
    if post != 1.0:
        r = r * post
    return xc * r


def _half_silu(h):
    return h * (1.0 + jnp.tanh(h))


U32 = jnp.uint32


def _pk(v):
    return pltpu.bitcast(v, U32)


def _un(v):
    return pltpu.bitcast(v, BF16)


def _dot(a, b):
    return jnp.dot(a, b, preferred_element_type=F32)


def _dot_nt(a, b):
    return lax.dot_general(a, b, (((1,), (1,)), ((), ())), preferred_element_type=F32)


def make_kernel(B, T, D, K, F, TM=400, phases="ABD", ffc=512, prewait=False, kc=512, qk_split=5,
                border="alpha", crc=16, cacc=2, brc=16, lplan=(10,10,5), lmode='mem', cmode='roll', fold_conv=True, aseed=True, dq=1, aplan0=(0,0,0,0,2,2,1), arc=80, arc2=80, ln2span=2000, aplan=(1,1,1,1,1), dseed=True, drc=16, dplan=(10,10,10,10,10,10,10,5), cplan=(0,0,0,0,0, 1,1,1,1,1,1,1,1, 0,0,0, 0,0), cplan_last=(1,1,1,1,1,1,1,1), do_conv=True, d_split=2, erc=16, qk_tail=0, e0pos=1, brep=0, dbg_aligned=False, dbg_taps=15, scopes=False):
    TP = (T + 127) // 128 * 128
    NT = T // TM
    NTT = B * NT
    assert NTT % 2 == 0 and NTT >= 6
    PAD = K // 2
    GH = 8
    scale = D ** -0.5
    NKC = TP // kc
    ND = D // 128
    NF = F // ffc

    def kernel(x_hbm, w1a_hbm, w1b_hbm, wq_hbm, wk_hbm, wv_hbm, wo_hbm, wp1_hbm, dw_hbm, wp2_hbm,
               w2a_hbm, w2b_hbm, o_hbm,
               x_v, w1a, w1b, wq, wk, wv, wo, wp1, dw_v, wp2, w2a, w2b, wqv, dwb,
               res, qbuf, kbuf, vbuf, gd,
               sbuf, pbuf, lbuf, mbuf, xnS, hS, xnA, xnB, hA, hB, fA, fB, gA, gB, stat, obuf,
               xsem, wsem, osem):
        def rows(i):
            if isinstance(i, int):
                return pl.ds(i * TM, TM)
            return pl.ds(pl.multiple_of(i * TM, 16), TM)

        def hrows(i):
            if isinstance(i, int):
                return pl.ds(i * (TM // 2), TM // 2)
            return pl.ds(pl.multiple_of(i * (TM // 2), 8), TM // 2)

        def bt(i):
            if isinstance(i, int):
                return i // NT, (i % NT) * TM
            b = lax.div(i, NT)
            return b, pl.multiple_of((i - b * NT) * TM, 16)

        def clamp_hi(i):
            if isinstance(i, int):
                return min(i, NTT - 1)
            return jnp.minimum(i, NTT - 1)

        def clamp_lo(i):
            if isinstance(i, int):
                return max(i, 0)
            return jnp.maximum(i, 0)

        def xcp(t0_, t1_, k_):
            return pltpu.make_async_copy(x_hbm.at[pl.ds(t0_ * TM, (t1_ - t0_) * TM)],
                                         x_v.at[pl.ds(t0_ * TM, (t1_ - t0_) * TM)], xsem.at[k_])
        xc0, xc1, xc2, xc3 = xcp(0, 1, 0), xcp(1, 2, 1), xcp(2, 4, 2), xcp(4, NTT, 3)
        wlist = [(wq_hbm, wq), (wk_hbm, wk), (wv_hbm, wv), (wo_hbm, wo), (w1a_hbm, w1a), (w1b_hbm, w1b),
                 (wp1_hbm, wp1), (dw_hbm, dw_v), (wp2_hbm, wp2), (w2a_hbm, w2a), (w2b_hbm, w2b)]
        wc = [pltpu.make_async_copy(s_, d_, wsem.at[j]) for j, (s_, d_) in enumerate(wlist)]
        w1ac = [pltpu.make_async_copy(w1a_hbm.at[:, cs_], w1a.at[:, cs_], wsem.at[11 + c])
                for c in range(NF) for cs_ in [pl.ds(c * ffc, ffc)]]
        w1bc = [pltpu.make_async_copy(w1b_hbm.at[cs_, :], w1b.at[cs_, :], wsem.at[11 + NF + c])
                for c in range(NF) for cs_ in [pl.ds(c * ffc, ffc)]]

        def scope(name):
            class _S:
                def __enter__(self_):
                    if scopes: self_.s = jax.named_scope(name); self_.s.__enter__()
                def __exit__(self_, *a):
                    if scopes: self_.s.__exit__(*a)
            return _S()

        sc0 = scope("s_0start"); sc0.__enter__()
        zdyn = lax.fori_loop(0, 2, lambda i_, c_: c_ + lax.shift_right_logical(i_, 20), jnp.int32(0))
        late = wc[6:11]
        if not prewait:
            xc0.start()
            w1ac[0].start()
            if dq == 0:
                w1bc[0].start()
        else:
            for c_ in [xc0, xc1, xc2, xc3] + w1ac + w1bc + wc[:4] + wc[6:]:
                c_.start()

        if prewait:
            allc = [xc0, xc1, xc2, xc3] + w1ac + w1bc + wc[:4] + wc[6:]
            for c_ in allc:
                c_.wait()

            class _C:
                def wait(self): pass
                def start(self): pass
            wc = [_C() for _ in range(11)]
            late = []
            xc0 = xc1 = xc2 = xc3 = _C()
            w1ac = [_C() for _ in range(NF)]
            w1bc = [_C() for _ in range(NF)]

        for b in range(B):
            kbuf[b, T // 2:TP // 2, :] = jnp.zeros(((TP - T) // 2, D), U32)
            vbuf[b, T // 2:TP // 2, :] = jnp.zeros(((TP - T) // 2, D), U32)
            for c in range(ND):
                gd[0, c, b, 0:GH, :] = jnp.zeros((GH, 128), F32)
                gd[0, c, b, GH + T:GH + T + GH, :] = jnp.zeros((GH, 128), F32)
        stat[...] = jnp.zeros(stat.shape, F32)

        def seed_of(t, tpos):
            n_, r_ = tpos // TM, (tpos % TM) // 8 * 8
            return t[r_:r_ + 8, n_ * 128:(n_ + 1) * 128]

        class Releaser:
            def __init__(self, pieces, plan, exact=False):
                self.pieces, self.cum, self.k = list(pieces), np.cumsum([0] + list(plan)), 0
                self.n = int(self.cum[-1]) if exact else len(self.pieces)

            def __call__(self, t):
                k0 = self.k
                self.k += 1
                if self.k >= len(self.cum):
                    return
                tot = int(self.cum[-1])
                n = int(self.cum[k0 + 1]) * self.n // tot - int(self.cum[k0]) * self.n // tot
                span = t.shape[1] // 128 * TM
                for q in range(n):
                    self.pieces.pop(0)(seed_of(t, (2 * q + 1) * span // (2 * n)))

        def ff_chunk(xn_ref, wa, wb, c, rel=None):
            h = _dot(_un(xn_ref[...]), wa[:, c * ffc:(c + 1) * ffc])
            if rel is not None:
                rel(h)
            a = _half_silu(h).astype(BF16)
            y = _dot(a, wb[c * ffc:(c + 1) * ffc, :])
            if rel is not None:
                rel(y)
            return y

        def a_ln1(i, sl):
            xnS[sl] = _pk(_ln(x_v[rows(i), :].astype(F32), 0.5).astype(BF16))

        def a_ln1_pieces(i, sl, first_wait=None):
            z = zdyn
            r0 = i * TM if isinstance(i, int) else pl.multiple_of(i * TM, 16)

            def piece(q, seed):
                if q == 0 and first_wait is not None:
                    first_wait.wait()
                if seed is not None:
                    x_v[pl.ds(pl.multiple_of(B * T + 16 * z, 16), 16), 0:128] = pltpu.bitcast(seed, BF16)
                rs = pl.ds(r0 + q * arc, arc)
                xnS[sl, q * arc // 2:(q + 1) * arc // 2, :] = _pk(_ln(x_v[rs, :].astype(F32), 0.5).astype(BF16))
            return [functools.partial(piece, q) for q in range(TM // arc)]

        def a_ff(i, sl, rel, waits=False, mid=None):
            y = None
            for c in range(NF):
                if waits:
                    w1ac[c].wait()
                    startq()
                h = _dot(_un(xnS[sl]), w1a[:, c * ffc:(c + 1) * ffc])
                rel(h)
                a = _half_silu(h).astype(BF16)
                if waits:
                    w1bc[c].wait()
                    startq()
                t = _dot(a, w1b[c * ffc:(c + 1) * ffc, :])
                rel(t)
                y = t if y is None else y + t
            res[rows(i), :] = x_v[rows(i), :].astype(F32) + 0.5 * y
            b, t0 = bt(i)
            h0 = t0 // 2 if isinstance(t0, int) else pl.multiple_of(lax.shift_right_logical(t0, 1), 8)
            z = zdyn
            r0 = i * TM if isinstance(i, int) else pl.multiple_of(i * TM, 16)

            def ln2(q, seed):
                if seed is not None:
                    res[pl.ds(pl.multiple_of(B * T + 8 * z, 8), 8), 0:128] = seed
                hn = _pk(_ln(res[pl.ds(r0 + q * arc2, arc2), :], 1.0).astype(BF16))
                kbuf[b, pl.ds(h0 + q * arc2 // 2, arc2 // 2), :] = hn
                hS[sl, q * arc2 // 2:(q + 1) * arc2 // 2, :] = hn
            pieces = [functools.partial(ln2, q) for q in range(TM // arc2)]
            if mid is not None:
                t = mid()
                for q, f_ in enumerate(pieces):
                    f_(seed_of(t, ln2span * q // len(pieces)))
            else:
                for f_ in pieces:
                    f_(None)

        def a_qv(i, hn):
            b, t0 = bt(i)
            raw = _dot(_un(hn), _un(wqv[...]))
            qv = _pk(raw.astype(BF16))
            h0 = t0 // 2 if isinstance(t0, int) else pl.multiple_of(lax.shift_right_logical(t0, 1), 8)
            qbuf[hrows(i), :] = qv[:, :D]
            vbuf[b, pl.ds(h0, TM // 2), :] = qv[:, D:]
            return raw

        if dq == 0:
            queue = [[w1ac[1]], [w1bc[1], xc1]]
            for c in range(2, NF):
                queue += [[w1ac[c]], [w1bc[c]]]
        elif dq == 1:
            queue = [[w1bc[0], w1ac[1]], [w1bc[1], xc1]]
            for c in range(2, NF):
                queue += [[w1ac[c]], [w1bc[c]]]
        elif dq == 2:
            queue = [[w1bc[0]], [w1ac[1], w1bc[1]], [w1ac[2], xc1]]
            for c in range(2, NF - 1):
                queue += [[w1bc[c]], [w1ac[c + 1]]]
            queue += [[w1bc[NF - 1]]]
        elif dq == 3:
            queue = [[w1bc[0], w1ac[1]], [w1bc[1], w1ac[2]], [xc1, w1bc[2]], [w1ac[3]], [w1bc[3]]]
        queue += [[wc[0], wc[1]], [wc[2], wc[3]], [xc2]]

        def startq():
            if queue:
                for c_ in queue.pop(0):
                    c_.start()

        xc0.wait()
        startq()
        a_ln1(0, 0)
        sc0.__exit__(None, None, None)
        if "A" in phases:
            with scope("s_1a0"):
                a_ff(0, 0, Releaser(a_ln1_pieces(1, 1, first_wait=xc1), aplan0), waits=True)
                while queue:
                    startq()
                xc2.wait()

            def a_iter(i, _):
                @pl.when(i == 1)
                def _():
                    wc[0].wait()
                    wc[1].wait()
                    wc[2].wait()
                    wc[3].wait()
                    xc3.start()
                    wqv[:, :D] = _pk((_dot_nt(wq[...], wk[...]) * (scale * LOG2E)).astype(BF16))
                    wqv[:, D:] = _pk(_dot(wv[...], wo[...]).astype(BF16))

                @pl.when(i == 3)
                def _():
                    xc3.wait()
                    for c_ in late:
                        c_.start()
                sl = lax.rem(i, 2)
                a_ff(i, sl, Releaser(a_ln1_pieces(clamp_hi(i + 1), 1 - sl), aplan),
                     mid=lambda: a_qv(i - 1, hS[1 - sl]))
            with scope("s_3aloop"):
                lax.fori_loop(1, NTT, a_iter, None)
            with scope("s_4alast"):
                a_qv(NTT - 1, hS[(NTT - 1) % 2])
        else:
            if not prewait:
                while queue:
                    startq()
                for c_ in [xc3] + late:
                    c_.start()
            for c_ in [xc1, xc2, xc3] + w1ac + w1bc + wc[:4]:
                c_.wait()

        wc[6].wait()
        wc[7].wait()
        for k in range(K):
            dwb[k] = jnp.broadcast_to(dw_v[k:k + 1, :].astype(F32), (8, D))

        def kslice(j):
            return slice(j * kc, (j + 1) * kc)

        def hslice(j):
            return slice(j * kc // 2, (j + 1) * kc // 2)

        def lane_fold(v, op):
            r = v[:, 0:128]
            for c in range(1, v.shape[1] // 128):
                r = op(r, v[:, c * 128:(c + 1) * 128])
            return r

        def b_qk(i, j, w):
            b, _ = bt(i)
            s = _dot_nt(_un(qbuf[hrows(i), :]), _un(kbuf[b, hslice(j), :]))
            raw = s
            if (j + 1) * kc > T:
                col = lax.broadcasted_iota(jnp.int32, (TM, kc), 1)
                s = jnp.where(col < (T - j * kc), s, -jnp.inf)
            sbuf[w, 0:TM, kslice(j)] = s
            return lane_fold(s, jnp.maximum), raw

        def b_glu(i, xn):
            b, t0 = bt(i)
            ab = _dot(xn, wp1[...])
            g = ab[:, :D] * (1.0 + jnp.tanh(ab[:, D:]))
            for c in range(ND):
                gd[0, c, b, pl.ds(GH + t0, TM), :] = g[:, c * 128:(c + 1) * 128]

        def conv_pieces(i, valid=None):
            b, t0 = bt(i)
            st = {}

            def piece(c, rc, seed=None):
                cs = slice(c * 128, (c + 1) * 128)
                if seed is not None:
                    gd[1, 0, b, pl.ds(pl.multiple_of(8 * zdyn, 8), 8), :] = seed
                nv = crc // 8
                if cmode == "unaligned":
                    accs = [None] * cacc
                    for k in range(K):
                        w = dwb[k, :, cs]
                        t = gd[0, c, b, pl.ds(t0 + GH - PAD + k + rc, crc), :]
                        t = t.reshape(crc // 8, 8, 128) * w[None]
                        accs[k % cacc] = t if accs[k % cacc] is None else accs[k % cacc] + t
                    while len(accs) > 1:
                        accs = [accs[u] + accs[u + 1] if u + 1 < len(accs) else accs[u] for u in range(0, len(accs), 2)]
                    acc = accs[0]
                else:
                    A = [gd[0, c, b, pl.ds(t0 + rc + 8 * m_, 8), :] for m_ in range(nv + 2)]
                    sub = lax.broadcasted_iota(jnp.int32, (8, 128), 0)
                    terms = [[A[v_ + 1] * dwb[PAD, :, cs]] for v_ in range(nv)]
                    for r_ in range(1, 8):
                        R = [pltpu.roll(x_, 8 - r_, 0) for x_ in A]
                        Sh = [jnp.where(sub < 8 - r_, R[m_], R[m_ + 1]) for m_ in range(nv + 1)]
                        for v_ in range(nv):
                            terms[v_].append(Sh[v_ + 1] * dwb[PAD + r_, :, cs])
                            terms[v_].append(Sh[v_] * dwb[PAD + r_ - 8, :, cs])
                    outs = []
                    for v_ in range(nv):
                        l_ = [None] * cacc
                        for u_, x_ in enumerate(terms[v_]):
                            l_[u_ % cacc] = x_ if l_[u_ % cacc] is None else l_[u_ % cacc] + x_
                        while len(l_) > 1:
                            l_ = [l_[u] + l_[u + 1] if u + 1 < len(l_) else l_[u] for u in range(0, len(l_), 2)]
                        outs.append(l_[0])
                    acc = jnp.stack(outs)
                gd[1, c, b, pl.ds(GH + t0 + rc, crc), :] = acc.reshape(crc, 128)
                a1 = jnp.sum(acc, axis=0)
                a2 = jnp.sum(acc * acc, axis=0)
                if rc == 0:
                    st[c] = (a1, a2)
                else:
                    st[c] = (st[c][0] + a1, st[c][1] + a2)
                if rc + crc == TM:
                    s1, s2 = st[c]
                    if valid is not None:
                        s1 = jnp.where(valid, s1, 0.0)
                        s2 = jnp.where(valid, s2, 0.0)
                    stat[0, :, cs] += s1
                    stat[1, :, cs] += s2

            return [functools.partial(piece, c, rc) for c in range(ND) for rc in range(0, TM, crc)]

        def conv_pieces_by_col(i):
            p_ = conv_pieces(i)
            n_ = TM // crc
            return [p_[c * n_:(c + 1) * n_] for c in range(ND)]

        def conv(i):
            for p_ in conv_pieces(i):
                p_()

        nq = TM // erc

        def lsum(r, j, rs):
            t = lane_fold(_un(pbuf[rs.start // 2:rs.stop // 2, kslice(j)]).astype(F32), jnp.add)
            if j == 0:
                lbuf[r, rs, :] = t
            else:
                lbuf[r, rs, :] += t

        def exp_piece(r, z, m, j, q, seed):
            rs = slice(q * erc, (q + 1) * erc)
            if seed is not None:
                sbuf[r, pl.ds(pl.multiple_of(TM + 8 * z, 8), 8), 0:128] = seed
            p = jnp.exp2(sbuf[r, rs, kslice(j)] - m[rs])
            pk = _pk(p.astype(BF16))
            pbuf[rs.start // 2:rs.stop // 2, kslice(j)] = pk
            if lmode == "mem":
                lsum(r, j, rs)
            else:
                t = lane_fold(_un(pk).astype(F32) if lmode.startswith("val") else p, jnp.add)
                sl = r + z if (j % 2 and lmode.endswith("pin")) else r
                if j == 0:
                    lbuf[sl, rs, :] = t
                else:
                    lbuf[sl, rs, :] += t

        def spread(t, items, phase):
            n = len(items)
            for q, f in enumerate(items):
                f(seed_of(t, (q * ND * TM) // n + phase * (ND * TM) // (2 * n)))

        def b_tile(i, r, w, do_next=True, conv_on=True):
            b, _ = bt(i)
            pcs = []
            if conv_on and do_conv:
                if isinstance(i, int):
                    if i >= 2:
                        pcs = conv_pieces(i - 2)
                else:
                    pcs = conv_pieces(clamp_lo(i - 2), valid=(i >= 2))
            tail_cols = None
            if not do_next and fold_conv and do_conv:
                p1, p0 = conv_pieces_by_col(i - 1), conv_pieces_by_col(i)
                pcs = pcs + [f_ for c in range(ND) for f_ in p1[c][:-1]]
                tail_cols = [[p1[c][-1]] + p0[c] for c in range(ND)]
            m = mbuf[r]
            z = zdyn
            eps_ = {j: [functools.partial(exp_piece, r, z, m, j, q) for q in range(nq)] for j in range(NKC)}
            plan = list(cplan) if do_next else [0] * qk_split + list(cplan_last) + [0] * (NKC - qk_split) + [0, 0]
            tot = sum(plan)
            npcs = len(pcs)
            cum = [0]
            for v in plan:
                cum.append(cum[-1] + v)
            site = [0]

            def release(t, exps=()):
                k0 = site[0]
                site[0] += 1
                n = (cum[k0 + 1] * npcs) // tot - (cum[k0] * npcs) // tot if npcs else 0
                items = [(q * ND * TM // n + ND * TM // (2 * n), 1, pcs.pop(0)) for q in range(n)]
                ne = len(exps)
                items += [(q * ND * TM // ne, 0, f_) for q, f_ in enumerate(exps)]
                items.sort(key=lambda u: u[:2])
                for tpos, _k, f_ in items:
                    f_(seed_of(t, tpos))

            mp = None
            if do_next:
                for j in range(qk_split):
                    t, raw = b_qk(i + 1, j, w)
                    mp = t if mp is None else jnp.maximum(mp, t)
                    release(raw, eps_[0] if j == qk_split - 1 - e0pos else ())
            else:
                site[0] = qk_split
                for f_ in eps_[0]:
                    f_(None)
            o = None
            for j in range(NKC):
                t = _dot(_un(pbuf[:, kslice(j)]), _un(vbuf[b, hslice(j), :]))
                o = t if o is None else o + t
                release(t, eps_[j + 1] if j + 1 < NKC else ())
            l = jnp.sum(lbuf[r], axis=-1, keepdims=True)
            res[rows(i), :] = res[rows(i), :] + o * (1.0 / l)
            r0 = i * TM if isinstance(i, int) else pl.multiple_of(i * TM, 16)

            def lnb(q, seed):
                if seed is not None:
                    res[pl.ds(pl.multiple_of(B * T + 8 * z, 8), 8), 0:128] = seed
                xnA[q * brc // 2:(q + 1) * brc // 2, :] = _pk(_ln(res[pl.ds(r0 + q * brc, brc), :], 0.5).astype(BF16))
            lps = [functools.partial(lnb, q) for q in range(TM // brc)]
            if do_next:
                for j in range(qk_split, NKC):
                    t, raw = b_qk(i + 1, j, w)
                    mp = t if mp is None else jnp.maximum(mp, t)
                    k_ = j - qk_split
                    if k_ < len(lplan):
                        n_ = lplan[k_]
                        release(raw, [functools.partial(lambda f_, sd: f_(sd), lps.pop(0)) for _ in range(n_)])
                    else:
                        release(raw)
                assert not lps
            else:
                site[0] = NKC + NKC
                for f_ in lps:
                    f_(None)
            xn = _un(xnA[...])
            bb, t0 = bt(i)
            if do_next or not fold_conv:
                a_ = _dot(xn, wp1[:, :D])
                release(a_)
                b_ = _dot(xn, wp1[:, D:])
                release(b_)
                g = a_ * (1.0 + jnp.tanh(b_))
                for c in range(ND):
                    gd[0, c, bb, pl.ds(GH + t0, TM), :] = g[:, c * 128:(c + 1) * 128]
            else:
                prev = []
                for c in range(ND):
                    cs = slice(c * 128, (c + 1) * 128)
                    wab = jnp.concatenate([wp1[:, cs], wp1[:, D + c * 128:D + (c + 1) * 128]], axis=1)
                    ab = _dot(xn, wab)
                    for q, f_ in enumerate(prev):
                        f_(seed_of(ab, (2 * TM * q) // len(prev)))
                    gd[0, c, bb, pl.ds(GH + t0, TM), :] = ab[:, :128] * (1.0 + jnp.tanh(ab[:, 128:]))
                    prev = tail_cols[c]
                for f_ in prev:
                    f_(None)
            assert not pcs
            if do_next:
                mbuf[w] = jnp.max(mp, axis=-1, keepdims=True)

        if "B" in phases:
            scx = scope("s_5aBpro"); scx.__enter__()
            mp = None
            for j in range(NKC):
                t, _ = b_qk(0, j, 0)
                mp = t if mp is None else jnp.maximum(mp, t)
            mbuf[0] = jnp.max(mp, axis=-1, keepdims=True)
            scx.__exit__(None, None, None)

            def b_iter(i, _):
                r = lax.rem(i, 2)
                b_tile(i, r, 1 - r)
            with scope("s_5bBloop"):
                lax.fori_loop(0, NTT - 1, b_iter, None)
            with scope("s_5cBlast"):
                b_tile(NTT - 1, (NTT - 1) % 2, NTT % 2, do_next=False)
            if do_conv and not fold_conv:
                with scope("s_5dconv"):
                    lax.fori_loop(NTT - 2, NTT, lambda i_, _: conv(i_), None)

        scd = scope("s_6aDpro"); scd.__enter__()
        n = float(B * T)
        mu = jnp.sum(stat[0], axis=0, keepdims=True) / n
        var = jnp.maximum(jnp.sum(stat[1], axis=0, keepdims=True) / n - mu * mu, 0.0)
        hr = 0.5 * lax.rsqrt(var + EPS)

        wc[8].wait()
        wc[9].wait()
        wc[10].wait()

        def ocopy(i, slot):
            return pltpu.make_async_copy(obuf.at[slot], o_hbm.at[rows(i)], osem.at[slot])

        def d_act_pieces(i, a_w):
            b, t0 = bt(i)
            z = zdyn

            def piece(q, seed):
                if seed is not None:
                    gd[0, 0, B - 1, pl.ds(pl.multiple_of(T + 2 * GH + 8 * z, 8), 8), :] = seed
                dcv = jnp.concatenate([gd[1, c, b, pl.ds(GH + t0 + q * drc, drc), :] for c in range(ND)], axis=1)
                a_w[q * drc // 2:(q + 1) * drc // 2, :] = _pk(_half_silu((dcv - mu) * hr).astype(BF16))
            return [functools.partial(piece, q) for q in range(TM // drc)]

        def d_act(i, a_w):
            for p_ in d_act_pieces(i, a_w):
                p_(None)

        def d_fin_pieces(i, g_r, slot):
            z = zdyn

            def piece(q, seed):
                if seed is not None:
                    g_r[pl.ds(pl.multiple_of(TM + 8 * z, 8), 8), 0:128] = seed
                rs = slice(q * drc, (q + 1) * drc)
                obuf[slot, rs, :] = _ln(g_r[rs, :], 1.0).astype(BF16)
            return [functools.partial(piece, q) for q in range(TM // drc)]

        def d_pw2(i, a_r, f_w, xn_w, seeded=True):
            f_w[0:TM, :] = res[rows(i), :] + _dot(_un(a_r[...]), wp2[...])
            z = zdyn

            def piece(q, seed):
                if seed is not None:
                    f_w[pl.ds(pl.multiple_of(TM + 8 * z, 8), 8), 0:128] = seed
                rs = slice(q * drc, (q + 1) * drc)
                xn_w[q * drc // 2:(q + 1) * drc // 2, :] = _pk(_ln(f_w[rs, :], 0.5).astype(BF16))
            pieces = [functools.partial(piece, q) for q in range(TM // drc)]
            if seeded:
                return pieces
            for f_ in pieces:
                f_(None)

        def d_fin(x4, slot):
            obuf[slot] = _ln(x4, 1.0).astype(BF16)

        def d_half(i, slot, a_r, a_w, f_r, f_w, xn_r, xn_w, g_r, g_w):
            fins = d_fin_pieces(i, g_r, slot)
            acts = d_act_pieces(clamp_hi(i + 2), a_w)
            mix = []
            for q in range(max(len(fins), len(acts))):
                mix += fins[q:q + 1] + acts[q:q + 1]
            rel = Releaser(mix, dplan, exact=True)
            y = None
            for c in range(NF):
                if c == d_split:
                    lnp = d_pw2(clamp_hi(i + 1), a_r, f_w, xn_w)
                    rel.pieces = lnp + rel.pieces
                t = ff_chunk(xn_r, w2a, w2b, c, rel)
                y = t if y is None else y + t
            g_w[0:TM, :] = f_r[0:TM, :] + 0.5 * y

        if "D" in phases:
            gB[...] = jnp.zeros(gB.shape, F32)
            d_act(0, hA)
            d_pw2(0, hA, fA, xnA, seeded=False)
            d_act(1, hB)

            def d_pair(p, _):
                i = 2 * p
                sb = 2 * lax.rem(p, 2)

                @pl.when(p >= 2)
                def _():
                    ocopy(i - 4, sb).wait()

                @pl.when(p >= 3)
                def _():
                    ocopy(i - 5, sb + 1).wait()
                d_half(i, sb + 1, hB, hA, fA, fB, xnA, xnB, gB, gA)
                d_half(i + 1, sb, hA, hB, fB, fA, xnB, xnA, gA, gB)

                @pl.when(p >= 1)
                def _():
                    ocopy(i - 1, sb + 1).start()
                ocopy(i, sb).start()
            scd.__exit__(None, None, None)
            with scope("s_6bDloop"):
                lax.fori_loop(0, NTT // 2, d_pair, None)
            scd = scope("s_6cDepi"); scd.__enter__()
            P = NTT // 2

            def oslot(t):
                pp = (t + 1) // 2
                return 2 * (pp % 2) + (t % 2)
            ocopy(NTT - 5, oslot(NTT - 5)).wait()
            d_fin(gB[0:TM, :], oslot(NTT - 5))
            ocopy(NTT - 1, oslot(NTT - 5)).start()
            for t in (NTT - 4, NTT - 3, NTT - 2):
                ocopy(t, oslot(t)).wait()
            ocopy(NTT - 1, oslot(NTT - 5)).wait()
        else:
            obuf[0] = x_v[0:TM, :].astype(obuf.dtype)
            ocopy(0, 0).start()
            ocopy(0, 0).wait()
        scd.__exit__(None, None, None)

    def fn(x, w_ff1_a, w_ff1_b, w_q, w_k, w_v, w_o, w_pw1, dw, w_pw2, w_ff2_a, w_ff2_b):
        x2 = x.reshape(B * T, D)
        any_spec = pl.BlockSpec(memory_space=pl.ANY)
        V = pltpu.VMEM
        out = pl.pallas_call(
            kernel,
            out_shape=jax.ShapeDtypeStruct((B * T, D), BF16),
            in_specs=[any_spec] * 12,
            out_specs=any_spec,
            scratch_shapes=[
                V((B * T + 16, D), BF16),
                V((D, F), BF16), V((F, D), BF16),
                V((D, D), BF16), V((D, D), BF16), V((D, D), BF16), V((D, D), BF16),
                V((D, 2 * D), BF16), V((K, D), BF16), V((D, D), BF16),
                V((D, F), BF16), V((F, D), BF16),
                V((D // 2, 2 * D), U32),
                V((K, 8, D), F32),
                V((B * T + 16, D), F32),
                V((B * T // 2, D), U32),
                V((B, TP // 2, D), U32), V((B, TP // 2, D), U32),
                V((2, ND, B, T + 2 * GH + 16, 128), F32),
                V((2, TM + 8, TP), F32),
                V((TM // 2, TP), U32),
                V((2, TM, 128), F32),
                V((2, TM, 1), F32),
                V((2, TM // 2, D), U32), V((2, TM // 2, D), U32),
                V((TM // 2, D), U32), V((TM // 2, D), U32),
                V((TM // 2, D), U32), V((TM // 2, D), U32),
                V((TM + 16, D), F32), V((TM + 16, D), F32),
                V((TM + 16, D), F32), V((TM + 16, D), F32),
                V((2, 8, D), F32),
                V((4, TM, D), BF16),
                pltpu.SemaphoreType.DMA((4,)),
                pltpu.SemaphoreType.DMA((11 + 2 * NF,)),
                pltpu.SemaphoreType.DMA((4,)),
            ],
            compiler_params=pltpu.CompilerParams(vmem_limit_bytes=127 * 1024 * 1024),
        )(x2, w_ff1_a, w_ff1_b, w_q, w_k, w_v, w_o, w_pw1, dw, w_pw2, w_ff2_a, w_ff2_b)
        return out.reshape(B, T, D)

    return fn


@jax.jit
def pallas_standalone__conformer_family_conformer__speech_kernel(
    x, w_ff1_a, w_ff1_b, w_q, w_k, w_v, w_o, w_pw1, dw, w_pw2, w_ff2_a, w_ff2_b):
    B, T, D = x.shape
    K = dw.shape[0]
    F = w_ff1_a.shape[1]
    return make_kernel(B, T, D, K, F)(
        x, w_ff1_a, w_ff1_b, w_q, w_k, w_v, w_o, w_pw1, dw, w_pw2, w_ff2_a, w_ff2_b)
```

```python
import functools

import jax
import jax.numpy as jnp
import numpy as np
from jax import lax
import jax.experimental.pallas as pl
import jax.experimental.pallas.tpu as pltpu

F32 = jnp.float32
BF16 = jnp.bfloat16
U32 = jnp.uint32
EPS = 1e-5
LOG2E = 1.4426950408889634

TM = 400
FFC = 512
KC = 512
QK_SPLIT = 5
GH = 8
CRC = 16
ERC = 16
ARC = 80
BRC = 16
DRC = 16
A_PLAN0 = (0, 0, 0, 2, 1, 1, 1)
A_PLAN = (1, 1, 1, 1, 1)
A_LN2_SPAN = 2000
B_LN_PLAN = (10, 10, 5)
B_CONV_PLAN = (0, 0, 0, 0, 0, 1, 1, 1, 1, 1, 1, 1, 1, 0, 0, 0, 0, 0)
B_CONV_PLAN_LAST = (1, 1, 1, 1, 1, 1, 1, 1)
D_PLAN = (10, 10, 10, 10, 10, 10, 10, 5)
D_SPLIT = 2


def _ln(xf, post):
    m = jnp.mean(xf, axis=-1, keepdims=True)
    xc = xf - m
    v = jnp.mean(xc * xc, axis=-1, keepdims=True)
    r = lax.rsqrt(v + EPS)
    if post != 1.0:
        r = r * post
    return xc * r


def _half_silu(h):
    return h * (1.0 + jnp.tanh(h))


def _pk(v):
    return pltpu.bitcast(v, U32)


def _un(v):
    return pltpu.bitcast(v, BF16)


def _dot(a, b):
    return jnp.dot(a, b, preferred_element_type=F32)


def _dot_nt(a, b):
    return lax.dot_general(a, b, (((1,), (1,)), ((), ())), preferred_element_type=F32)


def _lane_fold(v, op):
    r = v[:, 0:128]
    for c in range(1, v.shape[1] // 128):
        r = op(r, v[:, c * 128:(c + 1) * 128])
    return r


def _seed_of(t, tpos):
    n_, r_ = tpos // TM, (tpos % TM) // 8 * 8
    return t[r_:r_ + 8, n_ * 128:(n_ + 1) * 128]


class _Releaser:
    def __init__(self, pieces, plan, exact=False):
        self.pieces, self.cum, self.k = list(pieces), np.cumsum([0] + list(plan)), 0
        self.n = int(self.cum[-1]) if exact else len(self.pieces)

    def __call__(self, t):
        k0 = self.k
        self.k += 1
        if self.k >= len(self.cum):
            return
        tot = int(self.cum[-1])
        n = int(self.cum[k0 + 1]) * self.n // tot - int(self.cum[k0]) * self.n // tot
        span = t.shape[1] // 128 * TM
        for q in range(n):
            self.pieces.pop(0)(_seed_of(t, (2 * q + 1) * span // (2 * n)))


def make_kernel(B, T, D, K, F, **_unused):
    TP = (T + KC - 1) // KC * KC
    NT = T // TM
    NTT = B * NT
    PAD = K // 2
    NKC = TP // KC
    ND = D // 128
    NF = F // FFC
    NQ = TM // ERC
    scale = D ** -0.5
    assert T % TM == 0 and NTT % 2 == 0 and NTT >= 8 and NT >= 3
    assert K == 15 and D == 512 and F % FFC == 0 and NF == 4 and NKC == 8

    def kernel(x_hbm, w1a_hbm, w1b_hbm, wq_hbm, wk_hbm, wv_hbm, wo_hbm, wp1_hbm, dw_hbm, wp2_hbm,
               w2a_hbm, w2b_hbm, o_hbm,
               x_v, w1a, w1b, wq, wk, wv, wo, wp1, dw_v, wp2, w2a, w2b, wqv, dwb,
               res, qbuf, kbuf, vbuf, gd,
               sbuf, pbuf, lbuf, mbuf, xnS, hS, xnA, xnB, hA, hB, fA, fB, gA, gB, stat, obuf,
               xsem, wsem, osem):
        def rows(i):
            if isinstance(i, int):
                return pl.ds(i * TM, TM)
            return pl.ds(pl.multiple_of(i * TM, 16), TM)

        def row0(i):
            return i * TM if isinstance(i, int) else pl.multiple_of(i * TM, 16)

        def hrows(i):
            if isinstance(i, int):
                return pl.ds(i * (TM // 2), TM // 2)
            return pl.ds(pl.multiple_of(i * (TM // 2), 8), TM // 2)

        def bt(i):
            if isinstance(i, int):
                return i // NT, (i % NT) * TM
            b = lax.div(i, NT)
            return b, pl.multiple_of((i - b * NT) * TM, 16)

        def half(t0):
            return t0 // 2 if isinstance(t0, int) else pl.multiple_of(lax.shift_right_logical(t0, 1), 8)

        def clamp_hi(i):
            return min(i, NTT - 1) if isinstance(i, int) else jnp.minimum(i, NTT - 1)

        def pad8(base):
            return pl.ds(pl.multiple_of(base + 8 * zdyn, 8), 8)

        def xcp(t0_, t1_, k_):
            return pltpu.make_async_copy(x_hbm.at[pl.ds(t0_ * TM, (t1_ - t0_) * TM)],
                                         x_v.at[pl.ds(t0_ * TM, (t1_ - t0_) * TM)], xsem.at[k_])

        xc0, xc1, xc2, xc3 = xcp(0, 1, 0), xcp(1, 2, 1), xcp(2, 4, 2), xcp(4, NTT, 3)
        wlist = [(wq_hbm, wq), (wk_hbm, wk), (wv_hbm, wv), (wo_hbm, wo),
                 (wp1_hbm, wp1), (dw_hbm, dw_v), (wp2_hbm, wp2), (w2a_hbm, w2a), (w2b_hbm, w2b)]
        wc = [pltpu.make_async_copy(s_, d_, wsem.at[j]) for j, (s_, d_) in enumerate(wlist)]
        w1ac = [pltpu.make_async_copy(w1a_hbm.at[:, pl.ds(c * FFC, FFC)], w1a.at[:, pl.ds(c * FFC, FFC)],
                                      wsem.at[9 + c]) for c in range(NF)]
        w1bc = [pltpu.make_async_copy(w1b_hbm.at[pl.ds(c * FFC, FFC), :], w1b.at[pl.ds(c * FFC, FFC), :],
                                      wsem.at[9 + NF + c]) for c in range(NF)]
        xc0.start()
        w1ac[0].start()
        queue = [[w1bc[0], w1ac[1]], [w1bc[1], w1ac[2]], [xc1, w1bc[2]], [w1ac[3]], [w1bc[3]],
                 [wc[0], wc[1]], [wc[2], wc[3]], [xc2]]

        def startq():
            if queue:
                for c_ in queue.pop(0):
                    c_.start()

        zdyn = lax.fori_loop(0, 2, lambda i_, c_: c_ + lax.shift_right_logical(i_, 20), jnp.int32(0))

        for b in range(B):
            kbuf[b, T // 2:TP // 2, :] = jnp.zeros(((TP - T) // 2, D), U32)
            vbuf[b, T // 2:TP // 2, :] = jnp.zeros(((TP - T) // 2, D), U32)
            for c in range(ND):
                gd[0, c, b, 0:GH, :] = jnp.zeros((GH, 128), F32)
                gd[0, c, b, GH + T:GH + T + GH, :] = jnp.zeros((GH, 128), F32)
        stat[...] = jnp.zeros(stat.shape, F32)

        def a_ln1_pieces(i, sl, first_wait=None):
            r0 = row0(i)

            def piece(q, seed):
                if q == 0 and first_wait is not None:
                    first_wait.wait()
                if seed is not None:
                    x_v[pl.ds(pl.multiple_of(B * T + 16 * zdyn, 16), 16), 0:128] = pltpu.bitcast(seed, BF16)
                xf = x_v[pl.ds(r0 + q * ARC, ARC), :].astype(F32)
                xnS[sl, q * ARC // 2:(q + 1) * ARC // 2, :] = _pk(_ln(xf, 0.5).astype(BF16))
            return [functools.partial(piece, q) for q in range(TM // ARC)]

        def a_qv(i, hn):
            b, t0 = bt(i)
            raw = _dot(_un(hn), _un(wqv[...]))
            qv = _pk(raw.astype(BF16))
            qbuf[hrows(i), :] = qv[:, :D]
            vbuf[b, pl.ds(half(t0), TM // 2), :] = qv[:, D:]
            return raw

        def a_ff(i, sl, rel, waits=False, mid=None):
            y = None
            for c in range(NF):
                if waits:
                    w1ac[c].wait()
                    startq()
                h = _dot(_un(xnS[sl]), w1a[:, c * FFC:(c + 1) * FFC])
                rel(h)
                a = _half_silu(h).astype(BF16)
                if waits:
                    w1bc[c].wait()
                    startq()
                t = _dot(a, w1b[c * FFC:(c + 1) * FFC, :])
                rel(t)
                y = t if y is None else y + t
            res[rows(i), :] = x_v[rows(i), :].astype(F32) + 0.5 * y
            b, t0 = bt(i)
            h0, r0 = half(t0), row0(i)

            def ln2(q, seed):
                if seed is not None:
                    res[pad8(B * T), 0:128] = seed
                hn = _pk(_ln(res[pl.ds(r0 + q * ARC, ARC), :], 1.0).astype(BF16))
                kbuf[b, pl.ds(h0 + q * ARC // 2, ARC // 2), :] = hn
                hS[sl, q * ARC // 2:(q + 1) * ARC // 2, :] = hn
            n2 = TM // ARC
            if mid is not None:
                t = mid()
                for q in range(n2):
                    ln2(q, _seed_of(t, A_LN2_SPAN * q // n2))
            else:
                for q in range(n2):
                    ln2(q, None)

        xc0.wait()
        startq()
        xnS[0] = _pk(_ln(x_v[rows(0), :].astype(F32), 0.5).astype(BF16))
        a_ff(0, 0, _Releaser(a_ln1_pieces(1, 1, first_wait=xc1), A_PLAN0), waits=True)
        while queue:
            startq()
        xc2.wait()

        def a_iter(i, _):
            @pl.when(i == 1)
            def _():
                for j in range(4):
                    wc[j].wait()
                xc3.start()
                wqv[:, :D] = _pk((_dot_nt(wq[...], wk[...]) * (scale * LOG2E)).astype(BF16))
                wqv[:, D:] = _pk(_dot(wv[...], wo[...]).astype(BF16))

            @pl.when(i == 3)
            def _():
                xc3.wait()
                for c_ in wc[4:]:
                    c_.start()
            sl = lax.rem(i, 2)
            a_ff(i, sl, _Releaser(a_ln1_pieces(clamp_hi(i + 1), 1 - sl), A_PLAN),
                 mid=lambda: a_qv(i - 1, hS[1 - sl]))

        lax.fori_loop(1, NTT, a_iter, None)
        a_qv(NTT - 1, hS[(NTT - 1) % 2])

        wc[4].wait()
        wc[5].wait()
        for k in range(K):
            dwb[k] = jnp.broadcast_to(dw_v[k:k + 1, :].astype(F32), (8, D))

        def kslice(j):
            return slice(j * KC, (j + 1) * KC)

        def hslice(j):
            return slice(j * KC // 2, (j + 1) * KC // 2)

        def b_qk(i, j, w):
            b, _ = bt(i)
            s = _dot_nt(_un(qbuf[hrows(i), :]), _un(kbuf[b, hslice(j), :]))
            raw = s
            if (j + 1) * KC > T:
                col = lax.broadcasted_iota(jnp.int32, (TM, KC), 1)
                s = jnp.where(col < (T - j * KC), s, -jnp.inf)
            sbuf[w, 0:TM, kslice(j)] = s
            return _lane_fold(s, jnp.maximum), raw

        def conv_pieces(i, valid=None):
            b, t0 = bt(i)
            st = {}

            def piece(c, rc, seed=None):
                cs = slice(c * 128, (c + 1) * 128)
                if seed is not None:
                    gd[1, 0, b, pad8(0), :] = seed
                nv = CRC // 8
                A = [gd[0, c, b, pl.ds(t0 + rc + 8 * m_, 8), :] for m_ in range(nv + 2)]
                sub = lax.broadcasted_iota(jnp.int32, (8, 128), 0)
                terms = [[A[v + 1] * dwb[PAD, :, cs]] for v in range(nv)]
                for r_ in range(1, 8):
                    R = [pltpu.roll(a_, 8 - r_, 0) for a_ in A]
                    Sh = [jnp.where(sub < 8 - r_, R[m_], R[m_ + 1]) for m_ in range(nv + 1)]
                    for v in range(nv):
                        terms[v].append(Sh[v + 1] * dwb[PAD + r_, :, cs])
                        terms[v].append(Sh[v] * dwb[PAD + r_ - 8, :, cs])
                outs = []
                for v in range(nv):
                    e_, o_ = terms[v][0], terms[v][1]
                    for u in range(2, K):
                        if u % 2:
                            o_ = o_ + terms[v][u]
                        else:
                            e_ = e_ + terms[v][u]
                    outs.append(e_ + o_)
                acc = jnp.stack(outs)
                gd[1, c, b, pl.ds(GH + t0 + rc, CRC), :] = acc.reshape(CRC, 128)
                a1 = jnp.sum(acc, axis=0)
                a2 = jnp.sum(acc * acc, axis=0)
                st[c] = (a1, a2) if rc == 0 else (st[c][0] + a1, st[c][1] + a2)
                if rc + CRC == TM:
                    s1, s2 = st[c]
                    if valid is not None:
                        s1 = jnp.where(valid, s1, 0.0)
                        s2 = jnp.where(valid, s2, 0.0)
                    stat[0, :, cs] += s1
                    stat[1, :, cs] += s2

            return [[functools.partial(piece, c, rc) for rc in range(0, TM, CRC)] for c in range(ND)]

        def exp_piece(r, m, j, q, seed):
            rs = slice(q * ERC, (q + 1) * ERC)
            hs = slice(q * ERC // 2, (q + 1) * ERC // 2)
            if seed is not None:
                sbuf[r, pad8(TM), 0:128] = seed
            p = jnp.exp2(sbuf[r, rs, kslice(j)] - m[rs])
            pbuf[hs, kslice(j)] = _pk(p.astype(BF16))
            t = _lane_fold(_un(pbuf[hs, kslice(j)]).astype(F32), jnp.add)
            if j == 0:
                lbuf[r, rs, :] = t
            else:
                lbuf[r, rs, :] += t

        def b_tile(i, r, w, last=False):
            b, t0 = bt(i)
            tail_cols = None
            if last:
                p2, p1, p0 = conv_pieces(i - 2), conv_pieces(i - 1), conv_pieces(i)
                pcs = [f_ for col in p2 for f_ in col] + [f_ for col in p1 for f_ in col[:-1]]
                tail_cols = [[p1[c][-1]] + p0[c] for c in range(ND)]
                plan = [0] * QK_SPLIT + list(B_CONV_PLAN_LAST) + [0] * (NKC - QK_SPLIT) + [0, 0]
            else:
                pcs = [f_ for col in conv_pieces(jnp.maximum(i - 2, 0), valid=(i >= 2)) for f_ in col]
                plan = list(B_CONV_PLAN)
            m = mbuf[r]
            exps = [[functools.partial(exp_piece, r, m, j, q) for q in range(NQ)] for j in range(NKC)]
            cum = np.cumsum([0] + plan)
            tot, npcs, site = int(cum[-1]), len(pcs), [0]

            def release(t, extra=()):
                k0 = site[0]
                site[0] += 1
                n = int(cum[k0 + 1]) * npcs // tot - int(cum[k0]) * npcs // tot
                span = ND * TM
                items = [(q * span // n + span // (2 * n), 1, pcs.pop(0)) for q in range(n)]
                items += [(q * span // len(extra), 0, f_) for q, f_ in enumerate(extra)]
                items.sort(key=lambda u: u[:2])
                for tpos, _k, f_ in items:
                    f_(_seed_of(t, tpos))

            mp = None
            if last:
                site[0] = QK_SPLIT
                for f_ in exps[0]:
                    f_(None)
            else:
                for j in range(QK_SPLIT):
                    t, raw = b_qk(i + 1, j, w)
                    mp = t if mp is None else jnp.maximum(mp, t)
                    release(raw, exps[0] if j == QK_SPLIT - 2 else ())
            o = None
            for j in range(NKC):
                t = _dot(_un(pbuf[:, kslice(j)]), _un(vbuf[b, hslice(j), :]))
                o = t if o is None else o + t
                release(t, exps[j + 1] if j + 1 < NKC else ())
            l = jnp.sum(lbuf[r], axis=-1, keepdims=True)
            res[rows(i), :] = res[rows(i), :] + o * (1.0 / l)
            r0 = row0(i)

            def lnb(q, seed):
                if seed is not None:
                    res[pad8(B * T), 0:128] = seed
                xnA[q * BRC // 2:(q + 1) * BRC // 2, :] = _pk(_ln(res[pl.ds(r0 + q * BRC, BRC), :], 0.5).astype(BF16))
            lps = [functools.partial(lnb, q) for q in range(TM // BRC)]
            if last:
                site[0] = 2 * NKC
                for f_ in lps:
                    f_(None)
            else:
                for j in range(QK_SPLIT, NKC):
                    t, raw = b_qk(i + 1, j, w)
                    mp = t if mp is None else jnp.maximum(mp, t)
                    release(raw, [lps.pop(0) for _ in range(B_LN_PLAN[j - QK_SPLIT])])
                assert not lps
            xn = _un(xnA[...])
            if last:
                prev = []
                for c in range(ND):
                    cs = slice(c * 128, (c + 1) * 128)
                    ab = _dot(xn, jnp.concatenate([wp1[:, cs], wp1[:, D + c * 128:D + (c + 1) * 128]], axis=1))
                    for q, f_ in enumerate(prev):
                        f_(_seed_of(ab, (2 * TM * q) // len(prev)))
                    gd[0, c, b, pl.ds(GH + t0, TM), :] = ab[:, :128] * (1.0 + jnp.tanh(ab[:, 128:]))
                    prev = tail_cols[c]
                for f_ in prev:
                    f_(None)
            else:
                a_ = _dot(xn, wp1[:, :D])
                release(a_)
                b_ = _dot(xn, wp1[:, D:])
                release(b_)
                g = a_ * (1.0 + jnp.tanh(b_))
                for c in range(ND):
                    gd[0, c, b, pl.ds(GH + t0, TM), :] = g[:, c * 128:(c + 1) * 128]
                mbuf[w] = jnp.max(mp, axis=-1, keepdims=True)
            assert not pcs

        mp0 = None
        for j in range(NKC):
            t_, _ = b_qk(0, j, 0)
            mp0 = t_ if mp0 is None else jnp.maximum(mp0, t_)
        mbuf[0] = jnp.max(mp0, axis=-1, keepdims=True)

        def b_iter(i, _):
            r = lax.rem(i, 2)
            b_tile(i, r, 1 - r)

        lax.fori_loop(0, NTT - 1, b_iter, None)
        b_tile(NTT - 1, (NTT - 1) % 2, NTT % 2, last=True)

        n_rows = float(B * T)
        mu = jnp.sum(stat[0], axis=0, keepdims=True) / n_rows
        var = jnp.maximum(jnp.sum(stat[1], axis=0, keepdims=True) / n_rows - mu * mu, 0.0)
        hr = 0.5 * lax.rsqrt(var + EPS)

        wc[6].wait()
        wc[7].wait()
        wc[8].wait()

        def ocopy(i, slot):
            return pltpu.make_async_copy(obuf.at[slot], o_hbm.at[rows(i)], osem.at[slot])

        def d_act_pieces(i, a_w):
            b, t0 = bt(i)

            def piece(q, seed):
                if seed is not None:
                    gd[0, 0, B - 1, pad8(T + 2 * GH), :] = seed
                dcv = jnp.concatenate([gd[1, c, b, pl.ds(GH + t0 + q * DRC, DRC), :] for c in range(ND)], axis=1)
                a_w[q * DRC // 2:(q + 1) * DRC // 2, :] = _pk(_half_silu((dcv - mu) * hr).astype(BF16))
            return [functools.partial(piece, q) for q in range(TM // DRC)]

        def d_fin_pieces(g_r, slot):
            def piece(q, seed):
                if seed is not None:
                    g_r[pad8(TM), 0:128] = seed
                rs = slice(q * DRC, (q + 1) * DRC)
                obuf[slot, rs, :] = _ln(g_r[rs, :], 1.0).astype(BF16)
            return [functools.partial(piece, q) for q in range(TM // DRC)]

        def d_pw2(i, a_r, f_w, xn_w):
            f_w[0:TM, :] = res[rows(i), :] + _dot(_un(a_r[...]), wp2[...])

            def piece(q, seed):
                if seed is not None:
                    f_w[pad8(TM), 0:128] = seed
                xn_w[q * DRC // 2:(q + 1) * DRC // 2, :] = _pk(_ln(f_w[q * DRC:(q + 1) * DRC, :], 0.5).astype(BF16))
            return [functools.partial(piece, q) for q in range(TM // DRC)]

        def d_half(i, slot, a_r, a_w, f_r, f_w, xn_r, xn_w, g_r, g_w):
            mix = []
            for f_, a_ in zip(d_fin_pieces(g_r, slot), d_act_pieces(clamp_hi(i + 2), a_w)):
                mix += [f_, a_]
            rel = _Releaser(mix, D_PLAN, exact=True)
            y = None
            for c in range(NF):
                if c == D_SPLIT:
                    rel.pieces = d_pw2(clamp_hi(i + 1), a_r, f_w, xn_w) + rel.pieces
                h = _dot(_un(xn_r[...]), w2a[:, c * FFC:(c + 1) * FFC])
                rel(h)
                t = _dot(_half_silu(h).astype(BF16), w2b[c * FFC:(c + 1) * FFC, :])
                rel(t)
                y = t if y is None else y + t
            g_w[0:TM, :] = f_r[0:TM, :] + 0.5 * y

        gB[...] = jnp.zeros(gB.shape, F32)
        for f_ in d_act_pieces(0, hA):
            f_(None)
        for f_ in d_pw2(0, hA, fA, xnA):
            f_(None)
        for f_ in d_act_pieces(1, hB):
            f_(None)

        def d_pair(p, _):
            i = 2 * p
            sb = 2 * lax.rem(p, 2)

            @pl.when(p >= 2)
            def _():
                ocopy(i - 4, sb).wait()

            @pl.when(p >= 3)
            def _():
                ocopy(i - 5, sb + 1).wait()
            d_half(i, sb + 1, hB, hA, fA, fB, xnA, xnB, gB, gA)
            d_half(i + 1, sb, hA, hB, fB, fA, xnB, xnA, gA, gB)

            @pl.when(p >= 1)
            def _():
                ocopy(i - 1, sb + 1).start()
            ocopy(i, sb).start()

        lax.fori_loop(0, NTT // 2, d_pair, None)

        def oslot(t):
            return 2 * (((t + 1) // 2) % 2) + (t % 2)
        fs = oslot(NTT - 5)
        ocopy(NTT - 5, fs).wait()
        obuf[fs] = _ln(gB[0:TM, :], 1.0).astype(BF16)
        ocopy(NTT - 1, fs).start()
        for t_ in (NTT - 4, NTT - 3, NTT - 2):
            ocopy(t_, oslot(t_)).wait()
        ocopy(NTT - 1, fs).wait()

    def fn(x, w_ff1_a, w_ff1_b, w_q, w_k, w_v, w_o, w_pw1, dw, w_pw2, w_ff2_a, w_ff2_b):
        any_spec = pl.BlockSpec(memory_space=pl.ANY)
        V = pltpu.VMEM
        out = pl.pallas_call(
            kernel,
            out_shape=jax.ShapeDtypeStruct((B * T, D), BF16),
            in_specs=[any_spec] * 12,
            out_specs=any_spec,
            scratch_shapes=[
                V((B * T + 16, D), BF16),
                V((D, F), BF16), V((F, D), BF16),
                V((D, D), BF16), V((D, D), BF16), V((D, D), BF16), V((D, D), BF16),
                V((D, 2 * D), BF16), V((K, D), BF16), V((D, D), BF16),
                V((D, F), BF16), V((F, D), BF16),
                V((D // 2, 2 * D), U32),
                V((K, 8, D), F32),
                V((B * T + 16, D), F32),
                V((B * T // 2, D), U32),
                V((B, TP // 2, D), U32), V((B, TP // 2, D), U32),
                V((2, ND, B, T + 2 * GH + 16, 128), F32),
                V((2, TM + 8, TP), F32),
                V((TM // 2, TP), U32),
                V((2, TM, 128), F32),
                V((2, TM, 1), F32),
                V((2, TM // 2, D), U32), V((2, TM // 2, D), U32),
                V((TM // 2, D), U32), V((TM // 2, D), U32),
                V((TM // 2, D), U32), V((TM // 2, D), U32),
                V((TM + 16, D), F32), V((TM + 16, D), F32),
                V((TM + 16, D), F32), V((TM + 16, D), F32),
                V((2, 8, D), F32),
                V((4, TM, D), BF16),
                pltpu.SemaphoreType.DMA((4,)),
                pltpu.SemaphoreType.DMA((9 + 2 * NF,)),
                pltpu.SemaphoreType.DMA((4,)),
            ],
            compiler_params=pltpu.CompilerParams(vmem_limit_bytes=127 * 1024 * 1024),
        )(x.reshape(B * T, D), w_ff1_a, w_ff1_b, w_q, w_k, w_v, w_o, w_pw1, dw, w_pw2, w_ff2_a, w_ff2_b)
        return out.reshape(B, T, D)

    return fn


@jax.jit
def pallas_standalone__conformer_family_conformer__speech_kernel(
        x, w_ff1_a, w_ff1_b, w_q, w_k, w_v, w_o, w_pw1, dw, w_pw2, w_ff2_a, w_ff2_b):
    B, T, D = x.shape
    return make_kernel(B, T, D, dw.shape[0], w_ff1_a.shape[1])(
        x, w_ff1_a, w_ff1_b, w_q, w_k, w_v, w_o, w_pw1, dw, w_pw2, w_ff2_a, w_ff2_b)
```
